```python
import jax
import jax.numpy as jnp

def _softmax(x, axis=-1):
    return jax.nn.softmax(x, axis=axis)
def _gelu(x):
    return jax.nn.gelu(x, approximate=True)
def _silu(x):
    return jax.nn.silu(x)
def _sigmoid(x):
    return jax.nn.sigmoid(x)
def _layernorm(x, axis=-1, eps=1e-5):
    m = jnp.mean(x, axis=axis, keepdims=True)
    v = jnp.var(x, axis=axis, keepdims=True)
    return (x - m) / jnp.sqrt(v + eps)
def _scatter_add(tgt, idx, src, axis=0):
    return tgt.at[idx].add(src)
def _segment_sum(src, seg, n):
    return jax.ops.segment_sum(src, seg, n)
class _Rng:
    def __init__(self, key):
        self._k = key
    def _next(self):
        self._k, sub = jax.random.split(self._k)
        return sub
    def normal(self, shape):
        return jax.random.normal(self._next(), shape, dtype=jnp.bfloat16)
    def randint(self, lo, hi, shape):
        return jax.random.randint(self._next(), shape, lo, hi, dtype=jnp.int32)
    def uniform(self, shape, lo=0.0, hi=1.0):
        return jax.random.uniform(self._next(), shape, jnp.bfloat16, lo, hi)
    def permutation(self, n):
        return jax.random.permutation(self._next(), n)


kernel_name = 'interleave_layers__sliding_block_cached__dense_activation_gelu__decode'

def setup_inputs():
    _rng = _Rng(jax.random.key(int.from_bytes(__import__("os").urandom(4), "little")))
    _w = (lambda a: (lambda t: t.astype(jnp.bfloat16) if jnp.issubdtype(t.dtype, jnp.floating) else t)(jnp.asarray(a)))
    def _A_setup():
        B, Sq, D = 1, 1, 640
        Hq, Hkv, Sk, Dh = 32, 32, 32768, 192
        assert Hq % Hkv == 0, (Hq, Hkv)
        return {
            "x": _w((lambda *s: _rng.normal(s) * 0.05)(B, Sq, D)),
            "k_cache": _w((lambda *s: _rng.normal(s) * 0.05)(B, Hkv, Sk, Dh)),
            "v_cache": _w((lambda *s: _rng.normal(s) * 0.05)(B, Hkv, Sk, Dh)),
            "wq": _w((lambda *s: _rng.normal(s) * 0.05)(D, Hq * Dh) * (D ** -0.5)),
            "wo": _w((lambda *s: _rng.normal(s) * 0.05)(Hq * Dh, D) * ((Hq * Dh) ** -0.5)),
        }
    _A_in = _A_setup()

    def _B_setup():
        B, S, D, F = 1, 1, 640, 1536
        return {
            "x": _w((lambda *s: _rng.normal(s) * 0.05)(B, S, D)),
            "w1": _w((lambda *s: _rng.normal(s) * 0.05)(D, F) * (D ** -0.5)),
            "b1": _w((lambda *s: _rng.normal(s) * 0.05)(F) * 0.01),
            "w2": _w((lambda *s: _rng.normal(s) * 0.05)(F, D) * (F ** -0.5)),
            "b2": _w((lambda *s: _rng.normal(s) * 0.05)(D) * 0.01),
        }
    _B_in = _B_setup()

    return {
        "A_x": _A_in["x"],
        "A_k_cache": _A_in["k_cache"],
        "A_v_cache": _A_in["v_cache"],
        "A_wq": _A_in["wq"],
        "A_wo": _A_in["wo"],
        "B_x": _B_in["x"],
        "B_w1": _B_in["w1"],
        "B_b1": _B_in["b1"],
        "B_w2": _B_in["w2"],
        "B_b2": _B_in["b2"],
    }

def reference(A_x, A_k_cache, A_v_cache, A_wq, A_wo, B_x, B_w1, B_b1, B_w2, B_b2):
    def _A_ref(x, k_cache, v_cache, wq, wo):
        B, Sq, D = x.shape
        Hq, Dh = 32, 192
        Hkv, Sk = k_cache.shape[1], k_cache.shape[2]
        W = min(4096, max(256, Sk // 4))
        rep = Hq // Hkv
        q = (lambda x, *d: x.transpose(*d))((x @ wq).reshape(B, Sq, Hq, Dh), 0, 2, 1, 3)
        k = jnp.repeat(k_cache[:, :, Sk - W:, :], rep, axis=1)
        v = jnp.repeat(v_cache[:, :, Sk - W:, :], rep, axis=1)
        scores = jnp.einsum("bhqd,bhkd->bhqk", q, k) * (Dh ** -0.5)
        p = _softmax(scores, axis=-1)
        o = jnp.einsum("bhqk,bhkd->bhqd", p, v)
        return (lambda x, *d: x.transpose(*d))(o, 0, 2, 1, 3).reshape(B, Sq, Hq * Dh) @ wo

    def _B_ref(x, w1, b1, w2, b2):
        h = jnp.einsum("bsd,df->bsf", x, w1) + b1
        h = _gelu(h)
        return jnp.einsum("bsf,fd->bsd", h, w2) + b2

    x = A_x
    x = x + _A_ref(_layernorm(x, axis=-1), A_k_cache, A_v_cache, A_wq, A_wo)
    x = x + _B_ref(_layernorm(x, axis=-1), B_w1, B_b1, B_w2, B_b2)
    x = x + _A_ref(_layernorm(x, axis=-1), A_k_cache, A_v_cache, A_wq, A_wo)
    x = x + _B_ref(_layernorm(x, axis=-1), B_w1, B_b1, B_w2, B_b2)
    return x
```

```python
import functools
import jax
import jax.numpy as jnp
from jax import lax
import jax.experimental.pallas as pl
import jax.experimental.pallas.tpu as pltpu

D = 640
H = 32
DH = 192
F = 1536
G = 8
NG = H // G
GD = G * DH
EPS = 1e-5
bf16 = jnp.bfloat16
f32 = jnp.float32


def _ln(x):
    m = jnp.mean(x, axis=-1, keepdims=True)
    xc = x - m
    v = jnp.mean(xc * xc, axis=-1, keepdims=True)
    return xc * lax.rsqrt(v + EPS)


def _gelu(x):
    c = 0.7978845608028654
    return 0.5 * x * (1.0 + jnp.tanh(c * (x + 0.044715 * (x * x * x))))


def _make_kernel(SK, W):
    scale = DH ** -0.5

    def kernel(x_ref, k_hbm, v_hbm, wq_hbm, wo_hbm, w1_hbm, b1_ref, w2_hbm, b2_ref,
               o_ref, kbuf, vbuf, wqb, wob, w1b, w2b, sems):
        def kcopy(g):
            return pltpu.make_async_copy(
                k_hbm.at[pl.ds(g * GD, GD), pl.ds(SK - W, W)],
                kbuf.at[pl.ds(g * GD, GD), :], sems.at[4 + g])

        def vcopy(g):
            return pltpu.make_async_copy(
                v_hbm.at[pl.ds(g * GD, GD), pl.ds(SK - W, W)],
                vbuf.at[pl.ds(g * GD, GD), :], sems.at[4 + NG + g])

        cq = pltpu.make_async_copy(wq_hbm, wqb, sems.at[0])
        co = pltpu.make_async_copy(wo_hbm, wob, sems.at[1])
        c1 = pltpu.make_async_copy(w1_hbm, w1b, sems.at[2])
        c2 = pltpu.make_async_copy(w2_hbm, w2b, sems.at[3])
        cq.start()
        kcopy(0).start()
        vcopy(0).start()
        co.start()
        c1.start()
        c2.start()
        for g in range(1, NG):
            kcopy(g).start()
            vcopy(g).start()

        row = lax.broadcasted_iota(jnp.int32, (G, GD), 0)
        col = lax.broadcasted_iota(jnp.int32, (G, GD), 1)
        diag = (col >= row * DH) & (col < (row + 1) * DH)

        b1 = jnp.concatenate([b1_ref[i:i + 1, :] for i in range(F // 128)], axis=1).astype(f32)
        b2 = jnp.concatenate([b2_ref[i:i + 1, :] for i in range(D // 128)], axis=1).astype(f32)

        x = x_ref[0].astype(f32)

        def attn_group(g, xn8, acc, first):
            q = jnp.dot(xn8, wqb[:, pl.ds(pl.multiple_of(g * GD, 128), GD)], preferred_element_type=f32)
            qb = jnp.where(diag, q, 0.0).astype(bf16)
            if first:
                kcopy(g).wait()
            r0 = pl.multiple_of(g * GD, 16)
            s = jnp.dot(qb, kbuf[pl.ds(r0, GD), :], preferred_element_type=f32) * scale
            m = jnp.max(s, axis=-1, keepdims=True)
            p = jnp.exp(s - m)
            l = jnp.sum(p, axis=-1, keepdims=True)
            if first:
                vcopy(g).wait()
            o = lax.dot_general(p.astype(bf16), vbuf[pl.ds(r0, GD), :],
                                (((1,), (1,)), ((), ())), preferred_element_type=f32)
            ob = jnp.where(diag, o / l, 0.0).astype(bf16)
            if first:
                @pl.when(g == 0)
                def _():
                    co.wait()
            return acc + jnp.dot(ob, wob[pl.ds(r0, GD), :], preferred_element_type=f32)

        def layer(x, first):
            xn8 = jnp.broadcast_to(_ln(x), (G, D)).astype(bf16)
            if first:
                cq.wait()
            acc = lax.fori_loop(0, NG, lambda g, acc: attn_group(g, xn8, acc, first),
                                jnp.zeros((G, D), f32))
            x = x + jnp.sum(acc, axis=0, keepdims=True)
            xn8 = jnp.broadcast_to(_ln(x), (8, D)).astype(bf16)
            if first:
                c1.wait()
            h = jnp.dot(xn8, w1b[...], preferred_element_type=f32) + b1
            h = _gelu(h).astype(bf16)
            if first:
                c2.wait()
            y = jnp.dot(h, w2b[...], preferred_element_type=f32)
            return x + y[0:1, :] + b2

        x = layer(x, True)
        x = layer(x, False)
        o_ref[0] = x.astype(o_ref.dtype)

    return kernel


@jax.jit
def pallas_interleave_layers__sliding_block_cached__dense_activation_gelu__decode_kernel(
    A_x, A_k_cache, A_v_cache, A_wq, A_wo, B_x, B_w1, B_b1, B_w2, B_b2,
):
    SK = A_k_cache.shape[2]
    W = min(4096, max(256, SK // 4))
    kt = jnp.swapaxes(A_k_cache, 2, 3).reshape(H * DH, SK)
    vt = jnp.swapaxes(A_v_cache, 2, 3).reshape(H * DH, SK)
    b1 = B_b1.reshape(F // 128, 128)
    b2 = B_b2.reshape(D // 128, 128)
    anyspec = pl.BlockSpec(memory_space=pl.ANY)
    vmem = pl.BlockSpec(memory_space=pltpu.VMEM)
    return pl.pallas_call(
        _make_kernel(SK, W),
        out_shape=jax.ShapeDtypeStruct(A_x.shape, A_x.dtype),
        in_specs=[vmem, anyspec, anyspec, anyspec, anyspec, anyspec, vmem, anyspec, vmem],
        out_specs=vmem,
        scratch_shapes=[
            pltpu.VMEM((H * DH, W), bf16),
            pltpu.VMEM((H * DH, W), bf16),
            pltpu.VMEM((D, H * DH), bf16),
            pltpu.VMEM((H * DH, D), bf16),
            pltpu.VMEM((D, F), bf16),
            pltpu.VMEM((F, D), bf16),
            pltpu.SemaphoreType.DMA((4 + 2 * NG,)),
        ],
        compiler_params=pltpu.CompilerParams(vmem_limit_bytes=127 * 1024 * 1024),
    )(A_x, kt, vt, A_wq, A_wo, B_w1, b1, B_w2, b2)
```

```python
import functools
import jax
import jax.numpy as jnp
from jax import lax
import jax.experimental.pallas as pl
import jax.experimental.pallas.tpu as pltpu

D = 640
H = 32
DH = 192
F = 1536
G = 4
NG = H // G
GD = G * DH
RG = GD // 8
NJ = GD // 128
NT = 2 * NJ
KD = D // 128
KF = F // 128
EPS = 1e-5
LOG2E = 1.4426950408889634
bf16 = jnp.bfloat16
f32 = jnp.float32
u32 = jnp.uint32

RATE = 5.0


def _ln(x):
    m = jnp.mean(x, axis=-1, keepdims=True)
    xc = x - m
    v = jnp.mean(xc * xc, axis=-1, keepdims=True)
    return xc * lax.rsqrt(v + EPS)


def _gelu(x):
    c = 0.7978845608028654
    return 0.5 * x * (1.0 + jnp.tanh(c * (x + 0.044715 * (x * x * x))))


def _pack_rows(x8):
    x16 = jnp.concatenate([x8, jnp.zeros_like(x8)], axis=0).astype(bf16)
    return pltpu.bitcast(x16, u32)


def _tile_dot(lhs_u32, w_u32):
    return jnp.dot(pltpu.bitcast(lhs_u32, bf16), pltpu.bitcast(w_u32, bf16),
                   preferred_element_type=f32)[0:8]


def _tree_sum(xs):
    xs = list(xs)
    while len(xs) > 1:
        xs = [xs[i] + xs[i + 1] if i + 1 < len(xs) else xs[i] for i in range(0, len(xs), 2)]
    return xs[0]


def _make_kernel(SK, W):
    NCP = W // 256
    c_exp = (DH ** -0.5) * LOG2E

    def kernel(x_hbm, k_hbm, v_hbm, wq_hbm, wo_hbm, w1_hbm, b1_hbm, w2_hbm, b2_hbm,
               o_ref,
               kb, vb, wqb, wob, w1b, w2b, xin, b1v, b2v,
               xres, xl, lq, lq0, qraw, qraw0, sraw, pbuf, pd, acc_ref, ol, yraw, ysum, sems):
        ku = k_hbm.bitcast(u32)

        def kcopy(g):
            return pltpu.make_async_copy(
                ku.at[pl.ds(g * (RG // 2), RG // 2), :, pl.ds((SK - W) // 32, W // 32), :],
                kb.at[pl.ds(g * (RG // 2), RG // 2)], sems.at[8 + g])

        def vcopy(g):
            return pltpu.make_async_copy(
                v_hbm.at[pl.ds(g * RG, RG), pl.ds((SK - W) // 16, W // 16), :],
                vb.at[pl.ds(g * RG, RG)], sems.at[8 + NG + g])

        def wcopies(src, dst, sem):
            su = src.bitcast(u32)
            return [pltpu.make_async_copy(su.at[:, pl.ds(n * 128, 128)], dst.at[n], sem)
                    for n in range(dst.shape[0])]

        small = [pltpu.make_async_copy(x_hbm, xin, sems.at[0]),
                 pltpu.make_async_copy(b1_hbm, b1v, sems.at[1]),
                 pltpu.make_async_copy(b2_hbm, b2v, sems.at[2])]
        cq = wcopies(wq_hbm, wqb, sems.at[3])
        co = wcopies(wo_hbm, wob, sems.at[4])
        c1 = wcopies(w1_hbm, w1b, sems.at[5])
        c2 = wcopies(w2_hbm, w2b, sems.at[6])
        for c in small + cq + co:
            c.start()
        kcopy(0).start()
        for g in range(NG):
            if g + 1 < NG:
                kcopy(g + 1).start()
            vcopy(g).start()
        for c in c1 + c2:
            c.start()

        for c in small:
            c.wait()
        xres[...] = jnp.broadcast_to(xin[0].astype(f32), (8, D))

        def qproj_tile(wg, qr, n):
            j, kt = divmod(n, KD)
            qr[n] = _tile_dot(xl[:, pl.ds(kt * 128, 128)], wg[j, pl.ds(kt * 64, 64), :])

        def build_l(qr, lslot, j):
            row = lax.broadcasted_iota(jnp.int32, (8, 128), 0)
            lane = lax.broadcasted_iota(jnp.int32, (8, 128), 1)
            q = _tree_sum(qr[j * KD + kt] for kt in range(KD))
            qp = pltpu.roll(q, 8, 1)
            qm = pltpu.roll(q, 120, 1)
            h_lo = (j * 128) // DH
            split = (h_lo + 1) * DH - j * 128
            tgt = ((lane >> 1) & 4) + h_lo
            if split < 128:
                tgt = jnp.where(lane >= split, tgt + 1, tgt)
            hit = row == tgt
            low = row < 4
            lslot[2 * j] = _pack_rows(jnp.where(hit, jnp.where(low, q, qp), 0.0))
            lslot[2 * j + 1] = _pack_rows(jnp.where(hit, jnp.where(low, qm, q), 0.0))

        def qk_tile(kg, lslot, n):
            c4, rem = divmod(n, 4 * NT)
            t, i = divmod(rem, 4)
            cp = c4 * 4 + i
            w = kg[pl.ds((t // 2) * 8, 8), t % 2, pl.ds(cp * 8, 8), :].reshape(64, 128)
            sraw[cp, t] = _tile_dot(lslot[t], w)

        def s_sum(cp):
            return _tree_sum(sraw[cp, t] for t in range(NT))

        def s_presum(cp):
            sraw[cp, 0] = s_sum(cp)

        def softmax(npre):
            s = [sraw[cp, 0] if cp < npre else s_sum(cp) for cp in range(NCP)]
            xs = list(s)
            while len(xs) > 1:
                xs = [jnp.maximum(xs[i], xs[i + 1]) for i in range(0, len(xs), 2)]
            m = xs[0]
            m = jnp.maximum(m, pltpu.roll(m, 4, 0))
            m = jnp.max(m, axis=1, keepdims=True)
            e = [jnp.exp2((a - m) * c_exp) for a in s]
            l = _tree_sum(e)
            l = l + pltpu.roll(l, 4, 0)
            l = jnp.sum(l, axis=1, keepdims=True)
            r = 1.0 / l
            for cp in range(NCP):
                pbuf[cp] = e[cp] * r

        def reduce_o(j):
            blk = acc_ref[pl.ds(j * 16, 16)].reshape(128, 128)
            t = blk.T.reshape(16, 8, 128)
            ol[j] = _pack_rows(_tree_sum(t[i] for i in range(16)))

        def wo_tile(wg, n):
            j, nt = divmod(n, KD)
            yraw[n] = _tile_dot(ol[j], wg[nt, pl.ds(j * 64, 64), :])

        def y_fold(js):
            for nt in range(KD):
                ysum[nt] = _tree_sum([ysum[nt]] + [yraw[j * KD + nt] for j in js])

        def p_copy():
            for cp in range(NCP):
                pd[cp] = pbuf[cp]

        def layer(li, carry):
            first = li == 0
            xl[...] = _pack_rows(_ln(xres[...]))
            acc_ref[pl.ds(64, 32)] = jnp.zeros((32, 8, 128), f32)
            ol[3] = jnp.zeros((8, 128), u32)
            yraw[...] = jnp.zeros(yraw.shape, f32)
            ysum[...] = jnp.zeros(ysum.shape, f32)

            @pl.when(first)
            def _():
                for c in cq + co:
                    c.wait()
                kcopy(0).wait()

            kg0 = kb.at[pl.ds(0, RG // 2)]
            for n in range(NJ * KD):
                qproj_tile(wqb.at[pl.ds(0, NJ)], qraw0, n)
            for n in range(NJ * KD):
                qproj_tile(wqb.at[pl.ds(NJ, NJ)], qraw, n)
            for j in range(NJ):
                build_l(qraw0, lq0, j)
            for n in range(NCP * NT):
                qk_tile(kg0, lq0, n)
            for j in range(NJ):
                build_l(qraw, lq, j)
            for n in range(NJ * KD):
                qproj_tile(wqb.at[pl.ds(2 * NJ, NJ)], qraw, n)
            softmax(0)

            def block(g, hh):
                g1 = jnp.minimum(g + 1, NG - 1)
                g3 = jnp.minimum(g + 3, NG - 1)
                gm = jnp.maximum(g - 1, 0)
                if hh == 0:
                    @pl.when(first)
                    def _():
                        vcopy(g).wait()

                        @pl.when(g + 1 < NG)
                        def _():
                            kcopy(g + 1).wait()

                vg = vb.at[pl.ds(g * RG + hh * 24, 24)]
                pg = pbuf if hh < 3 else pd
                side = []
                P = functools.partial
                if hh < 3:
                    kg = kb.at[pl.ds(g1 * (RG // 2), RG // 2)]
                    for n in range(64):
                        side.append((int(n * RATE), P(qk_tile, kg, lq, hh * 64 + n)))
                else:
                    wqg = wqb.at[pl.ds(g3 * NJ, NJ)]
                    wog = wob.at[:, pl.ds(pl.multiple_of(g * (GD // 2), GD // 2), GD // 2), :]
                    wom = wob.at[:, pl.ds(pl.multiple_of(gm * (GD // 2), GD // 2), GD // 2), :]
                    for n in range(NJ * KD):
                        nn = (n + 15) % 30
                        side.append((int(n * RATE), P(wo_tile, wog if nn < 15 else wom, nn)))
                        side.append((int((n + 30) * RATE), P(qproj_tile, wqg, qraw, n)))
                if hh == 0:
                    side.append((20, P(reduce_o, 4)))
                    side.append((100, P(reduce_o, 5)))
                    side.append((200, P(y_fold, range(NJ))))
                if hh == 1:
                    side.append((20, P(reduce_o, 0)))
                    for cp in range(4):
                        side.append((100 + 40 * cp, P(s_presum, cp)))
                if hh == 2:
                    side.append((20, P(reduce_o, 1)))
                    side.append((100, P(reduce_o, 2)))
                    for cp in range(4, 8):
                        side.append((40 * cp, P(s_presum, cp)))
                    side.append((10, p_copy))
                if hh == 3:
                    side.append((0, P(softmax, 8)))
                    for j in range(NJ):
                        side.append((40 + 15 * j, P(build_l, qraw, lq, j)))
                    side.append((200, P(reduce_o, 3)))
                side.sort(key=lambda z: z[0])

                cnt = 0
                si = 0
                acc = [None] * 24
                for cp in range(NCP):
                    m0 = jnp.broadcast_to(pg[cp, pl.ds(hh, 1), :], (8, 128))
                    m1 = jnp.broadcast_to(pg[cp, pl.ds(4 + hh, 1), :], (8, 128))
                    for rg in range(24):
                        while si < len(side) and side[si][0] <= cnt:
                            side[si][1]()
                            si += 1
                        cnt += 1
                        v = vg[rg, pl.ds(cp * 16, 16), :].astype(f32)
                        if acc[rg] is None:
                            acc[rg] = v[:8] * m0 + v[8:] * m1
                        else:
                            acc[rg] = acc[rg] + v[:8] * m0 + v[8:] * m1
                        if cp == NCP - 1:
                            acc_ref[hh * 24 + rg] = acc[rg]
                while si < len(side):
                    side[si][1]()
                    si += 1

            def body(b, c):
                g = b // G
                for hh in range(G):
                    pl.when(b % G == hh)(functools.partial(block, g, hh))
                return c

            lax.fori_loop(0, H, body, 0)

            y_fold(range(NJ))
            reduce_o(4)
            reduce_o(5)
            wog = wob.at[:, pl.ds((NG - 1) * (GD // 2), GD // 2), :]
            for n in range(15, 30):
                wo_tile(wog, n)
            ys = [_tree_sum([ysum[nt]] + [yraw[j * KD + nt] for j in range(3, 6)]) for nt in range(KD)]
            y = jnp.sum(jnp.concatenate(ys, axis=1), axis=0, keepdims=True)
            x = xres[...] + y

            xn = pltpu.bitcast(_pack_rows(_ln(x)), bf16)

            @pl.when(first)
            def _():
                for c in c1:
                    c.wait()

            b1 = jnp.concatenate([b1v[i:i + 1, :] for i in range(KF)], axis=1).astype(f32)
            b2 = jnp.concatenate([b2v[i:i + 1, :] for i in range(KD)], axis=1).astype(f32)
            h = jnp.concatenate(
                [jnp.dot(xn, pltpu.bitcast(w1b[n], bf16), preferred_element_type=f32)[0:8]
                 for n in range(KF)], axis=1) + b1
            hl = pltpu.bitcast(_pack_rows(_gelu(h)), bf16)

            @pl.when(first)
            def _():
                for c in c2:
                    c.wait()

            y2 = jnp.concatenate(
                [jnp.dot(hl, pltpu.bitcast(w2b[n], bf16), preferred_element_type=f32)[0:8]
                 for n in range(KD)], axis=1)
            xres[...] = x + y2 + b2
            return carry

        lax.fori_loop(0, 2, layer, 0)
        o_ref[0] = xres[0:1, :].astype(o_ref.dtype)

    return kernel


@jax.jit
def pallas_interleave_layers__sliding_block_cached__dense_activation_gelu__decode_kernel(
    A_x, A_k_cache, A_v_cache, A_wq, A_wo, B_x, B_w1, B_b1, B_w2, B_b2,
):
    SK = A_k_cache.shape[2]
    W = min(4096, max(256, SK // 4))
    NR = H * DH // 8

    def tiled(a):
        t = jnp.swapaxes(a, 2, 3).reshape(NR, 8, SK // 128, 128)
        return t.transpose(0, 2, 1, 3).reshape(NR, SK // 16, 128)

    kt = tiled(A_k_cache).reshape(NR // 2, 2, SK // 16, 128)
    vt = tiled(A_v_cache)
    b1 = B_b1.reshape(F // 128, 128)
    b2 = B_b2.reshape(D // 128, 128)
    anyspec = pl.BlockSpec(memory_space=pl.ANY)
    NCP = W // 256
    return pl.pallas_call(
        _make_kernel(SK, W),
        out_shape=jax.ShapeDtypeStruct(A_x.shape, A_x.dtype),
        in_specs=[anyspec] * 9,
        out_specs=pl.BlockSpec(memory_space=pltpu.VMEM),
        scratch_shapes=[
            pltpu.VMEM((NR // 2, 2, W // 32, 128), u32),
            pltpu.VMEM((NR, W // 16, 128), bf16),
            pltpu.VMEM((H * DH // 128, D // 2, 128), u32),
            pltpu.VMEM((KD, H * DH // 2, 128), u32),
            pltpu.VMEM((KF, D // 2, 128), u32),
            pltpu.VMEM((KD, F // 2, 128), u32),
            pltpu.VMEM((1, 1, D), bf16),
            pltpu.VMEM((KF, 128), bf16),
            pltpu.VMEM((KD, 128), bf16),
            pltpu.VMEM((8, D), f32),
            pltpu.VMEM((8, D), u32),
            pltpu.VMEM((NT, 8, 128), u32),
            pltpu.VMEM((NT, 8, 128), u32),
            pltpu.VMEM((NJ * KD, 8, 128), f32),
            pltpu.VMEM((NJ * KD, 8, 128), f32),
            pltpu.VMEM((NCP, NT, 8, 128), f32),
            pltpu.VMEM((NCP, 8, 128), f32),
            pltpu.VMEM((NCP, 8, 128), f32),
            pltpu.VMEM((RG, 8, 128), f32),
            pltpu.VMEM((NJ, 8, 128), u32),
            pltpu.VMEM((NJ * KD, 8, 128), f32),
            pltpu.VMEM((KD, 8, 128), f32),
            pltpu.SemaphoreType.DMA((8 + 2 * NG,)),
        ],
        compiler_params=pltpu.CompilerParams(vmem_limit_bytes=127 * 1024 * 1024),
    )(A_x, kt, vt, A_wq, A_wo, B_w1, b1, B_w2, b2)
```

```python
import functools
import jax
import jax.numpy as jnp
from jax import lax
import jax.experimental.pallas as pl
import jax.experimental.pallas.tpu as pltpu

D = 640
H = 32
DH = 192
F = 1536
NP = H // 2
PD = 2 * DH
RH = DH // 8
RP = 2 * RH
NJ = PD // 128
NT = 2 * NJ
KD = D // 128
KF = F // 128
NW = NJ * KD
EPS = 1e-5
LOG2E = 1.4426950408889634
bf16 = jnp.bfloat16
f32 = jnp.float32
u32 = jnp.uint32

RATE = 6.0
SPOS = 450
LPOS = 0
RPOS = 300
RSTEP = 80
YPOS = 60
IPOS = 10
CPOS = 200
NL = 2
MORD = "hlwq"
SSPILL = 0
PACE = 3
NSLD = 4
D0 = 1
XA = 1
SETS = "10,10,10,18"
SETS14 = "16,16"
SETS15 = "24,8"
RATE14 = 5.5
RATE15 = 6.0
PACE14 = 3
PACE15 = 3
ONLY2 = 0
RF = 5
FSEL = "spread"
RP14 = 0
RP15 = 50
RS14 = 10
ORD14 = "hw"
ORD15 = "xw"


def _center(x):
    xc = x - jnp.mean(x, axis=-1, keepdims=True)
    v = jnp.mean(xc * xc, axis=-1, keepdims=True)
    return xc, lax.rsqrt(v + EPS)


def _gelu(x):
    c = 0.7978845608028654
    return 0.5 * x * (1.0 + jnp.tanh(c * (x + 0.044715 * (x * x * x))))


def _pack_rows(x8):
    x16 = jnp.concatenate([x8, x8], axis=0).astype(bf16)
    return pltpu.bitcast(x16, u32)


def _tile_dot(lhs_u32, w_u32):
    return jnp.dot(pltpu.bitcast(lhs_u32, bf16), pltpu.bitcast(w_u32, bf16),
                   preferred_element_type=f32)[0:8]


def _tree(op, xs):
    xs = list(xs)
    while len(xs) > 1:
        xs = [op(xs[i], xs[i + 1]) if i + 1 < len(xs) else xs[i] for i in range(0, len(xs), 2)]
    return xs[0]


def _tree_sum(xs):
    return _tree(jnp.add, xs)


def _make_kernel(SK, W):
    NCP = W // 256
    CA = 4 * XA
    CB = NCP - CA
    c_exp = (DH ** -0.5) * LOG2E
    P = functools.partial

    def kernel(x_hbm, k_hbm, v_hbm, wq_hbm, wo_hbm, w1_hbm, b1_hbm, w2_hbm, b2_hbm,
               o_ref,
               kb, vb, vx, vf, wqb, wob, w1b, w2b, xin, b1v, b2v, xl, rs_ref, ysum, ssum,
               ln0, ln1, lh0, lh1, lp, qr0, qr1, qr2, qr3, slo0, slo1, shi0, shi1, pb0, pb1,
               ls0, ls1, li0, li1, ac0, ac1, ol0, ol1, yr0, yr1, pk0, pk1, xr, tbl, sems):
        ln, lh, qr, slo, shi = (ln0, ln1), (lh0, lh1), (qr0, qr1), (slo0, slo1), (shi0, shi1)
        pb, ls, li, ac, ol, yr = (pb0, pb1), (ls0, ls1), (li0, li1), (ac0, ac1), (ol0, ol1), (yr0, yr1)
        pk = (pk0, pk1)
        ku = k_hbm.bitcast(u32)
        vu = v_hbm.bitcast(u32)
        NC = NP // 2

        def kcopy(c, s):
            return pltpu.make_async_copy(
                ku.at[pl.ds(c * RP, RP), :, pl.ds((SK - W) // 32, W // 32), :],
                kb.at[pl.ds(c * RP, RP)], sems.at[s])

        def vcopy(r0, n, s, shift=0):
            return pltpu.make_async_copy(
                v_hbm.at[pl.ds(r0, n), :, pl.ds((SK - W) // 16, W // 16), :],
                vb.at[pl.ds(r0 - shift, n)], sems.at[s])

        def wcopies(src, dst, s):
            su = src.bitcast(u32)
            return [pltpu.make_async_copy(su.at[:, pl.ds(n * 128, 128)], dst.at[n], sems.at[s])
                    for n in range(dst.shape[0])]

        head = [pltpu.make_async_copy(x_hbm, xin, sems.at[0]),
                pltpu.make_async_copy(b1_hbm, b1v, sems.at[0]),
                pltpu.make_async_copy(b2_hbm, b2v, sems.at[0])]
        head += [pltpu.make_async_copy(
            vu.at[pl.ds((NP - 2 + s) * RH, 8), :, pl.ds((SK - W) // 32, W // 32), :],
            vx.at[pl.ds(8 * s, 8)], sems.at[0]) for s in range(2)]
        head += wcopies(wq_hbm, wqb, 0) + wcopies(wo_hbm, wob, 0) + [kcopy(0, 0)]
        vlast = [vcopy((NP - 2 + s) * RH + 8, RH - 8, 3 + NC - 1, 8 * (s + 1)) for s in range(2)]
        c1 = wcopies(w1_hbm, w1b, 1)
        c2 = wcopies(w2_hbm, w2b, 2)
        for c in head:
            c.start()
        for c in range(NC - 1):
            kcopy(c + 1, 3 + c).start()
            vcopy(c * RP, RP, 3 + c).start()
        for c in vlast + c1 + c2:
            c.start()

        for i_ in range(NP):
            tbl[i_] = i_

        def qproj_tile(wg, dst, n):
            j, kt = divmod(n, KD)
            dst[n] = _tile_dot(xl[:, pl.ds(kt * 128, 128)], wg[j, pl.ds(kt * 64, 64), :])

        def build_l(src, dst, j):
            row = lax.broadcasted_iota(jnp.int32, (8, 128), 0)
            lane = lax.broadcasted_iota(jnp.int32, (8, 128), 1)
            q = _tree_sum(src[j * KD + kt] for kt in range(KD)) * rs_ref[...]
            qp = pltpu.roll(q, 8, 1)
            qm = pltpu.roll(q, 120, 1)
            tgt = (lane >> 1) & 4
            if j == 1:
                tgt = tgt + (lane >> 6)
            elif j == 2:
                tgt = tgt + 1
            hit = row == tgt
            low = row < 4
            dst[2 * j] = _pack_rows(jnp.where(hit, jnp.where(low, q, qp), 0.0))
            dst[2 * j + 1] = _pack_rows(jnp.where(hit, jnp.where(low, qm, q), 0.0))

        def qk_tile(kg, lsrc, sdst, c0, n):
            c4, rem = divmod(n, 4 * NT)
            t, i = divmod(rem, 4)
            c = c4 * 4 + i
            w = kg[pl.ds((t // 2) * 8, 8), t % 2, pl.ds((c0 + c) * 8, 8), :].reshape(64, 128)
            sdst[c, t] = _tile_dot(lsrc[t], w)

        def softmax(lo, hi, pdst, ldst, kdst=None):
            s = [_tree_sum(src[c, t] for t in range(NT)) for src in (lo, hi) for c in range(src.shape[0])]
            m = _tree(jnp.maximum, s)
            m = jnp.maximum(m, pltpu.roll(m, 4, 0))
            m = jnp.max(m, axis=1, keepdims=True)
            if SSPILL:
                for cp in range(NCP):
                    ssum[cp] = s[cp]
                s = [ssum[cp] for cp in range(NCP)]
            e = [jnp.exp2(a - m) for a in s]
            for cp in range(NCP):
                pdst[:, pl.ds(cp * 128, 128)] = e[cp]
                if kdst is not None:
                    kdst[cp] = _pack_rows(e[cp])
            ldst[...] = _tree_sum(e)

        def l_inv(lsrc, ldst):
            l = lsrc[...]
            l = l + pltpu.roll(l, 4, 0)
            l = jnp.sum(l, axis=1, keepdims=True)
            ldst[...] = jnp.broadcast_to(1.0 / l, (8, 128))

        def pack_p(psrc, kdst):
            for cp in range(NCP):
                kdst[cp] = _pack_rows(psrc[:, pl.ds(cp * 128, 128)])

        def reduce_o(asrc, lsrc, odst, j):
            blk = asrc[pl.ds(j * 16, 16)].reshape(128, 128)
            t = blk.T.reshape(16, 8, 128)
            if j == 1:
                lane = lax.broadcasted_iota(jnp.int32, (1, 128), 1)
                r = jnp.where(lane < 64, lsrc[0:1, :], lsrc[1:2, :])
            else:
                r = lsrc[j // 2:j // 2 + 1, :]
            odst[j] = _pack_rows(_tree_sum(t[i] for i in range(16)) * r)

        def x_tile(vg, n):
            s, rem = divmod(n, 2 * NCP)
            cp, e = divmod(rem, 2)
            w = vg[pl.ds(8 * s, 8), e, pl.ds(cp * 8, 8), :].reshape(64, 128)
            xr[s, e, cp] = _tile_dot(pk[s][cp], w)

        def x_finish(s):
            row = lax.broadcasted_iota(jnp.int32, (8, 128), 0)
            lane = lax.broadcasted_iota(jnp.int32, (8, 128), 1)
            o0 = _tree_sum(xr[s, 0, cp] for cp in range(NCP))
            o1 = _tree_sum(xr[s, 1, cp] for cp in range(NCP))
            low = row < 4
            direct = jnp.where(low, o0, o1)
            moved = jnp.where(low, pltpu.roll(o1, 8, 1), pltpu.roll(o0, 120, 1))
            o = jnp.where(((lane >> 1) & 4) == (row & 4), direct, moved)
            ol[s][0] = _pack_rows(jnp.where((row & 3) == 0, o, 0.0) * li[s][0:1, :])

        def wo_tile(wg, osrc, ydst, n):
            j, nt = divmod(n, KD)
            ydst[n] = _tile_dot(osrc[j], wg[nt, pl.ds(j * 64, 64), :])

        def y_fold(ysrc):
            for nt in range(KD):
                ysum[nt] = _tree_sum([ysum[nt]] + [ysrc[j * KD + nt] for j in range(NJ)])

        def copy(src, dst):
            for i in range(src.shape[0]):
                dst[i] = src[i]

        def kpair(i):
            return kb.at[pl.ds(i * RH, RH)]

        def wqpair(i):
            return wqb.at[pl.ds(i * NJ, NJ)]

        def wopair(i):
            r0 = i * (PD // 2)
            if not isinstance(i, int):
                r0 = pl.multiple_of(r0, PD // 2)
            return wob.at[:, pl.ds(r0, PD // 2), :]

        def run_block(first, i, a, rg0, sets, kinds, order, rate, pace_n, side):
            if rg0:
                vg = vb.at[pl.ds((NP - 2) * RH + a * (RH - 8), RH - 8)]
            else:
                vg = vb.at[pl.ds(i * RH, RH)]
            voff = rg0 // 2
            fg = vf.at[pl.ds(i * RF, RF)] if RF else None
            if FSEL == "last":
                fsel = {RP - RF + r: r for r in range(RF)}
            else:
                fsel = {RP - 1 - r * ((RP - 16) // max(RF, 1)): r for r in range(RF)}
            pace = dict(z=i, cnt=0, views={})

            def mxu_tile(key, n):
                if pace_n and pace["cnt"] % pace_n == 0:
                    z = pace["z"]
                    for _ in range(NSLD if pace["cnt"] > 0 else D0):
                        z = tbl[z]
                    pace["z"] = z
                    pace["views"] = {}
                pace["cnt"] += 1
                if key not in pace["views"]:
                    pace["views"][key] = kinds[key][1](pace["z"])
                kinds[key][2](pace["views"][key], n)

            mxu = [P(mxu_tile, key, n) for key in order for n in range(kinds[key][0])]
            side = sorted(side + [(int(n * rate), f) for n, f in enumerate(mxu)], key=lambda z: z[0])
            cnt = 0
            si = 0
            acc = {}
            sizes, ovl = sets.split(":") if ":" in sets else (sets, "0")
            groups = []
            for size in (int(z) for z in sizes.split(",")):
                groups.append(range(rg0, rg0 + size))
                rg0 += size
            step = NCP - int(ovl)
            seq = [(rgs, t - gi * step) for t in range((len(groups) - 1) * step + NCP)
                   for gi, rgs in enumerate(groups) if 0 <= t - gi * step < NCP]
            for rgs, cp in seq:
                mult = {hh: (pb[a][pl.ds(hh, 1), pl.ds(cp * 128, 128)],
                             pb[a][pl.ds(4 + hh, 1), pl.ds(cp * 128, 128)])
                        for hh in sorted({rg // RH for rg in rgs})}
                for rg in rgs:
                    while si < len(side) and side[si][0] <= cnt:
                        side[si][1]()
                        si += 1
                    cnt += 1
                    m0, m1 = mult[rg // RH]
                    if rg in fsel and not first:
                        v0, v1 = fg[fsel[rg], 2 * cp], fg[fsel[rg], 2 * cp + 1]
                    else:
                        v = vg[rg // 2 - voff, rg % 2, pl.ds(cp * 16, 16), :].astype(f32)
                        v0, v1 = v[:8], v[8:]
                        if rg in fsel:
                            fg[fsel[rg], 2 * cp] = v0
                            fg[fsel[rg], 2 * cp + 1] = v1
                    if rg not in acc:
                        acc[rg] = v0 * m0 + v1 * m1
                    else:
                        acc[rg] = acc[rg] + v0 * m0 + v1 * m1
                    if cp == NCP - 1:
                        ac[a][rg] = acc[rg]
            assert rg0 == RP
            for _, f in side[si:]:
                f()

        def layer(x, first):
            xc, rs = _center(x)
            xl[...] = _pack_rows(xc)
            rs_ref[...] = jnp.broadcast_to(rs * c_exp, (8, 128))
            ac1[...] = jnp.zeros(ac1.shape, f32)
            li1[...] = jnp.zeros(li1.shape, f32)
            ol0[...] = jnp.zeros(ol0.shape, u32)
            yr1[...] = jnp.zeros(yr1.shape, f32)
            ysum[...] = jnp.zeros(ysum.shape, f32)

            for i, dst in enumerate((qr2, qr3, qr0)):
                for n in range(NW):
                    qproj_tile(wqpair(i), dst, n)
            for j in range(NJ):
                build_l(qr2, lp, j)
            for n in range(CA * NT):
                qk_tile(kpair(0), lp, slo0, 0, n)
            for n in range(CB * NT):
                qk_tile(kpair(0), lp, shi0, CA, n)
            for j in range(NJ):
                build_l(qr3, lh1, j)
            for n in range(CA * NT):
                qk_tile(kpair(1), lh1, slo1, 0, n)
            for n in range(NW):
                qproj_tile(wqpair(3), qr1, n)
            for j in range(NJ):
                build_l(qr0, ln0, j)
            softmax(slo0, shi0, pb0, ls0)

            def kinds(a):
                b = 1 - a
                return dict(
                    h=(CB * NT, lambda z: kpair(z + 1),
                       lambda w, n: qk_tile(w, lh[b], shi[b], CA, n)),
                    l=(CA * NT, lambda z: kpair(z + 2),
                       lambda w, n: qk_tile(w, ln[a], slo[a], 0, n)),
                    q=(NW, lambda z: wqpair(jnp.minimum(z + 4, NP - 1)),
                       lambda w, n: qproj_tile(w, qr[a], n)),
                    w=(NW, lambda z: wopair(jnp.maximum(z - 2, 0)),
                       lambda w, n: wo_tile(w, ol[a], yr[a], n)),
                    x=(4 * NCP, lambda z: vx.at[pl.ds((z - (NP - 1)) * 16, 16)], x_tile))

            def block(i, a):
                b = 1 - a
                side = [(SPOS, P(softmax, slo[b], shi[b], pb[b], ls[b])),
                        (IPOS, P(l_inv, ls[a], li[a])),
                        (CPOS, P(copy, ln[a], lh[a])),
                        (YPOS, P(y_fold, yr[b]))]
                for j in range(NJ):
                    side.append((LPOS + 10 * j, P(build_l, qr[b], ln[b], j)))
                    side.append((RPOS + RSTEP * j, P(reduce_o, ac[b], li[b], ol[b], j)))
                run_block(first, i, a, 0, SETS, kinds(a), MORD, RATE, PACE, side)

            def block14(i):
                side = [(int((CB * NT + NW) * RATE14) + 10, P(softmax, slo1, shi1, pb1, ls1, pk1)),
                        (IPOS, P(l_inv, ls0, li0)),
                        (100, P(pack_p, pb0, pk0)),
                        (YPOS, P(y_fold, yr1))]
                for j in range(NJ):
                    side.append((RP14 + RS14 * j, P(reduce_o, ac1, li1, ol1, j)))
                run_block(first, i, 0, 16, SETS14, kinds(0), ORD14, RATE14, PACE14, side)

            def block15(i):
                side = [(IPOS, P(l_inv, ls1, li1)),
                        (YPOS, P(y_fold, yr0))]
                for j in range(1, NJ):
                    side.append((RP15 + RS14 * j, P(reduce_o, ac0, li0, ol0, j)))
                run_block(first, i, 1, 16, SETS15, kinds(1), ORD15, RATE15, PACE15, side)

            def body(i, c):
                if first:
                    @pl.when((i & 1) == 0)
                    def _():
                        ch = lax.shift_right_logical(i, 1)
                        vcopy(ch * RP, RP, 3 + ch).wait()
                        kcopy(ch + 1, 3 + ch).wait()

                for a in range(2):
                    pl.when((i & 1) == a)(P(block, i, a))
                return c

            lax.fori_loop(0, NP - 2, body, 0)
            if first:
                for c in vlast:
                    c.wait()

            def tail(i, c):
                pl.when(i == NP - 2)(P(block14, i))
                pl.when(i == NP - 1)(P(block15, i))
                return c

            lax.fori_loop(NP - 2, NP, tail, 0)

            x_finish(0)
            x_finish(1)
            for j in range(1, NJ):
                reduce_o(ac1, li1, ol1, j)
            order = list(range(KD, NW)) + list(range(KD))
            for n in order:
                wo_tile(wopair(NP - 2), ol0, yr0, n)
            for n in range(NW):
                wo_tile(wopair(NP - 1), ol1, qr0, n)
            ys = [_tree_sum([ysum[nt]] + [src[j * KD + nt] for src in (yr1, yr0, qr0) for j in range(NJ)])
                  for nt in range(KD)]
            y = jnp.sum(jnp.concatenate(ys, axis=1), axis=0, keepdims=True)
            x = x + y

            xc, rs = _center(x)
            xn = _pack_rows(xc)
            if first:
                for c in c1:
                    c.wait()
            hs = []
            for n in range(KF):
                h = _tree_sum(_tile_dot(xn[:, kt * 128:(kt + 1) * 128], w1b[n, pl.ds(kt * 64, 64), :])
                              for kt in range(KD))
                hs.append(_pack_rows(_gelu(h * rs + b1v[n:n + 1, :].astype(f32))))
            if first:
                for c in c2:
                    c.wait()
            parts = [[_tile_dot(hs[kt], w2b[nt, pl.ds(kt * 64, 64), :]) for nt in range(KD)]
                     for kt in range(KF)]
            y2 = jnp.concatenate(
                [_tree_sum(parts[kt][nt] for kt in range(KF)) + b2v[nt:nt + 1, :].astype(f32)
                 for nt in range(KD)], axis=1)
            return x + y2

        for c in head:
            c.wait()

        def transpose_tile(n, c):
            s8 = pl.multiple_of((n // (2 * NCP)) * 8, 8)
            e = n % 2
            c8 = pl.multiple_of(((n // 2) % NCP) * 8, 8)
            w = vx[pl.ds(s8, 8), e, pl.ds(c8, 8), :].reshape(64, 128)
            wt = pltpu.bitcast(w, bf16).astype(f32).T.astype(bf16)
            vx[pl.ds(s8, 8), e, pl.ds(c8, 8), :] = pltpu.bitcast(wt, u32).reshape(8, 8, 128)
            return c

        lax.fori_loop(0, 4 * NCP, transpose_tile, 0)

        if ONLY2:
            for c in c1 + c2 + vlast + [vcopy(c * RP, RP, 3 + c) for c in range(NC - 1)] + [kcopy(c + 1, 3 + c) for c in range(NC - 1)]:
                c.wait()
        x = jnp.broadcast_to(xin[0].astype(f32), (8, D))
        for l_ in range(1 if ONLY2 else NL):
            x = layer(x, l_ == 0 and not ONLY2)
        o_ref[0] = x[0:1, :].astype(o_ref.dtype)

    return kernel


@jax.jit
def pallas_interleave_layers__sliding_block_cached__dense_activation_gelu__decode_kernel(
    A_x, A_k_cache, A_v_cache, A_wq, A_wo, B_x, B_w1, B_b1, B_w2, B_b2,
):
    SK = A_k_cache.shape[2]
    W = min(4096, max(256, SK // 4))
    NR = H * DH // 8

    def tiled(a):
        t = jnp.swapaxes(a, 2, 3).reshape(NR, 8, SK // 128, 128)
        return t.transpose(0, 2, 1, 3).reshape(NR // 2, 2, SK // 16, 128)

    b1 = B_b1.reshape(F // 128, 128)
    b2 = B_b2.reshape(D // 128, 128)
    anyspec = pl.BlockSpec(memory_space=pl.ANY)
    NCP = W // 256
    vreg = lambda n, dt: pltpu.VMEM(n + (8, 128), dt)
    return pl.pallas_call(
        _make_kernel(SK, W),
        out_shape=jax.ShapeDtypeStruct(A_x.shape, A_x.dtype),
        in_specs=[anyspec] * 9,
        out_specs=pl.BlockSpec(memory_space=pltpu.VMEM),
        scratch_shapes=[
            pltpu.VMEM((NR // 2, 2, W // 32, 128), u32),
            pltpu.VMEM((NR // 2 - 16, 2, W // 16, 128), bf16),
            pltpu.VMEM((16, 2, W // 32, 128), u32),
            vreg((NP * max(RF, 1), 2 * NCP), f32),
            pltpu.VMEM((H * DH // 128, D // 2, 128), u32),
            pltpu.VMEM((KD, H * DH // 2, 128), u32),
            pltpu.VMEM((KF, D // 2, 128), u32),
            pltpu.VMEM((KD, F // 2, 128), u32),
            pltpu.VMEM((1, 1, D), bf16),
            pltpu.VMEM((KF, 128), bf16),
            pltpu.VMEM((KD, 128), bf16),
            pltpu.VMEM((8, D), u32),
            pltpu.VMEM((8, 128), f32),
            vreg((KD,), f32),
            vreg((NCP,), f32),
        ] + [vreg((NT,), u32)] * 5
          + [vreg((NW,), f32)] * 4
          + [vreg((4 * XA, NT), f32)] * 2
          + [vreg((NCP - 4 * XA, NT), f32)] * 2
          + [pltpu.VMEM((8, NCP * 128), f32)] * 2
          + [pltpu.VMEM((8, 128), f32)] * 4
          + [vreg((RP,), f32)] * 2
          + [vreg((NJ,), u32)] * 2
          + [vreg((NW,), f32)] * 2
          + [vreg((NCP,), u32)] * 2
          + [vreg((2, 2, NCP), f32)]
          + [pltpu.SMEM((NP,), jnp.int32)]
          + [pltpu.SemaphoreType.DMA((3 + NP // 2,))],
        compiler_params=pltpu.CompilerParams(vmem_limit_bytes=128 * 1024 * 1024),
    )(A_x, tiled(A_k_cache), tiled(A_v_cache), A_wq, A_wo, B_w1, b1, B_w2, b2)
```

```python
import functools
import jax
import jax.numpy as jnp
from jax import lax
import jax.experimental.pallas as pl
import jax.experimental.pallas.tpu as pltpu

D = 640
H = 32
DH = 192
F = 1536
NP = H // 2
PD = 2 * DH
RH = DH // 8
RP = 2 * RH
NJ = PD // 128
NT = 2 * NJ
KD = D // 128
KF = F // 128
NW = NJ * KD
EPS = 1e-5
LOG2E = 1.4426950408889634
bf16 = jnp.bfloat16
f32 = jnp.float32
u32 = jnp.uint32

RATE = 6.0
SPOS = 450
LPOS = 100
RPOS = 300
RSTEP = 80
YPOS = 5
IPOS = 150
IPOS14 = 10
IPOS15 = 10
SETS13 = "6,6,6,6,6,18"
CM = 2
RIN15 = 0
KPOS = 300
YP14 = 5
YP15 = 5
RS15 = 10
MORD13 = "hwlm"
RATE13 = 6.1
CPOS = 200
NL = 2
MORD = "hwql"
SSPILL = 0
PACE = 3
NSLD = 4
D0 = 1
XA = 1
SETS = "6,6,6,6,6,18"
SETS14 = "16,16"
SETS15 = "8,8,8,8"
RATE14 = 6.7
RATE15 = 6.2
PACE14 = 3
PACE15 = 3
ONLY2 = 0
NOSEM = 0
STAGED = 0
GPOS = 30
GLAG = 60
ELAG = 80
MOFF = 0
LSTEP = 10
WOSTEP = 256
W2STEP = 192
W2SPLIT = "0,9,11,12"
RF = 5
FSEL = "spread"
RP14 = 100
RP15 = 100
RS14 = 10
ORD14 = "gw"
WLAG = 2
ORD15 = "xw"
Q2EARLY = 1


def _center(x):
    xc = x - jnp.mean(x, axis=-1, keepdims=True)
    v = jnp.mean(xc * xc, axis=-1, keepdims=True)
    return xc, lax.rsqrt(v + EPS)


def _gelu(x):
    c = 0.7978845608028654
    return 0.5 * x * (1.0 + jnp.tanh(c * (x + 0.044715 * (x * x * x))))


def _pack_rows(x8):
    x16 = jnp.concatenate([x8, x8], axis=0).astype(bf16)
    return pltpu.bitcast(x16, u32)


def _tile_dot(lhs_u32, w_u32):
    return jnp.dot(pltpu.bitcast(lhs_u32, bf16), pltpu.bitcast(w_u32, bf16),
                   preferred_element_type=f32)[0:8]


def _tree(op, xs):
    xs = list(xs)
    while len(xs) > 1:
        xs = [op(xs[i], xs[i + 1]) if i + 1 < len(xs) else xs[i] for i in range(0, len(xs), 2)]
    return xs[0]


def _tree_sum(xs):
    return _tree(jnp.add, xs)


def _make_kernel(SK, W):
    NCP = W // 256
    CA = 4 * XA
    CB = NCP - CA
    c_exp = (DH ** -0.5) * LOG2E
    P = functools.partial

    def kernel(x_hbm, k_hbm, v_hbm, wq_hbm, wo_hbm, w1_hbm, b1_hbm, w2_hbm, b2_hbm,
               o_ref,
               kb, vb, vx, vf, wqb, wob, w1b, w2b, xin, b1v, b2v, xl, rs_ref, ysum, ssum,
               ln0, ln1, lp, qr0, qr1, qr2, qr3, slo0, slo1, smid, shi0, shi1, pb0, pb1,
               ls0, ls1, li0, li1, ac0, ac1, ol0, ol1, yr0, yr1, pk0, pk1, xr, tbl, sems):
        ln, qr, slo, shi = (ln0, ln1), (qr0, qr1), (slo0, slo1), (shi0, shi1)
        pb, ls, li, ac, ol, yr = (pb0, pb1), (ls0, ls1), (li0, li1), (ac0, ac1), (ol0, ol1), (yr0, yr1)
        pk = (pk0, pk1)
        ku = k_hbm.bitcast(u32)
        vu = v_hbm.bitcast(u32)
        NC = NP // 2

        def kcopy(c, s):
            return pltpu.make_async_copy(
                ku.at[pl.ds(c * RP, RP), :, pl.ds((SK - W) // 32, W // 32), :],
                kb.at[pl.ds(c * RP, RP)], sems.at[s])

        def vcopy(r0, n, s, shift=0):
            return pltpu.make_async_copy(
                v_hbm.at[pl.ds(r0, n), :, pl.ds((SK - W) // 16, W // 16), :],
                vb.at[pl.ds(r0 - shift, n)], sems.at[s])

        def wcopies(src, dst, s, r0=0, nrows=None, step=None):
            su = src.bitcast(u32)
            nrows = dst.shape[1] if nrows is None else nrows
            step = nrows if step is None else step
            return [pltpu.make_async_copy(su.at[pl.ds(r, step), pl.ds(n * 128, 128)],
                                          dst.at[n, pl.ds(r, step)], sems.at[s])
                    for r in range(r0, r0 + nrows, step) for n in range(dst.shape[0])]

        head = [pltpu.make_async_copy(x_hbm, xin, sems.at[0]),
                pltpu.make_async_copy(b1_hbm, b1v, sems.at[0]),
                pltpu.make_async_copy(b2_hbm, b2v, sems.at[0])]
        head += [pltpu.make_async_copy(
            vu.at[pl.ds((NP - 2 + s) * RH, 8), :, pl.ds((SK - W) // 32, W // 32), :],
            vx.at[pl.ds(8 * s, 8)], sems.at[0]) for s in range(2)]
        head += wcopies(wq_hbm, wqb, 0) + wcopies(wo_hbm, wob, 0, step=WOSTEP) + [kcopy(0, 0)]
        vlast = [vcopy((NP - 2 + s) * RH + 8, RH - 8, 2, 8 * (s + 1)) for s in range(2)]
        c1 = wcopies(w1_hbm, w1b, 1)
        w2_split = tuple(int(z) for z in W2SPLIT.split(','))
        c2 = [wcopies(w2_hbm, w2b, (0, 3, 4)[g], 64 * w2_split[g],
                      64 * (w2_split[g + 1] - w2_split[g]),
                      min(W2STEP, 64 * (w2_split[g + 1] - w2_split[g]))) for g in range(len(w2_split) - 1)]
        c2all = [c for g in c2 for c in g]
        for c in head:
            c.start()

        def chunk(c):
            s = 1 + (c & 1)
            return [kcopy(c + 1, s), vcopy(c * RP, RP, s)]

        for c in chunk(0) + chunk(1):
            c.start()

        for i_ in range(NP):
            tbl[i_] = i_

        def qproj_tile(wg, dst, n):
            j, kt = divmod(n, KD)
            dst[n] = _tile_dot(xl[:, pl.ds(kt * 128, 128)], wg[j, pl.ds(kt * 64, 64), :])

        def build_l(src, dst, j):
            row = lax.broadcasted_iota(jnp.int32, (8, 128), 0)
            lane = lax.broadcasted_iota(jnp.int32, (8, 128), 1)
            q = _tree_sum(src[j * KD + kt] for kt in range(KD)) * rs_ref[...]
            qp = pltpu.roll(q, 8, 1)
            qm = pltpu.roll(q, 120, 1)
            tgt = (lane >> 1) & 4
            if j == 1:
                tgt = tgt + (lane >> 6)
            elif j == 2:
                tgt = tgt + 1
            hit = row == tgt
            low = row < 4
            dst[2 * j] = _pack_rows(jnp.where(hit, jnp.where(low, q, qp), 0.0))
            dst[2 * j + 1] = _pack_rows(jnp.where(hit, jnp.where(low, qm, q), 0.0))

        def qk_tile(kg, lsrc, sdst, c0, n, ncp=NCP):
            c4, rem = divmod(n, 4 * NT)
            t, i = divmod(rem, min(4, ncp - c4 * 4))
            c = c4 * 4 + i
            w = kg[pl.ds((t // 2) * 8, 8), t % 2, pl.ds((c0 + c) * 8, 8), :].reshape(64, 128)
            sdst[c, t] = _tile_dot(lsrc[t], w)

        def s_group(st, src, c0, c1):
            s = [_tree_sum(src[c, t] for t in range(NT)) for c in range(c0, c1)]
            base = len(st.setdefault("s", []))
            if SSPILL:
                for k_, a_ in enumerate(s):
                    ssum[st.get("zero", 0) + base + k_] = a_
            st["s"] += s
            st["m"] = _tree(jnp.maximum, s + ([st["m"]] if "m" in st else []))

        def s_max(st):
            m = jnp.maximum(st["m"], pltpu.roll(st["m"], 4, 0))
            st["m"] = jnp.max(m, axis=1, keepdims=True)

        def s_exp(st, pdst, ldst, kdst=None):
            s = [ssum[cp] for cp in range(NCP)] if SSPILL else st["s"]
            e = [jnp.exp2(a - st["m"]) for a in s]
            for cp in range(NCP):
                pdst[:, pl.ds(cp * 128, 128)] = e[cp]
                if kdst is not None:
                    kdst[cp] = _pack_rows(e[cp])
            ldst[...] = _tree_sum(e)

        def softmax_steps(lo, hi, pdst, ldst, kdst=None, zero=None, mid=None):
            st = {} if zero is None else {"zero": zero}
            srcs = [(lo, CA), (hi, CB)] if mid is None else [(lo, CA), (mid, CM), (hi, CB - CM)]
            steps = [P(s_group, st, src, c0, min(c0 + 4, n)) for src, n in srcs for c0 in range(0, n, 4)]
            return steps + [P(s_max, st), P(s_exp, st, pdst, ldst, kdst)]

        def softmax(*args):
            for f in softmax_steps(*args):
                f()

        def l_inv(lsrc, ldst):
            l = lsrc[...]
            l = l + pltpu.roll(l, 4, 0)
            l = jnp.sum(l, axis=1, keepdims=True)
            ldst[...] = jnp.broadcast_to(1.0 / l, (8, 128))

        def pack_p(psrc, kdst):
            for cp in range(NCP):
                kdst[cp] = _pack_rows(psrc[:, pl.ds(cp * 128, 128)])

        def reduce_o(asrc, lsrc, odst, j):
            blk = asrc[pl.ds(j * 16, 16)].reshape(128, 128)
            t = blk.T.reshape(16, 8, 128)
            if j == 1:
                lane = lax.broadcasted_iota(jnp.int32, (1, 128), 1)
                r = jnp.where(lane < 64, lsrc[0:1, :], lsrc[1:2, :])
            else:
                r = lsrc[j // 2:j // 2 + 1, :]
            odst[j] = _pack_rows(_tree_sum(t[i] for i in range(16)) * r)

        def x_tile(vg, n):
            s, rem = divmod(n, 2 * NCP)
            cp, e = divmod(rem, 2)
            w = vg[pl.ds(8 * s, 8), e, pl.ds(cp * 8, 8), :].reshape(64, 128)
            xr[s, e, cp] = _tile_dot(pk[s][cp], w)

        def x_finish(s):
            row = lax.broadcasted_iota(jnp.int32, (8, 128), 0)
            lane = lax.broadcasted_iota(jnp.int32, (8, 128), 1)
            o0 = _tree_sum(xr[s, 0, cp] for cp in range(NCP))
            o1 = _tree_sum(xr[s, 1, cp] for cp in range(NCP))
            low = row < 4
            direct = jnp.where(low, o0, o1)
            moved = jnp.where(low, pltpu.roll(o1, 8, 1), pltpu.roll(o0, 120, 1))
            o = jnp.where(((lane >> 1) & 4) == (row & 4), direct, moved)
            ol[s][0] = _pack_rows(jnp.where((row & 3) == 0, o, 0.0) * li[s][0:1, :])

        def wo_tile(wg, osrc, ydst, n):
            j, nt = divmod(n, KD)
            ydst[n] = _tile_dot(osrc[j], wg[nt, pl.ds(j * 64, 64), :])

        def y_fold(ysrc):
            for nt in range(KD):
                ysum[nt] = _tree_sum([ysum[nt]] + [ysrc[j * KD + nt] for j in range(NJ)])

        def copy(src, dst):
            for i in range(src.shape[0]):
                dst[i] = src[i]

        def kpair(i):
            return kb.at[pl.ds(i * RH, RH)]

        def wqpair(i):
            return wqb.at[pl.ds(i * NJ, NJ)]

        def wopair(i):
            r0 = i * (PD // 2)
            if not isinstance(i, int):
                r0 = pl.multiple_of(r0, PD // 2)
            return wob.at[:, pl.ds(r0, PD // 2), :]

        def run_block(first, i, a, rg0, sets, kinds, order, rate, pace_n, side, moff=0):
            if rg0:
                vg = vb.at[pl.ds((NP - 2) * RH + a * (RH - 8), RH - 8)]
            else:
                vg = vb.at[pl.ds(i * RH, RH)]
            voff = rg0 // 2
            fg = vf.at[pl.ds(i * RF, RF)] if RF else None
            if FSEL == "last":
                fsel = {RP - RF + r: r for r in range(RF)}
            else:
                fsel = {RP - 1 - r * ((RP - 16) // max(RF, 1)): r for r in range(RF)}
            pace = dict(z=i, cnt=0, views={})

            def mxu_tile(key, n):
                if pace_n and pace["cnt"] % pace_n == 0:
                    z = pace["z"]
                    for _ in range(NSLD if pace["cnt"] > 0 else D0):
                        z = tbl[z]
                    pace["z"] = z
                    pace["views"] = {}
                pace["cnt"] += 1
                if key not in pace["views"]:
                    pace["views"][key] = kinds[key][1](pace["z"])
                kinds[key][2](pace["views"][key], n)

            mxu = [P(mxu_tile, key, n) for key in order for n in range(kinds[key][0])]
            side = sorted(side + [(moff + int(n * rate), f) for n, f in enumerate(mxu)], key=lambda z: z[0])
            cnt = 0
            si = 0
            acc = {}
            sizes, ovl = sets.split(":") if ":" in sets else (sets, "0")
            groups = []
            for size in (int(z) for z in sizes.split(",")):
                groups.append(range(rg0, rg0 + size))
                rg0 += size
            step = NCP - int(ovl)
            seq = [(rgs, t - gi * step) for t in range((len(groups) - 1) * step + NCP)
                   for gi, rgs in enumerate(groups) if 0 <= t - gi * step < NCP]
            for rgs, cp in seq:
                mult = {hh: (pb[a][pl.ds(hh, 1), pl.ds(cp * 128, 128)],
                             pb[a][pl.ds(4 + hh, 1), pl.ds(cp * 128, 128)])
                        for hh in sorted({rg // RH for rg in rgs})}
                for rg in rgs:
                    while si < len(side) and side[si][0] <= cnt:
                        side[si][1]()
                        si += 1
                    cnt += 1
                    m0, m1 = mult[rg // RH]
                    if rg in fsel and not first:
                        v0, v1 = fg[fsel[rg], 2 * cp], fg[fsel[rg], 2 * cp + 1]
                    else:
                        v = vg[rg // 2 - voff, rg % 2, pl.ds(cp * 16, 16), :].astype(f32)
                        v0, v1 = v[:8], v[8:]
                        if rg in fsel:
                            fg[fsel[rg], 2 * cp] = v0
                            fg[fsel[rg], 2 * cp + 1] = v1
                    if rg not in acc:
                        acc[rg] = v0 * m0 + v1 * m1
                    else:
                        acc[rg] = acc[rg] + v0 * m0 + v1 * m1
                    if cp == NCP - 1:
                        ac[a][rg] = acc[rg]
            assert rg0 == RP
            for _, f in side[si:]:
                f()

        def layer(x, first):
            xc, rs = _center(x)
            xl[...] = _pack_rows(xc)
            rs_ref[...] = jnp.broadcast_to(rs * c_exp, (8, 128))
            ac1[...] = jnp.zeros(ac1.shape, f32)
            li1[...] = jnp.zeros(li1.shape, f32)
            if WLAG == 1:
                yr0[...] = jnp.zeros(yr0.shape, f32)
            else:
                ol0[...] = jnp.zeros(ol0.shape, u32)
                yr1[...] = jnp.zeros(yr1.shape, f32)
            ysum[...] = jnp.zeros(ysum.shape, f32)

            for i, dst in enumerate((qr2, qr3)):
                for n in range(NW):
                    qproj_tile(wqpair(i), dst, n)
            if Q2EARLY:
                for n in range(NW):
                    qproj_tile(wqpair(2), qr0, n)
            for j in range(NJ):
                build_l(qr2, lp, j)
            for n in range(CA * NT):
                qk_tile(kpair(0), lp, slo0, 0, n)
            for n in range(CB * NT):
                qk_tile(kpair(0), lp, shi0, CA, n)
            for j in range(NJ):
                build_l(qr3, ln1, j)
            for n in range(CA * NT):
                qk_tile(kpair(1), ln1, slo1, 0, n)
            if not Q2EARLY:
                for n in range(NW):
                    qproj_tile(wqpair(2), qr0, n)
            softmax(slo0, shi0, pb0, ls0)

            wp = lambda a: 1 - a if WLAG == 1 else a

            def kinds(a):
                b = 1 - a
                return dict(
                    h=(CB * NT, lambda z: kpair(z + 1),
                       lambda w, n: qk_tile(w, ln[b], shi[b], CA, n)),
                    l=(CA * NT, lambda z: kpair(z + 2),
                       lambda w, n: qk_tile(w, ln[a], slo[a], 0, n)),
                    q=(NW, lambda z: wqpair(jnp.minimum(z + 3, NP - 1)),
                       lambda w, n: qproj_tile(w, qr[b], n)),
                    w=(NW, lambda z: wopair(jnp.maximum(z - WLAG, 0)),
                       lambda w, n: wo_tile(w, ol[wp(a)], yr[wp(a)], n)),
                    v=(2 * KD, lambda z: wopair(z - 1),
                       lambda w, n: wo_tile(w, ol[b], yr[b], KD + n)),
                    m=(CM * NT, lambda z: kpair(z + 2),
                       lambda w, n: qk_tile(w, ln[a], smid, CA, n, CM)),
                    g=((CB - CM) * NT, lambda z: kpair(z + 1),
                       lambda w, n: qk_tile(w, ln[b], shi[b], CA + CM, n, CB - CM)),
                    x=(4 * NCP, lambda z: vx.at[pl.ds((z - (NP - 1)) * 16, 16)], x_tile))

            def block(i, a, order=MORD, RATE=RATE, SETS=SETS):
                b = 1 - a
                steps = softmax_steps(slo[b], shi[b], pb[b], ls[b], None, tbl[i] - i if SSPILL == 2 else None)
                if STAGED:
                    pos = [GPOS] * XA + [MOFF + int(24 * (k_ + 1) * RATE) + GLAG for k_ in range(4 - XA)]
                    pos += [pos[-1] + 1, pos[-1] + ELAG]
                else:
                    pos = [max(SPOS, MOFF + int(CB * NT * RATE) + 1)] * len(steps)
                side = list(zip(pos, steps))
                side += [(IPOS, P(l_inv, ls[a], li[a])),
                         (YPOS, P(y_fold, yr[1 - wp(a)]))]
                for j in range(NJ):
                    side.append((LPOS + LSTEP * j, P(build_l, qr[a], ln[a], j)))
                    side.append((RPOS + RSTEP * j, P(reduce_o, ac[b], li[b], ol[b], j)))
                run_block(first, i, a, 0, SETS, kinds(a), order, RATE, PACE, side, MOFF)

            def block14(i):
                side = [(int(((CB - CM) * NT + NW) * RATE14) + 10, P(softmax, slo1, shi1, pb1, ls1, pk1, None, smid)),
                        (IPOS14, P(l_inv, ls0, li0)),
                        (KPOS, P(pack_p, pb0, pk0)),
                        (YP14, P(y_fold, yr[1 - wp(0)]))]
                for j in range(NJ):
                    side.append((RP14 + RS14 * j, P(reduce_o, ac1, li1, ol1, j)))
                run_block(first, i, 0, 16, SETS14, kinds(0), ORD14, RATE14, PACE14, side)

            def block15(i):
                side = [(IPOS15, P(l_inv, ls1, li1)),
                        (YP15, P(y_fold, yr[1 - wp(1)]))]
                for j in range(1, NJ):
                    side.append((RP15 + RS15 * j, P(reduce_o, ac0, li0, ol0, j)))
                if RIN15 >= 1:
                    side.append((16 * NCP + 1, P(reduce_o, ac1, li1, ol1, 1)))
                if RIN15 >= 2:
                    side.append((32 * NCP + 1, P(reduce_o, ac1, li1, ol1, 2)))
                run_block(first, i, 1, 16, SETS15, kinds(1), ORD15, RATE15, PACE15, side)

            def body(i, c):
                if first:
                    @pl.when((i & 1) == 0)
                    def _():
                        ch = lax.shift_right_logical(i, 1)
                        for c in chunk(ch):
                            c.wait()

                        @pl.when(ch + 2 < NC - 1)
                        def _():
                            for c in chunk(ch + 2):
                                c.start()

                        @pl.when(ch + 2 == NC - 1)
                        def _():
                            for c in vlast:
                                c.start()

                        @pl.when(ch + 1 == NC - 1)
                        def _():
                            for c in c1 + c2all:
                                c.start()

                for a in range(2):
                    pl.when((i & 1) == a)(P(block, i, a))
                return c

            lax.fori_loop(0, NP - 3, body, 0)

            def tail(i, c):
                pl.when(i == NP - 3)(P(block, i, 1, MORD13, RATE13, SETS13))
                if first:
                    @pl.when(i == NP - 2)
                    def _():
                        for c in vlast:
                            c.wait()

                pl.when(i == NP - 2)(P(block14, i))
                pl.when(i == NP - 1)(P(block15, i))
                return c

            lax.fori_loop(NP - 3, NP, tail, 0)

            x_finish(0)
            x_finish(1)
            for j in range(1 + RIN15, NJ):
                reduce_o(ac1, li1, ol1, j)
            for n in (range(KD) if WLAG == 1 else list(range(KD, NW)) + list(range(KD))):
                wo_tile(wopair(NP - 2), ol0, yr0, n)
            for n in range(NW):
                wo_tile(wopair(NP - 1), ol1, qr0, n)
            ys = [_tree_sum([ysum[nt]] + [src[j * KD + nt] for src in ((yr0, qr0) if WLAG == 1 else (yr1, yr0, qr0)) for j in range(NJ)])
                  for nt in range(KD)]
            y = jnp.sum(jnp.concatenate(ys, axis=1), axis=0, keepdims=True)
            x = x + y

            xc, rs = _center(x)
            xn = _pack_rows(xc)
            if first:
                for c in c1:
                    c.wait()
            hs = []
            for n in range(KF):
                h = _tree_sum(_tile_dot(xn[:, kt * 128:(kt + 1) * 128], w1b[n, pl.ds(kt * 64, 64), :])
                              for kt in range(KD))
                hs.append(_pack_rows(_gelu(h * rs + b1v[n:n + 1, :].astype(f32))))
            parts = []
            for kt in range(KF):
                if first and kt in w2_split:
                    for c in c2[w2_split.index(kt)]:
                        c.wait()
                parts.append([_tile_dot(hs[kt], w2b[nt, pl.ds(kt * 64, 64), :]) for nt in range(KD)])
            y2 = jnp.concatenate(
                [_tree_sum(parts[kt][nt] for kt in range(KF)) + b2v[nt:nt + 1, :].astype(f32)
                 for nt in range(KD)], axis=1)
            return x + y2

        for c in head:
            c.wait()

        def transpose_tile(n, c):
            s8 = pl.multiple_of((n // (2 * NCP)) * 8, 8)
            e = n % 2
            c8 = pl.multiple_of(((n // 2) % NCP) * 8, 8)
            w = vx[pl.ds(s8, 8), e, pl.ds(c8, 8), :].reshape(64, 128)
            wt = pltpu.bitcast(w, bf16).astype(f32).T.astype(bf16)
            vx[pl.ds(s8, 8), e, pl.ds(c8, 8), :] = pltpu.bitcast(wt, u32).reshape(8, 8, 128)
            return c

        lax.fori_loop(0, 4 * NCP, transpose_tile, 0)

        if ONLY2:
            for c in chunk(0) + chunk(1):
                c.wait()
        x = jnp.broadcast_to(xin[0].astype(f32), (8, D))
        for l_ in range(1 if ONLY2 else NL):
            x = layer(x, l_ == 0 and not ONLY2)
        o_ref[0] = x[0:1, :].astype(o_ref.dtype)

    return kernel


@jax.jit
def pallas_interleave_layers__sliding_block_cached__dense_activation_gelu__decode_kernel(
    A_x, A_k_cache, A_v_cache, A_wq, A_wo, B_x, B_w1, B_b1, B_w2, B_b2,
):
    SK = A_k_cache.shape[2]
    W = min(4096, max(256, SK // 4))
    NR = H * DH // 8

    def tiled(a):
        t = jnp.swapaxes(a, 2, 3).reshape(NR, 8, SK // 128, 128)
        return t.transpose(0, 2, 1, 3).reshape(NR // 2, 2, SK // 16, 128)

    b1 = B_b1.reshape(F // 128, 128)
    b2 = B_b2.reshape(D // 128, 128)
    anyspec = pl.BlockSpec(memory_space=pl.ANY)
    NCP = W // 256
    vreg = lambda n, dt: pltpu.VMEM(n + (8, 128), dt)
    return pl.pallas_call(
        _make_kernel(SK, W),
        out_shape=jax.ShapeDtypeStruct(A_x.shape, A_x.dtype),
        in_specs=[anyspec] * 9,
        out_specs=pl.BlockSpec(memory_space=pltpu.VMEM),
        scratch_shapes=[
            pltpu.VMEM((NR // 2, 2, W // 32, 128), u32),
            pltpu.VMEM((NR // 2 - 16, 2, W // 16, 128), bf16),
            pltpu.VMEM((16, 2, W // 32, 128), u32),
            vreg((NP * max(RF, 1), 2 * NCP), f32),
            pltpu.VMEM((H * DH // 128, D // 2, 128), u32),
            pltpu.VMEM((KD, H * DH // 2, 128), u32),
            pltpu.VMEM((KF, D // 2, 128), u32),
            pltpu.VMEM((KD, F // 2, 128), u32),
            pltpu.VMEM((1, 1, D), bf16),
            pltpu.VMEM((KF, 128), bf16),
            pltpu.VMEM((KD, 128), bf16),
            pltpu.VMEM((8, D), u32),
            pltpu.VMEM((8, 128), f32),
            vreg((KD,), f32),
            vreg((NCP,), f32),
        ] + [vreg((NT,), u32)] * 3
          + [vreg((NW,), f32)] * 4
          + [vreg((4 * XA, NT), f32)] * 2
          + [vreg((4, NT), f32)]
          + [vreg((NCP - 4 * XA, NT), f32)] * 2
          + [pltpu.VMEM((8, NCP * 128), f32)] * 2
          + [pltpu.VMEM((8, 128), f32)] * 4
          + [vreg((RP,), f32)] * 2
          + [vreg((NJ,), u32)] * 2
          + [vreg((NW,), f32)] * 2
          + [vreg((NCP,), u32)] * 2
          + [vreg((2, 2, NCP), f32)]
          + [pltpu.SMEM((NP,), jnp.int32)]
          + [pltpu.SemaphoreType.DMA((5,))],
        compiler_params=pltpu.CompilerParams(vmem_limit_bytes=128 * 1024 * 1024,
                                             disable_semaphore_checks=bool(NOSEM)),
    )(A_x, tiled(A_k_cache), tiled(A_v_cache), A_wq, A_wo, B_w1, b1, B_w2, b2)
```

```python
import functools
import jax
import jax.numpy as jnp
from jax import lax
import jax.experimental.pallas as pl
import jax.experimental.pallas.tpu as pltpu

D = 640
H = 32
DH = 192
F = 1536
NP = H // 2
PD = 2 * DH
RH = DH // 8
RP = 2 * RH
NJ = PD // 128
NT = 2 * NJ
KD = D // 128
KF = F // 128
NW = NJ * KD
EPS = 1e-5
LOG2E = 1.4426950408889634
bf16 = jnp.bfloat16
f32 = jnp.float32
u32 = jnp.uint32

RATE = 6.0
SPOS = 450
LPOS = 100
RPOS = 300
RSTEP = 80
YPOS = 5
IPOS = 150
IPOS14 = 10
IPOS15 = 10
SETS13 = "6,6,6,6,6,18"
CM = 2
RIN15 = 0
KPOS = 300
YP14 = 5
YP15 = 250
RS15 = 10
MORD13 = "hwlm"
RATE13 = 6.1
CPOS = 200
NL = 2
MORD = "hwql"
SSPILL = 0
PACE = 6
PACE13 = 3
D0 = 1
XA = 1
SETS = "10,10,10,18"
SETS14 = "4,4,4,4,16"
SETS15 = "8,8,10,6"
RATE14 = 6.7
RATE15 = 6.3
PACE14 = 3
PACE15 = 0
ONLY2 = 0
NOSEM = 0
STAGED = 0
GPOS = 30
GLAG = 60
ELAG = 80
MOFF = 0
LSTEP = 10
WOSTEP = 256
W2STEP = 192
W2SPLIT = "0,9,11,12"
RF = 8
F0 = 15
RP14 = 100
RP15 = 100
RS14 = 10
ORD14 = "gw"
WLAG = 2
ORD15 = "xw"
Q2EARLY = 1


def _center(x):
    xc = x - jnp.mean(x, axis=-1, keepdims=True)
    v = jnp.mean(xc * xc, axis=-1, keepdims=True)
    return xc, lax.rsqrt(v + EPS)


def _gelu(x):
    c = 0.7978845608028654
    return 0.5 * x * (1.0 + jnp.tanh(c * (x + 0.044715 * (x * x * x))))


def _pack_rows(x8):
    x16 = jnp.concatenate([x8, x8], axis=0).astype(bf16)
    return pltpu.bitcast(x16, u32)


def _tile_dot(lhs_u32, w_u32):
    return jnp.dot(pltpu.bitcast(lhs_u32, bf16), pltpu.bitcast(w_u32, bf16),
                   preferred_element_type=f32)[0:8]


def _tree(op, xs):
    xs = list(xs)
    while len(xs) > 1:
        xs = [op(xs[i], xs[i + 1]) if i + 1 < len(xs) else xs[i] for i in range(0, len(xs), 2)]
    return xs[0]


def _tree_sum(xs):
    return _tree(jnp.add, xs)


def _make_kernel(SK, W):
    NCP = W // 256
    CA = 4 * XA
    CB = NCP - CA
    c_exp = (DH ** -0.5) * LOG2E
    P = functools.partial

    def kernel(x_hbm, k_hbm, v_hbm, wq_hbm, wo_hbm, w1_hbm, b1_hbm, w2_hbm, b2_hbm,
               o_ref,
               kb, vb, vs, vx, vf, wqb, wob, w1b, w2b, xin, b1v, b2v, xl, rs_ref, ysum, ssum,
               ln0, ln1, lp, qr0, qr1, qr2, qr3, slo0, slo1, smid, shi0, shi1, pb0, pb1,
               ls0, ls1, li0, li1, ac0, ac1, ol0, ol1, yr0, yr1, pk0, pk1, xr, tbl, sems):
        ln, qr, slo, shi = (ln0, ln1), (qr0, qr1), (slo0, slo1), (shi0, shi1)
        pb, ls, li, ac, ol, yr = (pb0, pb1), (ls0, ls1), (li0, li1), (ac0, ac1), (ol0, ol1), (yr0, yr1)
        pk = (pk0, pk1)
        ku = k_hbm.bitcast(u32)
        vu = v_hbm.bitcast(u32)
        NC = NP // 2

        def kcopy(c, s):
            return pltpu.make_async_copy(
                ku.at[pl.ds(c * RP, RP), :, pl.ds((SK - W) // 32, W // 32), :],
                kb.at[pl.ds(c * RP, RP)], sems.at[s])

        RM = RH - RF // 2

        def vcopy(src0, n, dst, dst0, s):
            return pltpu.make_async_copy(
                v_hbm.at[pl.ds(src0, n), :, pl.ds((SK - W) // 16, W // 16), :],
                dst.at[pl.ds(dst0, n)], sems.at[s])

        def vstage(c):
            return [vcopy((2 * c + p) * RH + RM, RF // 2, vs, ((2 * c + p) & 3) * (RF // 2), 1 + (c & 1))
                    for p in range(2)]

        def wcopies(src, dst, s, r0=0, nrows=None, step=None):
            su = src.bitcast(u32)
            nrows = dst.shape[1] if nrows is None else nrows
            step = nrows if step is None else step
            return [pltpu.make_async_copy(su.at[pl.ds(r, step), pl.ds(n * 128, 128)],
                                          dst.at[n, pl.ds(r, step)], sems.at[s])
                    for r in range(r0, r0 + nrows, step) for n in range(dst.shape[0])]

        head = [pltpu.make_async_copy(x_hbm, xin, sems.at[0]),
                pltpu.make_async_copy(b1_hbm, b1v, sems.at[0]),
                pltpu.make_async_copy(b2_hbm, b2v, sems.at[0])]
        head += [pltpu.make_async_copy(
            vu.at[pl.ds((NP - 2 + s) * RH, 8), :, pl.ds((SK - W) // 32, W // 32), :],
            vx.at[pl.ds(8 * s, 8)], sems.at[0]) for s in range(2)]
        head += wcopies(wq_hbm, wqb, 0) + wcopies(wo_hbm, wob, 0, step=WOSTEP) + [kcopy(0, 0)]
        vlast = [vcopy((NP - 2 + s) * RH + 8, RM - 8, vb, (NP - 2) * RM + s * (RM - 8), 2) for s in range(2)]
        c1 = wcopies(w1_hbm, w1b, 1)
        w2_split = tuple(int(z) for z in W2SPLIT.split(','))
        c2 = [wcopies(w2_hbm, w2b, (0, 3, 4)[g], 64 * w2_split[g],
                      64 * (w2_split[g + 1] - w2_split[g]),
                      min(W2STEP, 64 * (w2_split[g + 1] - w2_split[g]))) for g in range(len(w2_split) - 1)]
        c2all = [c for g in c2 for c in g]
        for c in head:
            c.start()

        def chunk(c):
            s = 1 + (c & 1)
            return [kcopy(c + 1, s)] + [vcopy((2 * c + p) * RH, RM, vb, (2 * c + p) * RM, s) for p in range(2)]

        for c in chunk(0) + vstage(0) + chunk(1):
            c.start()

        for i_ in range(NP):
            tbl[i_] = i_

        def qproj_tile(wg, dst, n):
            j, kt = divmod(n, KD)
            dst[n] = _tile_dot(xl[:, pl.ds(kt * 128, 128)], wg[j, pl.ds(kt * 64, 64), :])

        def build_l(src, dst, j):
            row = lax.broadcasted_iota(jnp.int32, (8, 128), 0)
            lane = lax.broadcasted_iota(jnp.int32, (8, 128), 1)
            q = _tree_sum(src[j * KD + kt] for kt in range(KD)) * rs_ref[...]
            qp = pltpu.roll(q, 8, 1)
            qm = pltpu.roll(q, 120, 1)
            tgt = (lane >> 1) & 4
            if j == 1:
                tgt = tgt + (lane >> 6)
            elif j == 2:
                tgt = tgt + 1
            hit = row == tgt
            low = row < 4
            dst[2 * j] = _pack_rows(jnp.where(hit, jnp.where(low, q, qp), 0.0))
            dst[2 * j + 1] = _pack_rows(jnp.where(hit, jnp.where(low, qm, q), 0.0))

        def qk_tile(kg, lsrc, sdst, c0, n, ncp=NCP):
            c4, rem = divmod(n, 4 * NT)
            t, i = divmod(rem, min(4, ncp - c4 * 4))
            c = c4 * 4 + i
            w = kg[pl.ds((t // 2) * 8, 8), t % 2, pl.ds((c0 + c) * 8, 8), :].reshape(64, 128)
            sdst[c, t] = _tile_dot(lsrc[t], w)

        def s_group(st, src, c0, c1):
            s = [_tree_sum(src[c, t] for t in range(NT)) for c in range(c0, c1)]
            base = len(st.setdefault("s", []))
            if SSPILL:
                for k_, a_ in enumerate(s):
                    ssum[st.get("zero", 0) + base + k_] = a_
            st["s"] += s
            st["m"] = _tree(jnp.maximum, s + ([st["m"]] if "m" in st else []))

        def s_max(st):
            m = jnp.maximum(st["m"], pltpu.roll(st["m"], 4, 0))
            st["m"] = jnp.max(m, axis=1, keepdims=True)

        def s_exp(st, pdst, ldst, kdst=None):
            s = [ssum[cp] for cp in range(NCP)] if SSPILL else st["s"]
            e = [jnp.exp2(a - st["m"]) for a in s]
            for cp in range(NCP):
                pdst[:, pl.ds(cp * 128, 128)] = e[cp]
                if kdst is not None:
                    kdst[cp] = _pack_rows(e[cp])
            ldst[...] = _tree_sum(e)

        def softmax_steps(lo, hi, pdst, ldst, kdst=None, zero=None, mid=None):
            st = {} if zero is None else {"zero": zero}
            srcs = [(lo, CA), (hi, CB)] if mid is None else [(lo, CA), (mid, CM), (hi, CB - CM)]
            steps = [P(s_group, st, src, c0, min(c0 + 4, n)) for src, n in srcs for c0 in range(0, n, 4)]
            return steps + [P(s_max, st), P(s_exp, st, pdst, ldst, kdst)]

        def softmax(*args):
            for f in softmax_steps(*args):
                f()

        def l_inv(lsrc, ldst):
            l = lsrc[...]
            l = l + pltpu.roll(l, 4, 0)
            l = jnp.sum(l, axis=1, keepdims=True)
            ldst[...] = jnp.broadcast_to(1.0 / l, (8, 128))

        def pack_p(psrc, kdst):
            for cp in range(NCP):
                kdst[cp] = _pack_rows(psrc[:, pl.ds(cp * 128, 128)])

        def reduce_o(asrc, lsrc, odst, j):
            blk = asrc[pl.ds(j * 16, 16)].reshape(128, 128)
            t = blk.T.reshape(16, 8, 128)
            if j == 1:
                lane = lax.broadcasted_iota(jnp.int32, (1, 128), 1)
                r = jnp.where(lane < 64, lsrc[0:1, :], lsrc[1:2, :])
            else:
                r = lsrc[j // 2:j // 2 + 1, :]
            odst[j] = _pack_rows(_tree_sum(t[i] for i in range(16)) * r)

        def x_tile(vg, n):
            s, rem = divmod(n, 2 * NCP)
            cp, e = divmod(rem, 2)
            w = vg[pl.ds(8 * s, 8), e, pl.ds(cp * 8, 8), :].reshape(64, 128)
            xr[s, e, cp] = _tile_dot(pk[s][cp], w)

        def x_finish(s):
            row = lax.broadcasted_iota(jnp.int32, (8, 128), 0)
            lane = lax.broadcasted_iota(jnp.int32, (8, 128), 1)
            o0 = _tree_sum(xr[s, 0, cp] for cp in range(NCP))
            o1 = _tree_sum(xr[s, 1, cp] for cp in range(NCP))
            low = row < 4
            direct = jnp.where(low, o0, o1)
            moved = jnp.where(low, pltpu.roll(o1, 8, 1), pltpu.roll(o0, 120, 1))
            o = jnp.where(((lane >> 1) & 4) == (row & 4), direct, moved)
            ol[s][0] = _pack_rows(jnp.where((row & 3) == 0, o, 0.0) * li[s][0:1, :])

        def wo_tile(wg, osrc, ydst, n):
            j, nt = divmod(n, KD)
            ydst[n] = _tile_dot(osrc[j], wg[nt, pl.ds(j * 64, 64), :])

        def y_fold(ysrc):
            for nt in range(KD):
                ysum[nt] = _tree_sum([ysum[nt]] + [ysrc[j * KD + nt] for j in range(NJ)])

        def copy(src, dst):
            for i in range(src.shape[0]):
                dst[i] = src[i]

        def kpair(i):
            return kb.at[pl.ds(i * RH, RH)]

        def wqpair(i):
            return wqb.at[pl.ds(i * NJ, NJ)]

        def wopair(i):
            r0 = i * (PD // 2)
            if not isinstance(i, int):
                r0 = pl.multiple_of(r0, PD // 2)
            return wob.at[:, pl.ds(r0, PD // 2), :]

        def run_block(first, i, a, rg0, sets, kinds, order, rate, pace_n, side, moff=0):
            if rg0:
                vg = vb.at[pl.ds((NP - 2) * RM + a * (RM - 8), RM - 8)]
            else:
                vg = vb.at[pl.ds(i * RM, RM)]
            voff = rg0 // 2
            sg = vs.at[pl.ds((i & 3) * (RF // 2), RF // 2)]
            fg = vf.at[pl.ds(i * RF, RF)]
            plain, order_rg = list(range(rg0, RP - RF)), []
            n_all = RP - rg0
            f0 = min(F0, n_all - RF) * n_all // RP
            slots = {f0 + (k_ + 1) * (n_all - f0) // RF - 1 for k_ in range(RF)}
            nf = 0
            for pos_ in range(n_all):
                if pos_ in slots:
                    order_rg.append(RP - RF + nf)
                    nf += 1
                else:
                    order_rg.append(plain.pop(0))
            pace = dict(z=i, cnt=0, views={})

            def mxu_tile(key, n):
                if pace_n and pace["cnt"] % pace_n == 0:
                    z = pace["z"]
                    link = pace["cnt"] // pace_n
                    for _ in range(pace_n * 4 // 3 if link else D0):
                        z = tbl[z]
                    pace["z"] = z
                    pace["views"] = {}
                pace["cnt"] += 1
                if key not in pace["views"]:
                    pace["views"][key] = kinds[key][1](pace["z"])
                kinds[key][2](pace["views"][key], n)

            mxu = [P(mxu_tile, key, n) for key in order for n in range(kinds[key][0])]
            side = sorted(side + [(moff + int(n * rate), f) for n, f in enumerate(mxu)], key=lambda z: z[0])
            cnt = 0
            si = 0
            acc = {}
            sizes, ovl = sets.split(":") if ":" in sets else (sets, "0")
            groups = []
            for size in (int(z) for z in sizes.split(",")):
                groups.append(order_rg[:size])
                order_rg = order_rg[size:]
            step = NCP - int(ovl)
            seq = [(rgs, t - gi * step) for t in range((len(groups) - 1) * step + NCP)
                   for gi, rgs in enumerate(groups) if 0 <= t - gi * step < NCP]
            for rgs, cp in seq:
                mult = {hh: (pb[a][pl.ds(hh, 1), pl.ds(cp * 128, 128)],
                             pb[a][pl.ds(4 + hh, 1), pl.ds(cp * 128, 128)])
                        for hh in sorted({rg // RH for rg in rgs})}
                for rg in rgs:
                    while si < len(side) and side[si][0] <= cnt:
                        side[si][1]()
                        si += 1
                    cnt += 1
                    m0, m1 = mult[rg // RH]
                    r = rg - (RP - RF)
                    if r >= 0 and not first:
                        v0, v1 = fg[r, 2 * cp], fg[r, 2 * cp + 1]
                    else:
                        src = sg.at[r // 2, r % 2] if r >= 0 else vg.at[rg // 2 - voff, rg % 2]
                        v = src[pl.ds(cp * 16, 16), :].astype(f32)
                        v0, v1 = v[:8], v[8:]
                        if r >= 0:
                            fg[r, 2 * cp] = v0
                            fg[r, 2 * cp + 1] = v1
                    if rg not in acc:
                        acc[rg] = v0 * m0 + v1 * m1
                    else:
                        acc[rg] = acc[rg] + v0 * m0 + v1 * m1
                    if cp == NCP - 1:
                        ac[a][rg] = acc[rg]
            assert not order_rg
            for _, f in side[si:]:
                f()

        def layer(x, first):
            xc, rs = _center(x)
            xl[...] = _pack_rows(xc)
            rs_ref[...] = jnp.broadcast_to(rs * c_exp, (8, 128))
            ac1[...] = jnp.zeros(ac1.shape, f32)
            li1[...] = jnp.zeros(li1.shape, f32)
            if WLAG == 1:
                yr0[...] = jnp.zeros(yr0.shape, f32)
            else:
                ol0[...] = jnp.zeros(ol0.shape, u32)
                yr1[...] = jnp.zeros(yr1.shape, f32)
            ysum[...] = jnp.zeros(ysum.shape, f32)

            for i, dst in enumerate((qr2, qr3)):
                for n in range(NW):
                    qproj_tile(wqpair(i), dst, n)
            if Q2EARLY:
                for n in range(NW):
                    qproj_tile(wqpair(2), qr0, n)
            for j in range(NJ):
                build_l(qr2, lp, j)
            for n in range(CA * NT):
                qk_tile(kpair(0), lp, slo0, 0, n)
            for n in range(CB * NT):
                qk_tile(kpair(0), lp, shi0, CA, n)
            for j in range(NJ):
                build_l(qr3, ln1, j)
            for n in range(CA * NT):
                qk_tile(kpair(1), ln1, slo1, 0, n)
            if not Q2EARLY:
                for n in range(NW):
                    qproj_tile(wqpair(2), qr0, n)
            softmax(slo0, shi0, pb0, ls0)

            wp = lambda a: 1 - a if WLAG == 1 else a

            def kinds(a):
                b = 1 - a
                return dict(
                    h=(CB * NT, lambda z: kpair(z + 1),
                       lambda w, n: qk_tile(w, ln[b], shi[b], CA, n)),
                    l=(CA * NT, lambda z: kpair(z + 2),
                       lambda w, n: qk_tile(w, ln[a], slo[a], 0, n)),
                    q=(NW, lambda z: wqpair(jnp.minimum(z + 3, NP - 1)),
                       lambda w, n: qproj_tile(w, qr[b], n)),
                    w=(NW, lambda z: wopair(jnp.maximum(z - WLAG, 0)),
                       lambda w, n: wo_tile(w, ol[wp(a)], yr[wp(a)], n)),
                    v=(2 * KD, lambda z: wopair(z - 1),
                       lambda w, n: wo_tile(w, ol[b], yr[b], KD + n)),
                    m=(CM * NT, lambda z: kpair(z + 2),
                       lambda w, n: qk_tile(w, ln[a], smid, CA, n, CM)),
                    g=((CB - CM) * NT, lambda z: kpair(z + 1),
                       lambda w, n: qk_tile(w, ln[b], shi[b], CA + CM, n, CB - CM)),
                    x=(4 * NCP, lambda z: vx.at[pl.ds((z - (NP - 1)) * 16, 16)], x_tile))

            def block(i, a, order=MORD, RATE=RATE, SETS=SETS, PACE=PACE):
                b = 1 - a
                steps = softmax_steps(slo[b], shi[b], pb[b], ls[b], None, tbl[i] - i if SSPILL == 2 else None)
                if STAGED:
                    pos = [GPOS] * XA + [MOFF + int(24 * (k_ + 1) * RATE) + GLAG for k_ in range(4 - XA)]
                    pos += [pos[-1] + 1, pos[-1] + ELAG]
                else:
                    pos = [max(SPOS, MOFF + int(CB * NT * RATE) + 1)] * len(steps)
                side = list(zip(pos, steps))
                side += [(IPOS, P(l_inv, ls[a], li[a])),
                         (YPOS, P(y_fold, yr[1 - wp(a)]))]
                for j in range(NJ):
                    side.append((LPOS + LSTEP * j, P(build_l, qr[a], ln[a], j)))
                    side.append((RPOS + RSTEP * j, P(reduce_o, ac[b], li[b], ol[b], j)))
                run_block(first, i, a, 0, SETS, kinds(a), order, RATE, PACE, side, MOFF)

            def block14(i):
                side = [(int(((CB - CM) * NT + NW) * RATE14) + 10, P(softmax, slo1, shi1, pb1, ls1, pk1, None, smid)),
                        (IPOS14, P(l_inv, ls0, li0)),
                        (KPOS, P(pack_p, pb0, pk0)),
                        (YP14, P(y_fold, yr[1 - wp(0)]))]
                for j in range(NJ):
                    side.append((RP14 + RS14 * j, P(reduce_o, ac1, li1, ol1, j)))
                run_block(first, i, 0, 16, SETS14, kinds(0), ORD14, RATE14, PACE14, side)

            def block15(i):
                side = [(IPOS15, P(l_inv, ls1, li1)),
                        (YP15, P(y_fold, yr[1 - wp(1)]))]
                for j in range(1, NJ):
                    side.append((RP15 + RS15 * j, P(reduce_o, ac0, li0, ol0, j)))
                if RIN15 >= 1:
                    side.append((16 * NCP + 1, P(reduce_o, ac1, li1, ol1, 1)))
                if RIN15 >= 2:
                    side.append((32 * NCP + 1, P(reduce_o, ac1, li1, ol1, 2)))
                run_block(first, i, 1, 16, SETS15, kinds(1), ORD15, RATE15, PACE15, side)

            def body(i, c):
                if first:
                    @pl.when((i & 1) == 0)
                    def _():
                        ch = lax.shift_right_logical(i, 1)
                        for c in chunk(ch) + vstage(ch):
                            c.wait()
                        for c in vstage(ch + 1):
                            c.start()

                        @pl.when(ch + 2 < NC - 1)
                        def _():
                            for c in chunk(ch + 2):
                                c.start()

                        @pl.when(ch + 2 == NC - 1)
                        def _():
                            for c in vlast:
                                c.start()

                        @pl.when(ch + 1 == NC - 1)
                        def _():
                            for c in c1 + c2all:
                                c.start()

                for a in range(2):
                    pl.when((i & 1) == a)(P(block, i, a))
                return c

            lax.fori_loop(0, NP - 3, body, 0)

            def tail(i, c):
                pl.when(i == NP - 3)(P(block, i, 1, MORD13, RATE13, SETS13, PACE13))
                if first:
                    @pl.when(i == NP - 2)
                    def _():
                        for c in vlast + vstage(NC - 1):
                            c.wait()

                pl.when(i == NP - 2)(P(block14, i))
                pl.when(i == NP - 1)(P(block15, i))
                return c

            lax.fori_loop(NP - 3, NP, tail, 0)

            x_finish(0)
            x_finish(1)
            for j in range(1 + RIN15, NJ):
                reduce_o(ac1, li1, ol1, j)
            for n in (range(KD) if WLAG == 1 else list(range(KD, NW)) + list(range(KD))):
                wo_tile(wopair(NP - 2), ol0, yr0, n)
            for n in range(NW):
                wo_tile(wopair(NP - 1), ol1, qr0, n)
            ys = [_tree_sum([ysum[nt]] + [src[j * KD + nt] for src in ((yr0, qr0) if WLAG == 1 else (yr1, yr0, qr0)) for j in range(NJ)])
                  for nt in range(KD)]
            y = jnp.sum(jnp.concatenate(ys, axis=1), axis=0, keepdims=True)
            x = x + y

            xc, rs = _center(x)
            xn = _pack_rows(xc)
            if first:
                for c in c1:
                    c.wait()
            hs = []
            for n in range(KF):
                h = _tree_sum(_tile_dot(xn[:, kt * 128:(kt + 1) * 128], w1b[n, pl.ds(kt * 64, 64), :])
                              for kt in range(KD))
                hs.append(_pack_rows(_gelu(h * rs + b1v[n:n + 1, :].astype(f32))))
            parts = []
            for kt in range(KF):
                if first and kt in w2_split:
                    for c in c2[w2_split.index(kt)]:
                        c.wait()
                parts.append([_tile_dot(hs[kt], w2b[nt, pl.ds(kt * 64, 64), :]) for nt in range(KD)])
            y2 = jnp.concatenate(
                [_tree_sum(parts[kt][nt] for kt in range(KF)) + b2v[nt:nt + 1, :].astype(f32)
                 for nt in range(KD)], axis=1)
            return x + y2

        for c in head:
            c.wait()

        def transpose_tile(n, c):
            s8 = pl.multiple_of((n // (2 * NCP)) * 8, 8)
            e = n % 2
            c8 = pl.multiple_of(((n // 2) % NCP) * 8, 8)
            w = vx[pl.ds(s8, 8), e, pl.ds(c8, 8), :].reshape(64, 128)
            wt = pltpu.bitcast(w, bf16).astype(f32).T.astype(bf16)
            vx[pl.ds(s8, 8), e, pl.ds(c8, 8), :] = pltpu.bitcast(wt, u32).reshape(8, 8, 128)
            return c

        lax.fori_loop(0, 4 * NCP, transpose_tile, 0)

        if ONLY2:
            for c in chunk(0) + vstage(0) + chunk(1):
                c.wait()
        x = jnp.broadcast_to(xin[0].astype(f32), (8, D))
        for l_ in range(1 if ONLY2 else NL):
            x = layer(x, l_ == 0 and not ONLY2)
        o_ref[0] = x[0:1, :].astype(o_ref.dtype)

    return kernel


@jax.jit
def pallas_interleave_layers__sliding_block_cached__dense_activation_gelu__decode_kernel(
    A_x, A_k_cache, A_v_cache, A_wq, A_wo, B_x, B_w1, B_b1, B_w2, B_b2,
):
    SK = A_k_cache.shape[2]
    W = min(4096, max(256, SK // 4))
    NR = H * DH // 8

    def tiled(a):
        t = jnp.swapaxes(a, 2, 3).reshape(NR, 8, SK // 128, 128)
        return t.transpose(0, 2, 1, 3).reshape(NR // 2, 2, SK // 16, 128)

    b1 = B_b1.reshape(F // 128, 128)
    b2 = B_b2.reshape(D // 128, 128)
    anyspec = pl.BlockSpec(memory_space=pl.ANY)
    NCP = W // 256
    vreg = lambda n, dt: pltpu.VMEM(n + (8, 128), dt)
    return pl.pallas_call(
        _make_kernel(SK, W),
        out_shape=jax.ShapeDtypeStruct(A_x.shape, A_x.dtype),
        in_specs=[anyspec] * 9,
        out_specs=pl.BlockSpec(memory_space=pltpu.VMEM),
        scratch_shapes=[
            pltpu.VMEM((NR // 2, 2, W // 32, 128), u32),
            pltpu.VMEM((NR // 2 - 16 - NP * RF // 2, 2, W // 16, 128), bf16),
            pltpu.VMEM((2 * RF, 2, W // 16, 128), bf16),
            pltpu.VMEM((16, 2, W // 32, 128), u32),
            vreg((NP * max(RF, 1), 2 * NCP), f32),
            pltpu.VMEM((H * DH // 128, D // 2, 128), u32),
            pltpu.VMEM((KD, H * DH // 2, 128), u32),
            pltpu.VMEM((KF, D // 2, 128), u32),
            pltpu.VMEM((KD, F // 2, 128), u32),
            pltpu.VMEM((1, 1, D), bf16),
            pltpu.VMEM((KF, 128), bf16),
            pltpu.VMEM((KD, 128), bf16),
            pltpu.VMEM((8, D), u32),
            pltpu.VMEM((8, 128), f32),
            vreg((KD,), f32),
            vreg((NCP,), f32),
        ] + [vreg((NT,), u32)] * 3
          + [vreg((NW,), f32)] * 4
          + [vreg((4 * XA, NT), f32)] * 2
          + [vreg((4, NT), f32)]
          + [vreg((NCP - 4 * XA, NT), f32)] * 2
          + [pltpu.VMEM((8, NCP * 128), f32)] * 2
          + [pltpu.VMEM((8, 128), f32)] * 4
          + [vreg((RP,), f32)] * 2
          + [vreg((NJ,), u32)] * 2
          + [vreg((NW,), f32)] * 2
          + [vreg((NCP,), u32)] * 2
          + [vreg((2, 2, NCP), f32)]
          + [pltpu.SMEM((NP,), jnp.int32)]
          + [pltpu.SemaphoreType.DMA((5,))],
        compiler_params=pltpu.CompilerParams(vmem_limit_bytes=128 * 1024 * 1024,
                                             disable_semaphore_checks=bool(NOSEM)),
    )(A_x, tiled(A_k_cache), tiled(A_v_cache), A_wq, A_wo, B_w1, b1, B_w2, b2)
```

```python
import functools
import jax
import jax.numpy as jnp
from jax import lax
import jax.experimental.pallas as pl
import jax.experimental.pallas.tpu as pltpu

D = 640
H = 32
DH = 192
F = 1536
NP = H // 2
PD = 2 * DH
RH = DH // 8
RP = 2 * RH
NJ = PD // 128
NT = 2 * NJ
KD = D // 128
KF = F // 128
NW = NJ * KD
EPS = 1e-5
LOG2E = 1.4426950408889634
bf16 = jnp.bfloat16
f32 = jnp.float32
u32 = jnp.uint32

RATE = 6.0
SPOS = 450
LPOS = 100
RPOS = 300
RSTEP = 80
YPOS = 5
IPOS = 150
IPOS14 = 10
IPOS15 = 10
SETS13 = "6,6,6,6,6,18"
CM = 2
RIN15 = 0
NV2 = 5
NV1 = 3
CIN = 0
ONEPASS = 0
KPOS = 300
YP14 = 5
YP15 = 250
RS15 = 10
MORD13 = "hwlm"
RATE13 = 6.1
CPOS = 200
NL = 2
MORD = "hwql"
SSPILL = 0
PACE = 6
PACE13 = 3
D0 = 1
XA = 1
SETS = "10,10,10,18"
SETS14 = "4,4,4,4,16"
SETS15 = "8,8,10,6"
RATE14 = 6.7
RATE15 = 6.3
PACE14 = 3
PACE15 = 0
ONLY2 = 0
NOSEM = 0
STAGED = 0
GPOS = 30
GLAG = 60
ELAG = 80
MOFF = 0
LSTEP = 10
WOSTEP = 256
W2STEP = 192
W2SPLIT = "0,9,11,12"
RF = 8
F0 = 15
RP14 = 100
RP15 = 100
RS14 = 10
ORD14 = "gw"
WLAG = 2
ORD15 = "xw"
Q2EARLY = 1


def _center(x, mean=None):
    if mean is not None:
        xc = x - mean
        v = jnp.mean(xc * xc, axis=-1, keepdims=True)
        return xc, lax.rsqrt(v + EPS)
    if ONEPASS:
        m = jnp.mean(x, axis=-1, keepdims=True)
        v = jnp.maximum(jnp.mean(x * x, axis=-1, keepdims=True) - m * m, 0.0)
        return x - m, lax.rsqrt(v + EPS)
    xc = x - jnp.mean(x, axis=-1, keepdims=True)
    v = jnp.mean(xc * xc, axis=-1, keepdims=True)
    return xc, lax.rsqrt(v + EPS)


def _gelu(x):
    c = 0.7978845608028654
    return 0.5 * x * (1.0 + jnp.tanh(c * (x + 0.044715 * (x * x * x))))


def _pack_rows(x8):
    x16 = jnp.concatenate([x8, x8], axis=0).astype(bf16)
    return pltpu.bitcast(x16, u32)


def _tile_dot(lhs_u32, w_u32):
    return jnp.dot(pltpu.bitcast(lhs_u32, bf16), pltpu.bitcast(w_u32, bf16),
                   preferred_element_type=f32)[0:8]


def _columns(x8):
    return jnp.concatenate([x8] * 16, axis=0).T


def _sublane_sum(x8):
    for sh in (4, 2, 1):
        x8 = x8 + pltpu.roll(x8, sh, 0)
    return x8


def _tree(op, xs):
    xs = list(xs)
    while len(xs) > 1:
        xs = [op(xs[i], xs[i + 1]) if i + 1 < len(xs) else xs[i] for i in range(0, len(xs), 2)]
    return xs[0]


def _tree_sum(xs):
    return _tree(jnp.add, xs)


def _make_kernel(SK, W):
    NCP = W // 256
    CA = 4 * XA
    CB = NCP - CA
    c_exp = (DH ** -0.5) * LOG2E
    P = functools.partial

    def kernel(x_hbm, k_hbm, v_hbm, wq_hbm, wo_hbm, w1_hbm, b1_hbm, w2_hbm, b2_hbm,
               o_ref,
               kb, vb, vs, vx, vf, wqb, wob, w1b, w2b, xin, b1v, b2v, xl, rs_ref, ysum, ssum,
               ln0, ln1, lp, qr0, qr1, qr2, qr3, slo0, slo1, smid, shi0, shi1, pb0, pb1,
               ls0, ls1, li0, li1, ac0, ac1, ol0, ol1, yr0, yr1, pk0, pk1, xr, wsc, wsl, tbl, sems):
        ln, qr, slo, shi = (ln0, ln1), (qr0, qr1), (slo0, slo1), (shi0, shi1)
        pb, ls, li, ac, ol, yr = (pb0, pb1), (ls0, ls1), (li0, li1), (ac0, ac1), (ol0, ol1), (yr0, yr1)
        pk = (pk0, pk1)
        ku = k_hbm.bitcast(u32)
        vu = v_hbm.bitcast(u32)
        NC = NP // 2

        def kcopy(c, s):
            return pltpu.make_async_copy(
                ku.at[pl.ds(c * RP, RP), :, pl.ds((SK - W) // 32, W // 32), :],
                kb.at[pl.ds(c * RP, RP)], sems.at[s])

        RM = RH - RF // 2

        def vcopy(src0, n, dst, dst0, s):
            return pltpu.make_async_copy(
                v_hbm.at[pl.ds(src0, n), :, pl.ds((SK - W) // 16, W // 16), :],
                dst.at[pl.ds(dst0, n)], sems.at[s])

        def vstage(c):
            return [vcopy((2 * c + p) * RH + RM, RF // 2, vs, ((2 * c + p) & 3) * (RF // 2), 1 + (c & 1))
                    for p in range(2)]

        def wcopies(src, dst, s, r0=0, nrows=None, step=None):
            su = src.bitcast(u32)
            nrows = dst.shape[1] if nrows is None else nrows
            step = nrows if step is None else step
            return [pltpu.make_async_copy(su.at[pl.ds(r, step), pl.ds(n * 128, 128)],
                                          dst.at[n, pl.ds(r, step)], sems.at[s])
                    for r in range(r0, r0 + nrows, step) for n in range(dst.shape[0])]

        head = [pltpu.make_async_copy(x_hbm, xin, sems.at[0]),
                pltpu.make_async_copy(b1_hbm, b1v, sems.at[0]),
                pltpu.make_async_copy(b2_hbm, b2v, sems.at[0])]
        head += [pltpu.make_async_copy(
            vu.at[pl.ds((NP - 2 + s) * RH, 8), :, pl.ds((SK - W) // 32, W // 32), :],
            vx.at[pl.ds(8 * s, 8)], sems.at[0]) for s in range(2)]
        head += wcopies(wq_hbm, wqb, 0) + wcopies(wo_hbm, wob, 0, step=WOSTEP) + [kcopy(0, 0)]
        vlast = [vcopy((NP - 2 + s) * RH + 8, RM - 8, vb, (NP - 2) * RM + s * (RM - 8), 2) for s in range(2)]
        c1 = wcopies(w1_hbm, w1b, 1)
        w2_split = tuple(int(z) for z in W2SPLIT.split(','))
        c2 = [wcopies(w2_hbm, w2b, (0, 3, 4)[g], 64 * w2_split[g],
                      64 * (w2_split[g + 1] - w2_split[g]),
                      min(W2STEP, 64 * (w2_split[g + 1] - w2_split[g]))) for g in range(len(w2_split) - 1)]
        c2all = [c for g in c2 for c in g]
        for c in head:
            c.start()

        def chunk(c):
            s = 1 + (c & 1)
            return [kcopy(c + 1, s)] + [vcopy((2 * c + p) * RH, RM, vb, (2 * c + p) * RM, s) for p in range(2)]

        for c in chunk(0) + vstage(0) + chunk(1):
            c.start()

        for i_ in range(NP):
            tbl[i_] = i_

        def qproj_tile(wg, dst, n):
            j, kt = divmod(n, KD)
            dst[n] = _tile_dot(xl[:, pl.ds(kt * 128, 128)], wg[j, pl.ds(kt * 64, 64), :])

        def build_l(src, dst, j):
            row = lax.broadcasted_iota(jnp.int32, (8, 128), 0)
            lane = lax.broadcasted_iota(jnp.int32, (8, 128), 1)
            q = _tree_sum(src[j * KD + kt] for kt in range(KD)) * rs_ref[...]
            qp = pltpu.roll(q, 8, 1)
            qm = pltpu.roll(q, 120, 1)
            tgt = (lane >> 1) & 4
            if j == 1:
                tgt = tgt + (lane >> 6)
            elif j == 2:
                tgt = tgt + 1
            hit = row == tgt
            low = row < 4
            dst[2 * j] = _pack_rows(jnp.where(hit, jnp.where(low, q, qp), 0.0))
            dst[2 * j + 1] = _pack_rows(jnp.where(hit, jnp.where(low, qm, q), 0.0))

        def qk_tile(kg, lsrc, sdst, c0, n, ncp=NCP):
            c4, rem = divmod(n, 4 * NT)
            t, i = divmod(rem, min(4, ncp - c4 * 4))
            c = c4 * 4 + i
            w = kg[pl.ds((t // 2) * 8, 8), t % 2, pl.ds((c0 + c) * 8, 8), :].reshape(64, 128)
            sdst[c, t] = _tile_dot(lsrc[t], w)

        def s_group(st, src, c0, c1):
            s = [_tree_sum(src[c, t] for t in range(NT)) for c in range(c0, c1)]
            base = len(st.setdefault("s", []))
            if SSPILL:
                for k_, a_ in enumerate(s):
                    ssum[st.get("zero", 0) + base + k_] = a_
            st["s"] += s
            st["m"] = _tree(jnp.maximum, s + ([st["m"]] if "m" in st else []))

        def s_max(st):
            m = jnp.maximum(st["m"], pltpu.roll(st["m"], 4, 0))
            st["m"] = jnp.max(m, axis=1, keepdims=True)

        def s_exp(st, pdst, ldst, kdst=None):
            s = [ssum[cp] for cp in range(NCP)] if SSPILL else st["s"]
            e = [jnp.exp2(a - st["m"]) for a in s]
            for cp in range(NCP):
                pdst[:, pl.ds(cp * 128, 128)] = e[cp]
                if kdst is not None:
                    kdst[cp] = _pack_rows(e[cp])
            ldst[...] = _tree_sum(e)

        def softmax_steps(lo, hi, pdst, ldst, kdst=None, zero=None, mid=None):
            st = {} if zero is None else {"zero": zero}
            srcs = [(lo, CA), (hi, CB)] if mid is None else [(lo, CA), (mid, CM), (hi, CB - CM)]
            steps = [P(s_group, st, src, c0, min(c0 + 4, n)) for src, n in srcs for c0 in range(0, n, 4)]
            return steps + [P(s_max, st), P(s_exp, st, pdst, ldst, kdst)]

        def softmax(*args):
            for f in softmax_steps(*args):
                f()

        def l_inv(lsrc, ldst):
            l = lsrc[...]
            l = l + pltpu.roll(l, 4, 0)
            l = jnp.sum(l, axis=1, keepdims=True)
            ldst[...] = jnp.broadcast_to(1.0 / l, (8, 128))

        def pack_p(psrc, kdst):
            for cp in range(NCP):
                kdst[cp] = _pack_rows(psrc[:, pl.ds(cp * 128, 128)])

        def reduce_o(asrc, lsrc, odst, j):
            blk = asrc[pl.ds(j * 16, 16)].reshape(128, 128)
            t = blk.T.reshape(16, 8, 128)
            if j == 1:
                lane = lax.broadcasted_iota(jnp.int32, (1, 128), 1)
                r = jnp.where(lane < 64, lsrc[0:1, :], lsrc[1:2, :])
            else:
                r = lsrc[j // 2:j // 2 + 1, :]
            odst[j] = _pack_rows(_tree_sum(t[i] for i in range(16)) * r)

        def x_tile(vg, n):
            s, rem = divmod(n, 2 * NCP)
            cp, e = divmod(rem, 2)
            w = vg[pl.ds(8 * s, 8), e, pl.ds(cp * 8, 8), :].reshape(64, 128)
            xr[s, e, cp] = _tile_dot(pk[s][cp], w)

        def x_finish(s):
            row = lax.broadcasted_iota(jnp.int32, (8, 128), 0)
            lane = lax.broadcasted_iota(jnp.int32, (8, 128), 1)
            o0 = _tree_sum(xr[s, 0, cp] for cp in range(NCP))
            o1 = _tree_sum(xr[s, 1, cp] for cp in range(NCP))
            low = row < 4
            direct = jnp.where(low, o0, o1)
            moved = jnp.where(low, pltpu.roll(o1, 8, 1), pltpu.roll(o0, 120, 1))
            o = jnp.where(((lane >> 1) & 4) == (row & 4), direct, moved)
            o = jnp.where((row & 3) == 0, o, 0.0) * li[s][0:1, :]
            ol[s][0] = _pack_rows(o)
            return o

        def wo_tile(wg, osrc, ydst, n):
            j, nt = divmod(n, KD)
            ydst[n] = _tile_dot(osrc[j], wg[nt, pl.ds(j * 64, 64), :])

        def y_fold(ysrc):
            for nt in range(KD):
                ysum[nt] = _tree_sum([ysum[nt]] + [ysrc[j * KD + nt] for j in range(NJ)])

        def copy(src, dst):
            for i in range(src.shape[0]):
                dst[i] = src[i]

        def kpair(i):
            return kb.at[pl.ds(i * RH, RH)]

        def wqpair(i):
            return wqb.at[pl.ds(i * NJ, NJ)]

        def wopair(i):
            r0 = i * (PD // 2)
            if not isinstance(i, int):
                r0 = pl.multiple_of(r0, PD // 2)
            return wob.at[:, pl.ds(r0, PD // 2), :]

        def run_block(first, i, a, rg0, sets, kinds, order, rate, pace_n, side, moff=0, done=None):
            if rg0:
                vg = vb.at[pl.ds((NP - 2) * RM + a * (RM - 8), RM - 8)]
            else:
                vg = vb.at[pl.ds(i * RM, RM)]
            voff = rg0 // 2
            sg = vs.at[pl.ds((i & 3) * (RF // 2), RF // 2)]
            fg = vf.at[pl.ds(i * RF, RF)]
            plain, order_rg = list(range(rg0, RP - RF)), []
            n_all = RP - rg0
            f0 = min(F0, n_all - RF) * n_all // RP
            slots = {f0 + (k_ + 1) * (n_all - f0) // RF - 1 for k_ in range(RF)}
            nf = 0
            for pos_ in range(n_all):
                if pos_ in slots:
                    order_rg.append(RP - RF + nf)
                    nf += 1
                else:
                    order_rg.append(plain.pop(0))
            pace = dict(z=i, cnt=0, views={})

            def mxu_tile(key, n):
                if pace_n and pace["cnt"] % pace_n == 0:
                    z = pace["z"]
                    link = pace["cnt"] // pace_n
                    for _ in range(pace_n * 4 // 3 if link else D0):
                        z = tbl[z]
                    pace["z"] = z
                    pace["views"] = {}
                pace["cnt"] += 1
                if key not in pace["views"]:
                    pace["views"][key] = kinds[key][1](pace["z"])
                kinds[key][2](pace["views"][key], n)

            mxu = [P(mxu_tile, key, n) for key in order for n in range(kinds[key][0])]
            side = sorted(side + [(moff + int(n * rate), f) for n, f in enumerate(mxu)], key=lambda z: z[0])
            cnt = 0
            si = 0
            acc = {}
            sizes, ovl = sets.split(":") if ":" in sets else (sets, "0")
            groups = []
            for size in (int(z) for z in sizes.split(",")):
                groups.append(order_rg[:size])
                order_rg = order_rg[size:]
            step = NCP - int(ovl)
            seq = [(rgs, t - gi * step) for t in range((len(groups) - 1) * step + NCP)
                   for gi, rgs in enumerate(groups) if 0 <= t - gi * step < NCP]
            for rgs, cp in seq:
                mult = {hh: (pb[a][pl.ds(hh, 1), pl.ds(cp * 128, 128)],
                             pb[a][pl.ds(4 + hh, 1), pl.ds(cp * 128, 128)])
                        for hh in sorted({rg // RH for rg in rgs})}
                for rg in rgs:
                    while si < len(side) and side[si][0] <= cnt:
                        side[si][1]()
                        si += 1
                    cnt += 1
                    m0, m1 = mult[rg // RH]
                    r = rg - (RP - RF)
                    if r >= 0 and not first:
                        v0, v1 = fg[r, 2 * cp], fg[r, 2 * cp + 1]
                    else:
                        src = sg.at[r // 2, r % 2] if r >= 0 else vg.at[rg // 2 - voff, rg % 2]
                        v = src[pl.ds(cp * 16, 16), :].astype(f32)
                        v0, v1 = v[:8], v[8:]
                        if r >= 0:
                            fg[r, 2 * cp] = v0
                            fg[r, 2 * cp + 1] = v1
                    if rg not in acc:
                        acc[rg] = v0 * m0 + v1 * m1
                    else:
                        acc[rg] = acc[rg] + v0 * m0 + v1 * m1
                    if cp == NCP - 1:
                        ac[a][rg] = acc[rg]
                        if done is not None and cnt <= CIN * NCP:
                            done(rg)
            assert not order_rg
            for _, f in side[si:]:
                f()

        def layer(x, first):
            xc, rs = _center(x)
            xl[...] = _pack_rows(xc)
            rs_ref[...] = jnp.broadcast_to(rs * c_exp, (8, 128))
            ac1[...] = jnp.zeros(ac1.shape, f32)
            li1[...] = jnp.zeros(li1.shape, f32)
            if WLAG == 1:
                yr0[...] = jnp.zeros(yr0.shape, f32)
            else:
                ol0[...] = jnp.zeros(ol0.shape, u32)
                yr1[...] = jnp.zeros(yr1.shape, f32)
            ysum[...] = jnp.zeros(ysum.shape, f32)

            for i, dst in enumerate((qr2, qr3)):
                for n in range(NW):
                    qproj_tile(wqpair(i), dst, n)
            if Q2EARLY:
                for n in range(NW):
                    qproj_tile(wqpair(2), qr0, n)
            for j in range(NJ):
                build_l(qr2, lp, j)
            for n in range(CA * NT):
                qk_tile(kpair(0), lp, slo0, 0, n)
            for n in range(CB * NT):
                qk_tile(kpair(0), lp, shi0, CA, n)
            for j in range(NJ):
                build_l(qr3, ln1, j)
            for n in range(CA * NT):
                qk_tile(kpair(1), ln1, slo1, 0, n)
            if not Q2EARLY:
                for n in range(NW):
                    qproj_tile(wqpair(2), qr0, n)
            softmax(slo0, shi0, pb0, ls0)

            wp = lambda a: 1 - a if WLAG == 1 else a

            def kinds(a):
                b = 1 - a
                return dict(
                    h=(CB * NT, lambda z: kpair(z + 1),
                       lambda w, n: qk_tile(w, ln[b], shi[b], CA, n)),
                    l=(CA * NT, lambda z: kpair(z + 2),
                       lambda w, n: qk_tile(w, ln[a], slo[a], 0, n)),
                    q=(NW, lambda z: wqpair(jnp.minimum(z + 3, NP - 1)),
                       lambda w, n: qproj_tile(w, qr[b], n)),
                    w=(NW, lambda z: wopair(jnp.maximum(z - WLAG, 0)),
                       lambda w, n: wo_tile(w, ol[wp(a)], yr[wp(a)], n)),
                    v=(2 * KD, lambda z: wopair(z - 1),
                       lambda w, n: wo_tile(w, ol[b], yr[b], KD + n)),
                    m=(CM * NT, lambda z: kpair(z + 2),
                       lambda w, n: qk_tile(w, ln[a], smid, CA, n, CM)),
                    g=((CB - CM) * NT, lambda z: kpair(z + 1),
                       lambda w, n: qk_tile(w, ln[b], shi[b], CA + CM, n, CB - CM)),
                    x=(4 * NCP, lambda z: vx.at[pl.ds((z - (NP - 1)) * 16, 16)], x_tile))

            def block(i, a, order=MORD, RATE=RATE, SETS=SETS, PACE=PACE):
                b = 1 - a
                steps = softmax_steps(slo[b], shi[b], pb[b], ls[b], None, tbl[i] - i if SSPILL == 2 else None)
                if STAGED:
                    pos = [GPOS] * XA + [MOFF + int(24 * (k_ + 1) * RATE) + GLAG for k_ in range(4 - XA)]
                    pos += [pos[-1] + 1, pos[-1] + ELAG]
                else:
                    pos = [max(SPOS, MOFF + int(CB * NT * RATE) + 1)] * len(steps)
                side = list(zip(pos, steps))
                side += [(IPOS, P(l_inv, ls[a], li[a])),
                         (YPOS, P(y_fold, yr[1 - wp(a)]))]
                for j in range(NJ):
                    side.append((LPOS + LSTEP * j, P(build_l, qr[a], ln[a], j)))
                    side.append((RPOS + RSTEP * j, P(reduce_o, ac[b], li[b], ol[b], j)))
                run_block(first, i, a, 0, SETS, kinds(a), order, RATE, PACE, side, MOFF)

            def block14(i):
                side = [(int(((CB - CM) * NT + NW) * RATE14) + 10, P(softmax, slo1, shi1, pb1, ls1, pk1, None, smid)),
                        (IPOS14, P(l_inv, ls0, li0)),
                        (KPOS, P(pack_p, pb0, pk0)),
                        (YP14, P(y_fold, yr[1 - wp(0)]))]
                for j in range(NJ):
                    side.append((RP14 + RS14 * j, P(reduce_o, ac1, li1, ol1, j)))
                run_block(first, i, 0, 16, SETS14, kinds(0), ORD14, RATE14, PACE14, side)

            cin = set()

            def col_sum(rg):
                cin.add(rg)
                ac0[rg - 16] = jnp.broadcast_to(jnp.sum(ac1[rg], axis=1, keepdims=True), (8, 128))

            def block15(i):
                side = [(IPOS15, P(l_inv, ls1, li1)),
                        (YP15, P(y_fold, yr[1 - wp(1)]))]
                for j in range(1, NJ):
                    side.append((RP15 + RS15 * j, P(reduce_o, ac0, li0, ol0, j)))
                if RIN15 >= 1:
                    side.append((16 * NCP + 1, P(reduce_o, ac1, li1, ol1, 1)))
                if RIN15 >= 2:
                    side.append((32 * NCP + 1, P(reduce_o, ac1, li1, ol1, 2)))
                run_block(first, i, 1, 16, SETS15, kinds(1), ORD15, RATE15, PACE15, side, 0, col_sum)

            def body(i, c):
                if first:
                    @pl.when((i & 1) == 0)
                    def _():
                        ch = lax.shift_right_logical(i, 1)
                        for c in chunk(ch) + vstage(ch):
                            c.wait()
                        for c in vstage(ch + 1):
                            c.start()

                        @pl.when(ch + 2 < NC - 1)
                        def _():
                            for c in chunk(ch + 2):
                                c.start()

                        @pl.when(ch + 2 == NC - 1)
                        def _():
                            for c in vlast:
                                c.start()

                        @pl.when(ch + 1 == NC - 1)
                        def _():
                            for c in c1 + c2all:
                                c.start()

                for a in range(2):
                    pl.when((i & 1) == a)(P(block, i, a))
                return c

            lax.fori_loop(0, NP - 3, body, 0)

            def tail(i, c):
                pl.when(i == NP - 3)(P(block, i, 1, MORD13, RATE13, SETS13, PACE13))
                if first:
                    @pl.when(i == NP - 2)
                    def _():
                        for c in vlast + vstage(NC - 1):
                            c.wait()

                pl.when(i == NP - 2)(P(block14, i))
                pl.when(i == NP - 1)(P(block15, i))
                return c

            lax.fori_loop(NP - 3, NP, tail, 0)

            ox = [x_finish(0), x_finish(1)]
            for n in list(range(KD, NW)) + list(range(KD)):
                wo_tile(wopair(NP - 2), ol0, yr0, n)
            for n in range(KD):
                wo_tile(wopair(NP - 1), ol1, qr0, n)
            wl = wopair(NP - 1)
            yv, mv = {}, {}
            for m in range(8, RH):
                c0, c1_ = [ac0[rg - 16] if rg in cin else jnp.sum(ac1[rg], axis=1, keepdims=True)
                           for rg in (2 * m, 2 * m + 1)]
                hh = 2 * m // RH
                for nt in range(KD):
                    w = pltpu.bitcast(wl[nt, pl.ds(8 * m, 8), :], bf16).astype(f32)
                    t = w[:8] * c0 + w[8:] * c1_
                    yv[hh, nt] = t if (hh, nt) not in yv else yv[hh, nt] + t
                t = wsc[2 * m - 16] * c0 + wsc[2 * m - 15] * c1_
                mv[hh] = t if hh not in mv else mv[hh] + t
            early = [_tree_sum([ysum[nt]] + [yr1[j * KD + nt] for j in range(NJ)]
                               + [yr0[j * KD + nt] for j in range(1, NJ)]) for nt in range(KD)]
            ys = [_tree_sum([early[nt], yr0[nt], qr0[nt],
                             yv[0, nt] * li1[0:1, :], yv[1, nt] * li1[1:2, :]]) for nt in range(KD)]
            y = jnp.sum(jnp.concatenate(ys, axis=1), axis=0, keepdims=True)
            lanes = _tree_sum(early + [x[:, nt * 128:(nt + 1) * 128] * 0.125 for nt in range(KD)]
                              + [ox[0] * wsl[0], ox[1] * wsl[1]])
            tot = (jnp.sum(lanes, axis=1, keepdims=True)
                   + mv[0] * li1[0:1, :] + mv[1] * li1[1:2, :])
            mean = jnp.concatenate([_sublane_sum(tot) * (1.0 / D)] * KD, axis=1)
            x = x + y

            xc, rs = _center(x, mean)
            xn = _pack_rows(xc)
            if first:
                for c in c1:
                    c.wait()
            nv = 0 if first else NV2
            gs = {}
            nv1 = 0 if first else NV1
            for n in range(KF - nv1):
                h = _tree_sum(_tile_dot(xn[:, kt * 128:(kt + 1) * 128], w1b[n, pl.ds(kt * 64, 64), :])
                              for kt in range(KD))
                gs[n] = _gelu(h * rs + b1v[n:n + 1, :].astype(f32))
            hacc = {}
            for kt in range(KD if nv1 else 0):
                col = _columns(xc[:, kt * 128:(kt + 1) * 128])
                for v in range(8):
                    for n in range(KF - nv1, KF):
                        w = pltpu.bitcast(w1b[n, pl.ds(kt * 64 + 8 * v, 8), :], bf16).astype(f32)
                        t = w[:8] * col[16 * v:16 * v + 8] + w[8:] * col[16 * v + 8:16 * v + 16]
                        hacc[n] = t if n not in hacc else hacc[n] + t
            for n in hacc:
                gs[n] = _gelu(_sublane_sum(hacc[n]) * rs + b1v[n:n + 1, :].astype(f32))
            vacc = [None] * KD
            for kt in range(nv):
                col = _columns(gs[kt])
                for v in range(8):
                    for nt in range(KD):
                        w = pltpu.bitcast(w2b[nt, pl.ds(kt * 64 + 8 * v, 8), :], bf16).astype(f32)
                        t = w[:8] * col[16 * v:16 * v + 8] + w[8:] * col[16 * v + 8:16 * v + 16]
                        vacc[nt] = t if vacc[nt] is None else vacc[nt] + t
            parts = []
            for kt in range(nv, KF):
                if first and kt in w2_split:
                    for c in c2[w2_split.index(kt)]:
                        c.wait()
                hk = _pack_rows(gs[kt])
                parts.append([_tile_dot(hk, w2b[nt, pl.ds(kt * 64, 64), :]) for nt in range(KD)])
            y2 = jnp.concatenate(
                [_tree_sum([p[nt] for p in parts] + [b2v[nt:nt + 1, :].astype(f32)]
                           + ([_sublane_sum(vacc[nt])] if nv else []))
                 for nt in range(KD)], axis=1)
            return x + y2

        for c in head:
            c.wait()

        def transpose_tile(n, c):
            s8 = pl.multiple_of((n // (2 * NCP)) * 8, 8)
            e = n % 2
            c8 = pl.multiple_of(((n // 2) % NCP) * 8, 8)
            w = vx[pl.ds(s8, 8), e, pl.ds(c8, 8), :].reshape(64, 128)
            wt = pltpu.bitcast(w, bf16).astype(f32).T.astype(bf16)
            vx[pl.ds(s8, 8), e, pl.ds(c8, 8), :] = pltpu.bitcast(wt, u32).reshape(8, 8, 128)
            return c

        lax.fori_loop(0, 4 * NCP, transpose_tile, 0)

        def wo_rowsums(r0):
            w = _tree_sum(pltpu.bitcast(wob[nt, pl.ds(r0, 8), :], bf16).astype(f32) for nt in range(KD))
            return jnp.broadcast_to(jnp.sum(w, axis=1, keepdims=True), (16, 128))

        for m in range(8, RH):
            wsc[pl.ds(2 * m - 16, 2)] = wo_rowsums((NP - 1) * (PD // 2) + 8 * m).reshape(2, 8, 128)
        for s_ in range(2):
            cols = jnp.concatenate([wo_rowsums((NP - 2 + s_) * (PD // 2) + 8 * m) for m in range(8)], axis=0)
            wsl[s_] = cols.T[0:8]

        if ONLY2:
            for c in chunk(0) + vstage(0) + chunk(1):
                c.wait()
        x = jnp.broadcast_to(xin[0].astype(f32), (8, D))
        for l_ in range(1 if ONLY2 else NL):
            x = layer(x, l_ == 0 and not ONLY2)
        o_ref[0] = x[0:1, :].astype(o_ref.dtype)

    return kernel


@jax.jit
def pallas_interleave_layers__sliding_block_cached__dense_activation_gelu__decode_kernel(
    A_x, A_k_cache, A_v_cache, A_wq, A_wo, B_x, B_w1, B_b1, B_w2, B_b2,
):
    SK = A_k_cache.shape[2]
    W = min(4096, max(256, SK // 4))
    NR = H * DH // 8

    def tiled(a):
        t = jnp.swapaxes(a, 2, 3).reshape(NR, 8, SK // 128, 128)
        return t.transpose(0, 2, 1, 3).reshape(NR // 2, 2, SK // 16, 128)

    b1 = B_b1.reshape(F // 128, 128)
    b2 = B_b2.reshape(D // 128, 128)
    anyspec = pl.BlockSpec(memory_space=pl.ANY)
    NCP = W // 256
    vreg = lambda n, dt: pltpu.VMEM(n + (8, 128), dt)
    return pl.pallas_call(
        _make_kernel(SK, W),
        out_shape=jax.ShapeDtypeStruct(A_x.shape, A_x.dtype),
        in_specs=[anyspec] * 9,
        out_specs=pl.BlockSpec(memory_space=pltpu.VMEM),
        scratch_shapes=[
            pltpu.VMEM((NR // 2, 2, W // 32, 128), u32),
            pltpu.VMEM((NR // 2 - 16 - NP * RF // 2, 2, W // 16, 128), bf16),
            pltpu.VMEM((2 * RF, 2, W // 16, 128), bf16),
            pltpu.VMEM((16, 2, W // 32, 128), u32),
            vreg((NP * max(RF, 1), 2 * NCP), f32),
            pltpu.VMEM((H * DH // 128, D // 2, 128), u32),
            pltpu.VMEM((KD, H * DH // 2, 128), u32),
            pltpu.VMEM((KF, D // 2, 128), u32),
            pltpu.VMEM((KD, F // 2, 128), u32),
            pltpu.VMEM((1, 1, D), bf16),
            pltpu.VMEM((KF, 128), bf16),
            pltpu.VMEM((KD, 128), bf16),
            pltpu.VMEM((8, D), u32),
            pltpu.VMEM((8, 128), f32),
            vreg((KD,), f32),
            vreg((NCP,), f32),
        ] + [vreg((NT,), u32)] * 3
          + [vreg((NW,), f32)] * 4
          + [vreg((4 * XA, NT), f32)] * 2
          + [vreg((4, NT), f32)]
          + [vreg((NCP - 4 * XA, NT), f32)] * 2
          + [pltpu.VMEM((8, NCP * 128), f32)] * 2
          + [pltpu.VMEM((8, 128), f32)] * 4
          + [vreg((RP,), f32)] * 2
          + [vreg((NJ,), u32)] * 2
          + [vreg((NW,), f32)] * 2
          + [vreg((NCP,), u32)] * 2
          + [vreg((2, 2, NCP), f32)]
          + [vreg((32,), f32), vreg((2,), f32)]
          + [pltpu.SMEM((NP,), jnp.int32)]
          + [pltpu.SemaphoreType.DMA((5,))],
        compiler_params=pltpu.CompilerParams(vmem_limit_bytes=128 * 1024 * 1024,
                                             disable_semaphore_checks=bool(NOSEM)),
    )(A_x, tiled(A_k_cache), tiled(A_v_cache), A_wq, A_wo, B_w1, b1, B_w2, b2)
```

```python
import functools
import jax
import jax.numpy as jnp
from jax import lax
import jax.experimental.pallas as pl
import jax.experimental.pallas.tpu as pltpu

D = 640
H = 32
DH = 192
F = 1536
NP = H // 2
PD = 2 * DH
RH = DH // 8
RP = 2 * RH
NJ = PD // 128
NT = 2 * NJ
KD = D // 128
KF = F // 128
NW = NJ * KD
EPS = 1e-5
LOG2E = 1.4426950408889634
bf16 = jnp.bfloat16
f32 = jnp.float32
u32 = jnp.uint32

RATE = 6.0
SPOS = 450
LPOS = 100
RPOS = 300
RSTEP = 80
YPOS = 5
IPOS = 150
IPOS14 = 10
IPOS15 = 10
SETS13 = "6,6,6,6,6,18"
CM = 2
RIN15 = 0
NV2 = 5
NV1 = 3
CIN = 0
ONEPASS = 0
NVQ = 6
VFIRST = 0
VGRP = 2
QRND = 1
CUMQ = 1
KPOS = 300
YP14 = 5
YP15 = 250
RS15 = 10
MORD13 = "hwlm"
RATE13 = 6.1
CPOS = 200
NL = 2
MORD = "hwql"
SSPILL = 0
PACE = 6
PACE13 = 3
D0 = 1
XA = 1
SETS = "10,10,10,18"
SETS14 = "4,4,4,4,16"
SETS15 = "8,8,10,6"
RATE14 = 6.7
RATE15 = 6.3
PACE14 = 3
PACE15 = 0
ONLY2 = 0
NOSEM = 0
STAGED = 0
GPOS = 30
GLAG = 60
ELAG = 80
MOFF = 0
LSTEP = 10
WOSTEP = 256
W2STEP = 192
W2SPLIT = "0,9,11,12"
RF = 8
F0 = 15
RP14 = 100
RP15 = 100
RS14 = 10
ORD14 = "gw"
WLAG = 2
ORD15 = "xw"
Q2EARLY = 1


def _center(x, mean=None):
    if mean is not None:
        xc = x - mean
        v = jnp.mean(xc * xc, axis=-1, keepdims=True)
        return xc, lax.rsqrt(v + EPS)
    if ONEPASS:
        m = jnp.mean(x, axis=-1, keepdims=True)
        v = jnp.maximum(jnp.mean(x * x, axis=-1, keepdims=True) - m * m, 0.0)
        return x - m, lax.rsqrt(v + EPS)
    xc = x - jnp.mean(x, axis=-1, keepdims=True)
    v = jnp.mean(xc * xc, axis=-1, keepdims=True)
    return xc, lax.rsqrt(v + EPS)


def _gelu(x):
    c = 0.7978845608028654
    return 0.5 * x * (1.0 + jnp.tanh(c * (x + 0.044715 * (x * x * x))))


def _pack_rows(x8):
    x16 = jnp.concatenate([x8, x8], axis=0).astype(bf16)
    return pltpu.bitcast(x16, u32)


def _tile_dot(lhs_u32, w_u32):
    return jnp.dot(pltpu.bitcast(lhs_u32, bf16), pltpu.bitcast(w_u32, bf16),
                   preferred_element_type=f32)[0:8]


def _columns(x8):
    return jnp.concatenate([x8] * 16, axis=0).T


def _sublane_sum(x8):
    for sh in (4, 2, 1):
        x8 = x8 + pltpu.roll(x8, sh, 0)
    return x8


def _tree(op, xs):
    xs = list(xs)
    while len(xs) > 1:
        xs = [op(xs[i], xs[i + 1]) if i + 1 < len(xs) else xs[i] for i in range(0, len(xs), 2)]
    return xs[0]


def _tree_sum(xs):
    return _tree(jnp.add, xs)


def _make_kernel(SK, W):
    NCP = W // 256
    CA = 4 * XA
    CB = NCP - CA
    c_exp = (DH ** -0.5) * LOG2E
    P = functools.partial

    def kernel(x_hbm, k_hbm, v_hbm, wq_hbm, wo_hbm, w1_hbm, b1_hbm, w2_hbm, b2_hbm,
               o_ref,
               kb, vb, vs, vx, vf, wqb, wob, w1b, w2b, xin, b1v, b2v, xl, rs_ref, ysum, ssum,
               ln0, ln1, lp, qr0, qr1, qr2, qr3, slo0, slo1, smid, shi0, shi1, pb0, pb1,
               ls0, ls1, li0, li1, ac0, ac1, ol0, ol1, yr0, yr1, pk0, pk1, wsc, wsl, svq, tbl, sems):
        ln, qr, slo, shi = (ln0, ln1), (qr0, qr1), (slo0, slo1), (shi0, shi1)
        pb, ls, li, ac, ol, yr = (pb0, pb1), (ls0, ls1), (li0, li1), (ac0, ac1), (ol0, ol1), (yr0, yr1)
        pk = (pk0, pk1)
        ku = k_hbm.bitcast(u32)
        vu = v_hbm.bitcast(u32)
        NC = NP // 2

        def kcopy(c, s):
            return pltpu.make_async_copy(
                ku.at[pl.ds(c * RP, RP), :, pl.ds((SK - W) // 32, W // 32), :],
                kb.at[pl.ds(c * RP, RP)], sems.at[s])

        RM = RH - RF // 2

        def vcopy(src0, n, dst, dst0, s):
            return pltpu.make_async_copy(
                v_hbm.at[pl.ds(src0, n), :, pl.ds((SK - W) // 16, W // 16), :],
                dst.at[pl.ds(dst0, n)], sems.at[s])

        def vstage(c):
            return [vcopy((2 * c + p) * RH + RM, RF // 2, vs, ((2 * c + p) & 3) * (RF // 2), 1 + (c & 1))
                    for p in range(2)]

        def wcopies(src, dst, s, r0=0, nrows=None, step=None):
            su = src.bitcast(u32)
            nrows = dst.shape[1] if nrows is None else nrows
            step = nrows if step is None else step
            return [pltpu.make_async_copy(su.at[pl.ds(r, step), pl.ds(n * 128, 128)],
                                          dst.at[n, pl.ds(r, step)], sems.at[s])
                    for r in range(r0, r0 + nrows, step) for n in range(dst.shape[0])]

        head = [pltpu.make_async_copy(x_hbm, xin, sems.at[0]),
                pltpu.make_async_copy(b1_hbm, b1v, sems.at[0]),
                pltpu.make_async_copy(b2_hbm, b2v, sems.at[0])]
        head += [pltpu.make_async_copy(
            vu.at[pl.ds((NP - 2 + s) * RH, 8), :, pl.ds((SK - W) // 32, W // 32), :],
            vx.at[pl.ds(8 * s, 8)], sems.at[0]) for s in range(2)]
        head += wcopies(wq_hbm, wqb, 0) + wcopies(wo_hbm, wob, 0, step=WOSTEP) + [kcopy(0, 0)]
        vlast = [vcopy((NP - 2 + s) * RH + 8, RM - 8, vb, (NP - 2) * RM + s * (RM - 8), 2) for s in range(2)]
        c1 = wcopies(w1_hbm, w1b, 1)
        w2_split = tuple(int(z) for z in W2SPLIT.split(','))
        c2 = [wcopies(w2_hbm, w2b, (0, 3, 4)[g], 64 * w2_split[g],
                      64 * (w2_split[g + 1] - w2_split[g]),
                      min(W2STEP, 64 * (w2_split[g + 1] - w2_split[g]))) for g in range(len(w2_split) - 1)]
        c2all = [c for g in c2 for c in g]
        for c in head:
            c.start()

        def chunk(c):
            s = 1 + (c & 1)
            return [kcopy(c + 1, s)] + [vcopy((2 * c + p) * RH, RM, vb, (2 * c + p) * RM, s) for p in range(2)]

        for c in chunk(0) + vstage(0) + chunk(1):
            c.start()

        for i_ in range(NP):
            tbl[i_] = i_

        def qproj_tile(wg, dst, n):
            j, kt = divmod(n, KD)
            dst[n] = _tile_dot(xl[:, pl.ds(kt * 128, 128)], wg[j, pl.ds(kt * 64, 64), :])

        def build_l(src, dst, j):
            row = lax.broadcasted_iota(jnp.int32, (8, 128), 0)
            lane = lax.broadcasted_iota(jnp.int32, (8, 128), 1)
            q = _tree_sum(src[j * KD + kt] for kt in range(KD)) * rs_ref[...]
            qp = pltpu.roll(q, 8, 1)
            qm = pltpu.roll(q, 120, 1)
            tgt = (lane >> 1) & 4
            if j == 1:
                tgt = tgt + (lane >> 6)
            elif j == 2:
                tgt = tgt + 1
            hit = row == tgt
            low = row < 4
            dst[2 * j] = _pack_rows(jnp.where(hit, jnp.where(low, q, qp), 0.0))
            dst[2 * j + 1] = _pack_rows(jnp.where(hit, jnp.where(low, qm, q), 0.0))

        def qk_tile(kg, lsrc, sdst, c0, n, ncp=NCP):
            c4, rem = divmod(n, 4 * NT)
            t, i = divmod(rem, min(4, ncp - c4 * 4))
            c = c4 * 4 + i
            w = kg[pl.ds((t // 2) * 8, 8), t % 2, pl.ds((c0 + c) * 8, 8), :].reshape(64, 128)
            sdst[c, t] = _tile_dot(lsrc[t], w)

        def s_group(st, src, c0, c1):
            s = [_tree_sum(src[c, t] for t in range(src.shape[1])) for c in range(c0, c1)]
            base = len(st.setdefault("s", []))
            if SSPILL:
                for k_, a_ in enumerate(s):
                    ssum[st.get("zero", 0) + base + k_] = a_
            st["s"] += s
            st["m"] = _tree(jnp.maximum, s + ([st["m"]] if "m" in st else []))

        def s_max(st):
            m = jnp.maximum(st["m"], pltpu.roll(st["m"], 4, 0))
            st["m"] = jnp.max(m, axis=1, keepdims=True)

        def s_exp(st, pdst, ldst, kdst=None):
            s = [ssum[cp] for cp in range(NCP)] if SSPILL else st["s"]
            e = [jnp.exp2(a - st["m"]) for a in s]
            for cp in range(NCP):
                pdst[:, pl.ds(cp * 128, 128)] = e[cp]
                if kdst is not None:
                    kdst[cp] = _pack_rows(e[cp])
            ldst[...] = _tree_sum(e)

        def softmax_steps(lo, hi, pdst, ldst, kdst=None, zero=None, mid=None, tail=None):
            st = {} if zero is None else {"zero": zero}
            srcs = [(lo, CA), (hi, CB)] if mid is None else [(lo, CA), (mid, CM), (hi, CB - CM)]
            if tail is not None:
                srcs = [(lo, CA), (hi, CB - NVQ), (tail, NVQ)]
            steps = [P(s_group, st, src, c0, min(c0 + 4, n)) for src, n in srcs for c0 in range(0, n, 4)]
            return steps + [P(s_max, st), P(s_exp, st, pdst, ldst, kdst)]

        def softmax(*args):
            for f in softmax_steps(*args):
                f()

        def l_inv(lsrc, ldst):
            l = lsrc[...]
            l = l + pltpu.roll(l, 4, 0)
            l = jnp.sum(l, axis=1, keepdims=True)
            ldst[...] = jnp.broadcast_to(1.0 / l, (8, 128))

        def pack_p(psrc, kdst):
            for cp in range(NCP):
                kdst[cp] = _pack_rows(psrc[:, pl.ds(cp * 128, 128)])

        def reduce_o(asrc, lsrc, odst, j):
            blk = asrc[pl.ds(j * 16, 16)].reshape(128, 128)
            t = blk.T.reshape(16, 8, 128)
            if j == 1:
                lane = lax.broadcasted_iota(jnp.int32, (1, 128), 1)
                r = jnp.where(lane < 64, lsrc[0:1, :], lsrc[1:2, :])
            else:
                r = lsrc[j // 2:j // 2 + 1, :]
            odst[j] = _pack_rows(_tree_sum(t[i] for i in range(16)) * r)

        def x_tile(vg, n):
            s, rem = divmod(n, 2 * NCP)
            cp, e = divmod(rem, 2)
            w = vg[pl.ds(8 * s, 8), e, pl.ds(cp * 8, 8), :].reshape(64, 128)
            shi0[divmod(n, NT)] = _tile_dot(pk[s][cp], w)

        def x_finish(s):
            row = lax.broadcasted_iota(jnp.int32, (8, 128), 0)
            lane = lax.broadcasted_iota(jnp.int32, (8, 128), 1)
            o0 = _tree_sum(shi0[divmod((s * NCP + cp) * 2, NT)] for cp in range(NCP))
            o1 = _tree_sum(shi0[divmod((s * NCP + cp) * 2 + 1, NT)] for cp in range(NCP))
            low = row < 4
            direct = jnp.where(low, o0, o1)
            moved = jnp.where(low, pltpu.roll(o1, 8, 1), pltpu.roll(o0, 120, 1))
            o = jnp.where(((lane >> 1) & 4) == (row & 4), direct, moved)
            o = jnp.where((row & 3) == 0, o, 0.0) * li[s][0:1, :]
            ol[s][0] = _pack_rows(o)
            return o

        def wo_tile(wg, osrc, ydst, n):
            j, nt = divmod(n, KD)
            ydst[n] = _tile_dot(osrc[j], wg[nt, pl.ds(j * 64, 64), :])

        def y_fold(ysrc):
            for nt in range(KD):
                ysum[nt] = _tree_sum([ysum[nt]] + [ysrc[j * KD + nt] for j in range(NJ)])

        def copy(src, dst):
            for i in range(src.shape[0]):
                dst[i] = src[i]

        def kpair(i):
            return kb.at[pl.ds(i * RH, RH)]

        def wqpair(i):
            return wqb.at[pl.ds(i * NJ, NJ)]

        def wopair(i):
            r0 = i * (PD // 2)
            if not isinstance(i, int):
                r0 = pl.multiple_of(r0, PD // 2)
            return wob.at[:, pl.ds(r0, PD // 2), :]

        def run_block(first, i, a, rg0, sets, kinds, order, rate, pace_n, side, moff=0, done=None):
            if rg0:
                vg = vb.at[pl.ds((NP - 2) * RM + a * (RM - 8), RM - 8)]
            else:
                vg = vb.at[pl.ds(i * RM, RM)]
            voff = rg0 // 2
            sg = vs.at[pl.ds((i & 3) * (RF // 2), RF // 2)]
            fg = vf.at[pl.ds(i * RF, RF)]
            plain, order_rg = list(range(rg0, RP - RF)), []
            n_all = RP - rg0
            f0 = min(F0, n_all - RF) * n_all // RP
            slots = {f0 + (k_ + 1) * (n_all - f0) // RF - 1 for k_ in range(RF)}
            nf = 0
            for pos_ in range(n_all):
                if pos_ in slots:
                    order_rg.append(RP - RF + nf)
                    nf += 1
                else:
                    order_rg.append(plain.pop(0))
            pace = dict(z=i, cnt=0, views={})

            def mxu_tile(key, n):
                if pace_n and pace["cnt"] % pace_n == 0:
                    z = pace["z"]
                    link = pace["cnt"] // pace_n
                    for _ in range(pace_n * 4 // 3 if link else D0):
                        z = tbl[z]
                    pace["z"] = z
                    pace["views"] = {}
                pace["cnt"] += 1
                if key not in pace["views"]:
                    pace["views"][key] = kinds[key][1](pace["z"])
                kinds[key][2](pace["views"][key], n)

            mxu = [P(mxu_tile, key, n) for key in order for n in range(kinds[key][0])]
            side = sorted(side + [(moff + int(n * rate), f) for n, f in enumerate(mxu)], key=lambda z: z[0])
            cnt = 0
            si = 0
            acc = {}
            sizes, ovl = sets.split(":") if ":" in sets else (sets, "0")
            groups = []
            for size in (int(z) for z in sizes.split(",")):
                groups.append(order_rg[:size])
                order_rg = order_rg[size:]
            step = NCP - int(ovl)
            seq = [(rgs, t - gi * step) for t in range((len(groups) - 1) * step + NCP)
                   for gi, rgs in enumerate(groups) if 0 <= t - gi * step < NCP]
            for rgs, cp in seq:
                mult = {hh: (pb[a][pl.ds(hh, 1), pl.ds(cp * 128, 128)],
                             pb[a][pl.ds(4 + hh, 1), pl.ds(cp * 128, 128)])
                        for hh in sorted({rg // RH for rg in rgs})}
                for rg in rgs:
                    while si < len(side) and side[si][0] <= cnt:
                        side[si][1]()
                        si += 1
                    cnt += 1
                    m0, m1 = mult[rg // RH]
                    r = rg - (RP - RF)
                    if r >= 0 and not first:
                        v0, v1 = fg[r, 2 * cp], fg[r, 2 * cp + 1]
                    else:
                        src = sg.at[r // 2, r % 2] if r >= 0 else vg.at[rg // 2 - voff, rg % 2]
                        v = src[pl.ds(cp * 16, 16), :].astype(f32)
                        v0, v1 = v[:8], v[8:]
                        if r >= 0:
                            fg[r, 2 * cp] = v0
                            fg[r, 2 * cp + 1] = v1
                    if rg not in acc:
                        acc[rg] = v0 * m0 + v1 * m1
                    else:
                        acc[rg] = acc[rg] + v0 * m0 + v1 * m1
                    if cp == NCP - 1:
                        ac[a][rg] = acc[rg]
                        if done is not None and cnt <= CIN * NCP:
                            done(rg)
            assert not order_rg
            for _, f in side[si:]:
                f()

        def layer(x, first):
            nvq = 0 if first else NVQ
            xc, rs = _center(x)
            xl[...] = _pack_rows(xc)
            rs_ref[...] = jnp.broadcast_to(rs * c_exp, (8, 128))
            ac1[...] = jnp.zeros(ac1.shape, f32)
            li1[...] = jnp.zeros(li1.shape, f32)
            if WLAG == 1:
                yr0[...] = jnp.zeros(yr0.shape, f32)
            else:
                ol0[...] = jnp.zeros(ol0.shape, u32)
                yr1[...] = jnp.zeros(yr1.shape, f32)
            ysum[...] = jnp.zeros(ysum.shape, f32)

            for i, dst in enumerate((qr2, qr3)):
                for n in range(NW):
                    qproj_tile(wqpair(i), dst, n)
            if Q2EARLY:
                for n in range(NW):
                    qproj_tile(wqpair(2), qr0, n)
            def vpu_qk():
                if not nvq:
                    return
                row = lax.broadcasted_iota(jnp.int32, (8, 128), 0)
                cols = jnp.concatenate(
                    [_columns((_tree_sum(qr2[j * KD + kt] for kt in range(KD)) * rs_ref[...])
                              .astype(bf16 if QRND else f32).astype(f32)) for j in range(NJ)], axis=0)
                sacc = {}
                for rg, cp in [(rg, cp) for c0_ in range(NCP - NVQ, NCP, VGRP) for rg in range(RP)
                               for cp in range(c0_, min(c0_ + VGRP, NCP))]:
                    if True:
                        kv = pltpu.bitcast(kb[rg // 2, rg % 2, pl.ds(cp * 8, 8), :], bf16).astype(f32)
                        for p_ in range(2):
                            t = kv[8 * p_:8 * p_ + 8] * cols[8 * rg:8 * rg + 8]
                            key = (cp, 4 * p_ + rg // RH)
                            prev = (cp - VGRP, key[1])
                            if key in sacc:
                                sacc[key] = sacc[key] + t
                            elif CUMQ and prev in sacc:
                                sacc[key] = sacc[prev] + t
                            else:
                                sacc[key] = t
                for cp in range(NCP - NVQ, NCP):
                    a_ = jnp.zeros((8, 128), f32)
                    for r_ in (0, 1, 4, 5):
                        z_ = sacc[cp, r_]
                        if CUMQ and (cp - VGRP, r_) in sacc:
                            z_ = z_ - sacc[cp - VGRP, r_]
                        a_ = jnp.where(row == r_, _sublane_sum(z_), a_)
                    svq[cp - (NCP - NVQ), 0] = a_

            for j in range(NJ):
                build_l(qr2, lp, j)
            if VFIRST:
                vpu_qk()
            for n in range(CA * NT):
                qk_tile(kpair(0), lp, slo0, 0, n)
            for n in range((CB - nvq) * NT):
                qk_tile(kpair(0), lp, shi0, CA, n, CB - nvq)
            if not VFIRST:
                vpu_qk()
            for j in range(NJ):
                build_l(qr3, ln1, j)
            for n in range(CA * NT):
                qk_tile(kpair(1), ln1, slo1, 0, n)
            if not Q2EARLY:
                for n in range(NW):
                    qproj_tile(wqpair(2), qr0, n)
            softmax(slo0, shi0, pb0, ls0, None, None, None, svq if nvq else None)

            wp = lambda a: 1 - a if WLAG == 1 else a

            def kinds(a):
                b = 1 - a
                return dict(
                    h=(CB * NT, lambda z: kpair(z + 1),
                       lambda w, n: qk_tile(w, ln[b], shi[b], CA, n)),
                    l=(CA * NT, lambda z: kpair(z + 2),
                       lambda w, n: qk_tile(w, ln[a], slo[a], 0, n)),
                    q=(NW, lambda z: wqpair(jnp.minimum(z + 3, NP - 1)),
                       lambda w, n: qproj_tile(w, qr[b], n)),
                    w=(NW, lambda z: wopair(jnp.maximum(z - WLAG, 0)),
                       lambda w, n: wo_tile(w, ol[wp(a)], yr[wp(a)], n)),
                    v=(2 * KD, lambda z: wopair(z - 1),
                       lambda w, n: wo_tile(w, ol[b], yr[b], KD + n)),
                    m=(CM * NT, lambda z: kpair(z + 2),
                       lambda w, n: qk_tile(w, ln[a], smid, CA, n, CM)),
                    g=((CB - CM) * NT, lambda z: kpair(z + 1),
                       lambda w, n: qk_tile(w, ln[b], shi[b], CA + CM, n, CB - CM)),
                    x=(4 * NCP, lambda z: vx.at[pl.ds((z - (NP - 1)) * 16, 16)], x_tile))

            def block(i, a, order=MORD, RATE=RATE, SETS=SETS, PACE=PACE):
                b = 1 - a
                steps = softmax_steps(slo[b], shi[b], pb[b], ls[b], None, tbl[i] - i if SSPILL == 2 else None)
                if STAGED:
                    pos = [GPOS] * XA + [MOFF + int(24 * (k_ + 1) * RATE) + GLAG for k_ in range(4 - XA)]
                    pos += [pos[-1] + 1, pos[-1] + ELAG]
                else:
                    pos = [max(SPOS, MOFF + int(CB * NT * RATE) + 1)] * len(steps)
                side = list(zip(pos, steps))
                side += [(IPOS, P(l_inv, ls[a], li[a])),
                         (YPOS, P(y_fold, yr[1 - wp(a)]))]
                for j in range(NJ):
                    side.append((LPOS + LSTEP * j, P(build_l, qr[a], ln[a], j)))
                    side.append((RPOS + RSTEP * j, P(reduce_o, ac[b], li[b], ol[b], j)))
                run_block(first, i, a, 0, SETS, kinds(a), order, RATE, PACE, side, MOFF)

            def block14(i):
                side = [(int(((CB - CM) * NT + NW) * RATE14) + 10, P(softmax, slo1, shi1, pb1, ls1, pk1, None, smid)),
                        (IPOS14, P(l_inv, ls0, li0)),
                        (KPOS, P(pack_p, pb0, pk0)),
                        (YP14, P(y_fold, yr[1 - wp(0)]))]
                for j in range(NJ):
                    side.append((RP14 + RS14 * j, P(reduce_o, ac1, li1, ol1, j)))
                run_block(first, i, 0, 16, SETS14, kinds(0), ORD14, RATE14, PACE14, side)

            cin = set()

            def col_sum(rg):
                cin.add(rg)
                ac0[rg - 16] = jnp.broadcast_to(jnp.sum(ac1[rg], axis=1, keepdims=True), (8, 128))

            def block15(i):
                side = [(IPOS15, P(l_inv, ls1, li1)),
                        (YP15, P(y_fold, yr[1 - wp(1)]))]
                for j in range(1, NJ):
                    side.append((RP15 + RS15 * j, P(reduce_o, ac0, li0, ol0, j)))
                if RIN15 >= 1:
                    side.append((16 * NCP + 1, P(reduce_o, ac1, li1, ol1, 1)))
                if RIN15 >= 2:
                    side.append((32 * NCP + 1, P(reduce_o, ac1, li1, ol1, 2)))
                run_block(first, i, 1, 16, SETS15, kinds(1), ORD15, RATE15, PACE15, side, 0, col_sum)

            def body(i, c):
                if first:
                    @pl.when((i & 1) == 0)
                    def _():
                        ch = lax.shift_right_logical(i, 1)
                        for c in chunk(ch) + vstage(ch):
                            c.wait()
                        for c in vstage(ch + 1):
                            c.start()

                        @pl.when(ch + 2 < NC - 1)
                        def _():
                            for c in chunk(ch + 2):
                                c.start()

                        @pl.when(ch + 2 == NC - 1)
                        def _():
                            for c in vlast:
                                c.start()

                        @pl.when(ch + 1 == NC - 1)
                        def _():
                            for c in c1 + c2all:
                                c.start()

                for a in range(2):
                    pl.when((i & 1) == a)(P(block, i, a))
                return c

            lax.fori_loop(0, NP - 3, body, 0)

            def tail(i, c):
                pl.when(i == NP - 3)(P(block, i, 1, MORD13, RATE13, SETS13, PACE13))
                if first:
                    @pl.when(i == NP - 2)
                    def _():
                        for c in vlast + vstage(NC - 1):
                            c.wait()

                pl.when(i == NP - 2)(P(block14, i))
                pl.when(i == NP - 1)(P(block15, i))
                return c

            lax.fori_loop(NP - 3, NP, tail, 0)

            ox = [x_finish(0), x_finish(1)]
            for n in list(range(KD, NW)) + list(range(KD)):
                wo_tile(wopair(NP - 2), ol0, yr0, n)
            for n in range(KD):
                wo_tile(wopair(NP - 1), ol1, qr0, n)
            wl = wopair(NP - 1)
            yv, mv = {}, {}
            for m in range(8, RH):
                c0, c1_ = [ac0[rg - 16] if rg in cin else jnp.sum(ac1[rg], axis=1, keepdims=True)
                           for rg in (2 * m, 2 * m + 1)]
                hh = 2 * m // RH
                for nt in range(KD):
                    w = pltpu.bitcast(wl[nt, pl.ds(8 * m, 8), :], bf16).astype(f32)
                    t = w[:8] * c0 + w[8:] * c1_
                    yv[hh, nt] = t if (hh, nt) not in yv else yv[hh, nt] + t
                t = wsc[2 * m - 16] * c0 + wsc[2 * m - 15] * c1_
                mv[hh] = t if hh not in mv else mv[hh] + t
            early = [_tree_sum([ysum[nt]] + [yr1[j * KD + nt] for j in range(NJ)]
                               + [yr0[j * KD + nt] for j in range(1, NJ)]) for nt in range(KD)]
            ys = [_tree_sum([early[nt], yr0[nt], qr0[nt],
                             yv[0, nt] * li1[0:1, :], yv[1, nt] * li1[1:2, :]]) for nt in range(KD)]
            y = jnp.sum(jnp.concatenate(ys, axis=1), axis=0, keepdims=True)
            lanes = _tree_sum(early + [x[:, nt * 128:(nt + 1) * 128] * 0.125 for nt in range(KD)]
                              + [ox[0] * wsl[0], ox[1] * wsl[1]])
            tot = (jnp.sum(lanes, axis=1, keepdims=True)
                   + mv[0] * li1[0:1, :] + mv[1] * li1[1:2, :])
            mean = jnp.concatenate([_sublane_sum(tot) * (1.0 / D)] * KD, axis=1)
            x = x + y

            xc, rs = _center(x, mean)
            xn = _pack_rows(xc)
            if first:
                for c in c1:
                    c.wait()
            nv = 0 if first else NV2
            gs = {}
            nv1 = 0 if first else NV1
            for n in range(KF - nv1):
                h = _tree_sum(_tile_dot(xn[:, kt * 128:(kt + 1) * 128], w1b[n, pl.ds(kt * 64, 64), :])
                              for kt in range(KD))
                gs[n] = _gelu(h * rs + b1v[n:n + 1, :].astype(f32))
            hacc = {}
            for kt in range(KD if nv1 else 0):
                col = _columns(xc[:, kt * 128:(kt + 1) * 128])
                for v in range(8):
                    for n in range(KF - nv1, KF):
                        w = pltpu.bitcast(w1b[n, pl.ds(kt * 64 + 8 * v, 8), :], bf16).astype(f32)
                        t = w[:8] * col[16 * v:16 * v + 8] + w[8:] * col[16 * v + 8:16 * v + 16]
                        hacc[n] = t if n not in hacc else hacc[n] + t
            for n in hacc:
                gs[n] = _gelu(_sublane_sum(hacc[n]) * rs + b1v[n:n + 1, :].astype(f32))
            vacc = [None] * KD
            for kt in range(nv):
                col = _columns(gs[kt])
                for v in range(8):
                    for nt in range(KD):
                        w = pltpu.bitcast(w2b[nt, pl.ds(kt * 64 + 8 * v, 8), :], bf16).astype(f32)
                        t = w[:8] * col[16 * v:16 * v + 8] + w[8:] * col[16 * v + 8:16 * v + 16]
                        vacc[nt] = t if vacc[nt] is None else vacc[nt] + t
            parts = []
            for kt in range(nv, KF):
                if first and kt in w2_split:
                    for c in c2[w2_split.index(kt)]:
                        c.wait()
                hk = _pack_rows(gs[kt])
                parts.append([_tile_dot(hk, w2b[nt, pl.ds(kt * 64, 64), :]) for nt in range(KD)])
            y2 = jnp.concatenate(
                [_tree_sum([p[nt] for p in parts] + [b2v[nt:nt + 1, :].astype(f32)]
                           + ([_sublane_sum(vacc[nt])] if nv else []))
                 for nt in range(KD)], axis=1)
            return x + y2

        for c in head:
            c.wait()

        def wo_rowsums(r0):
            w = _tree_sum(pltpu.bitcast(wob[nt, pl.ds(r0, 8), :], bf16).astype(f32) for nt in range(KD))
            return jnp.broadcast_to(jnp.sum(w, axis=1, keepdims=True), (16, 128))

        for m in range(8, RH):
            wsc[pl.ds(2 * m - 16, 2)] = wo_rowsums((NP - 1) * (PD // 2) + 8 * m).reshape(2, 8, 128)
        for s_ in range(2):
            cols = jnp.concatenate([wo_rowsums((NP - 2 + s_) * (PD // 2) + 8 * m) for m in range(8)], axis=0)
            wsl[s_] = cols.T[0:8]

        def transpose_tile(n, c):
            s8 = pl.multiple_of((n // (2 * NCP)) * 8, 8)
            e = n % 2
            c8 = pl.multiple_of(((n // 2) % NCP) * 8, 8)
            w = vx[pl.ds(s8, 8), e, pl.ds(c8, 8), :].reshape(64, 128)
            wt = pltpu.bitcast(w, bf16).astype(f32).T.astype(bf16)
            vx[pl.ds(s8, 8), e, pl.ds(c8, 8), :] = pltpu.bitcast(wt, u32).reshape(8, 8, 128)
            return c

        lax.fori_loop(0, 4 * NCP, transpose_tile, 0)

        if ONLY2:
            for c in chunk(0) + vstage(0) + chunk(1):
                c.wait()
        x = jnp.broadcast_to(xin[0].astype(f32), (8, D))
        for l_ in range(1 if ONLY2 else NL):
            x = layer(x, l_ == 0 and not ONLY2)
        o_ref[0] = x[0:1, :].astype(o_ref.dtype)

    return kernel


@jax.jit
def pallas_interleave_layers__sliding_block_cached__dense_activation_gelu__decode_kernel(
    A_x, A_k_cache, A_v_cache, A_wq, A_wo, B_x, B_w1, B_b1, B_w2, B_b2,
):
    SK = A_k_cache.shape[2]
    W = min(4096, max(256, SK // 4))
    NR = H * DH // 8

    def tiled(a):
        t = jnp.swapaxes(a, 2, 3).reshape(NR, 8, SK // 128, 128)
        return t.transpose(0, 2, 1, 3).reshape(NR // 2, 2, SK // 16, 128)

    b1 = B_b1.reshape(F // 128, 128)
    b2 = B_b2.reshape(D // 128, 128)
    anyspec = pl.BlockSpec(memory_space=pl.ANY)
    NCP = W // 256
    vreg = lambda n, dt: pltpu.VMEM(n + (8, 128), dt)
    return pl.pallas_call(
        _make_kernel(SK, W),
        out_shape=jax.ShapeDtypeStruct(A_x.shape, A_x.dtype),
        in_specs=[anyspec] * 9,
        out_specs=pl.BlockSpec(memory_space=pltpu.VMEM),
        scratch_shapes=[
            pltpu.VMEM((NR // 2, 2, W // 32, 128), u32),
            pltpu.VMEM((NR // 2 - 16 - NP * RF // 2, 2, W // 16, 128), bf16),
            pltpu.VMEM((2 * RF, 2, W // 16, 128), bf16),
            pltpu.VMEM((16, 2, W // 32, 128), u32),
            vreg((NP * max(RF, 1), 2 * NCP), f32),
            pltpu.VMEM((H * DH // 128, D // 2, 128), u32),
            pltpu.VMEM((KD, H * DH // 2, 128), u32),
            pltpu.VMEM((KF, D // 2, 128), u32),
            pltpu.VMEM((KD, F // 2, 128), u32),
            pltpu.VMEM((1, 1, D), bf16),
            pltpu.VMEM((KF, 128), bf16),
            pltpu.VMEM((KD, 128), bf16),
            pltpu.VMEM((8, D), u32),
            pltpu.VMEM((8, 128), f32),
            vreg((KD,), f32),
            vreg((NCP if SSPILL else 1,), f32),
        ] + [vreg((NT,), u32)] * 3
          + [vreg((NW,), f32)] * 4
          + [vreg((4 * XA, NT), f32)] * 2
          + [vreg((CM, NT), f32)]
          + [vreg((NCP - 4 * XA, NT), f32)] * 2
          + [pltpu.VMEM((8, NCP * 128), f32)] * 2
          + [pltpu.VMEM((8, 128), f32)] * 4
          + [vreg((RP,), f32)] * 2
          + [vreg((NJ,), u32)] * 2
          + [vreg((NW,), f32)] * 2
          + [vreg((NCP,), u32)] * 2
          + [vreg((32,), f32), vreg((2,), f32)]
          + [vreg((max(NVQ, 1), 1), f32)]
          + [pltpu.SMEM((NP,), jnp.int32)]
          + [pltpu.SemaphoreType.DMA((5,))],
        compiler_params=pltpu.CompilerParams(vmem_limit_bytes=128 * 1024 * 1024,
                                             disable_semaphore_checks=bool(NOSEM)),
    )(A_x, tiled(A_k_cache), tiled(A_v_cache), A_wq, A_wo, B_w1, b1, B_w2, b2)
```

```python
import functools
import jax
import jax.numpy as jnp
from jax import lax
import jax.experimental.pallas as pl
import jax.experimental.pallas.tpu as pltpu

D = 640
H = 32
DH = 192
F = 1536
NP = H // 2
PD = 2 * DH
RH = DH // 8
RP = 2 * RH
NJ = PD // 128
NT = 2 * NJ
KD = D // 128
KF = F // 128
NW = NJ * KD
EPS = 1e-5
LOG2E = 1.4426950408889634
bf16 = jnp.bfloat16
f32 = jnp.float32
u32 = jnp.uint32

RATE = 6.0
SPOS = 450
LPOS = 100
RPOS = 300
RSTEP = 80
YPOS = 5
IPOS = 150
IPOS14 = 10
IPOS15 = 10
SETS13 = "6,6,6,6,6,18"
CM = 2
RIN15 = 0
NV2 = 5
NV1 = 3
CIN = 0
ONEPASS = 0
NVQ = 6
VFIRST = 0
VGRP = 2
QRND = 1
CUMQ = 1
SL14 = 10
KPOS = 100
YP14 = 5
YP15 = 5
RS15 = 10
MORD13 = "hwlm"
RATE13 = 6.1
CPOS = 200
NL = 2
MORD = "hwql"
SSPILL = 0
PACE = 6
PACE13 = 3
D0 = 1
XA = 1
SETS = "10,10,10,18"
SETS14 = "8,8,8,8"
SETS15 = "8,8,10,6"
RATE14 = 5.6
RATE15 = 6.2
PACE14 = 3
PACE15 = 3
ONLY2 = 0
NOSEM = 0
STAGED = 0
GPOS = 30
GLAG = 60
ELAG = 80
MOFF = 0
LSTEP = 10
WOSTEP = 256
W2STEP = 192
W2SPLIT = "0,9,11,12"
RF = 8
F0 = 15
RP14 = 100
RP15 = 100
RS14 = 10
ORD14 = "gwu"
WLAG = 2
ORD15 = "xv"
Q2EARLY = 1


def _center(x, mean=None):
    if mean is not None:
        xc = x - mean
        v = jnp.mean(xc * xc, axis=-1, keepdims=True)
        return xc, lax.rsqrt(v + EPS)
    if ONEPASS:
        m = jnp.mean(x, axis=-1, keepdims=True)
        v = jnp.maximum(jnp.mean(x * x, axis=-1, keepdims=True) - m * m, 0.0)
        return x - m, lax.rsqrt(v + EPS)
    xc = x - jnp.mean(x, axis=-1, keepdims=True)
    v = jnp.mean(xc * xc, axis=-1, keepdims=True)
    return xc, lax.rsqrt(v + EPS)


def _gelu(x):
    c = 0.7978845608028654
    return 0.5 * x * (1.0 + jnp.tanh(c * (x + 0.044715 * (x * x * x))))


def _pack_rows(x8):
    x16 = jnp.concatenate([x8, x8], axis=0).astype(bf16)
    return pltpu.bitcast(x16, u32)


def _tile_dot(lhs_u32, w_u32):
    return jnp.dot(pltpu.bitcast(lhs_u32, bf16), pltpu.bitcast(w_u32, bf16),
                   preferred_element_type=f32)[0:8]


def _columns(x8):
    return jnp.concatenate([x8] * 16, axis=0).T


def _sublane_sum(x8):
    for sh in (4, 2, 1):
        x8 = x8 + pltpu.roll(x8, sh, 0)
    return x8


def _tree(op, xs):
    xs = list(xs)
    while len(xs) > 1:
        xs = [op(xs[i], xs[i + 1]) if i + 1 < len(xs) else xs[i] for i in range(0, len(xs), 2)]
    return xs[0]


def _tree_sum(xs):
    return _tree(jnp.add, xs)


def _make_kernel(SK, W):
    NCP = W // 256
    CA = 4 * XA
    CB = NCP - CA
    c_exp = (DH ** -0.5) * LOG2E
    P = functools.partial

    def kernel(x_hbm, k_hbm, v_hbm, wq_hbm, wo_hbm, w1_hbm, b1_hbm, w2_hbm, b2_hbm,
               o_ref,
               kb, vb, vs, vx, vf, wqb, wob, w1b, w2b, xin, b1v, b2v, xl, rs_ref, ysum, ssum,
               ln0, ln1, lp, qr0, qr1, qr2, qr3, slo0, slo1, smid, shi0, shi1, pb0, pb1,
               ls0, ls1, li0, li1, ac0, ac1, ol0, ol1, yr0, yr1, pk0, pk1, wsc, wsl, svq, tbl, sems):
        ln, qr, slo, shi = (ln0, ln1), (qr0, qr1), (slo0, slo1), (shi0, shi1)
        pb, ls, li, ac, ol, yr = (pb0, pb1), (ls0, ls1), (li0, li1), (ac0, ac1), (ol0, ol1), (yr0, yr1)
        pk = (pk0, pk1)
        ku = k_hbm.bitcast(u32)
        vu = v_hbm.bitcast(u32)
        NC = NP // 2

        def kcopy(c, s):
            return pltpu.make_async_copy(
                ku.at[pl.ds(c * RP, RP), :, pl.ds((SK - W) // 32, W // 32), :],
                kb.at[pl.ds(c * RP, RP)], sems.at[s])

        RM = RH - RF // 2

        def vcopy(src0, n, dst, dst0, s):
            return pltpu.make_async_copy(
                v_hbm.at[pl.ds(src0, n), :, pl.ds((SK - W) // 16, W // 16), :],
                dst.at[pl.ds(dst0, n)], sems.at[s])

        def vstage(c):
            return [vcopy((2 * c + p) * RH + RM, RF // 2, vs, ((2 * c + p) & 3) * (RF // 2), 1 + (c & 1))
                    for p in range(2)]

        def wcopies(src, dst, s, r0=0, nrows=None, step=None):
            su = src.bitcast(u32)
            nrows = dst.shape[1] if nrows is None else nrows
            step = nrows if step is None else step
            return [pltpu.make_async_copy(su.at[pl.ds(r, step), pl.ds(n * 128, 128)],
                                          dst.at[n, pl.ds(r, step)], sems.at[s])
                    for r in range(r0, r0 + nrows, step) for n in range(dst.shape[0])]

        head = [pltpu.make_async_copy(x_hbm, xin, sems.at[0]),
                pltpu.make_async_copy(b1_hbm, b1v, sems.at[0]),
                pltpu.make_async_copy(b2_hbm, b2v, sems.at[0])]
        head += [pltpu.make_async_copy(
            vu.at[pl.ds((NP - 2 + s) * RH, 8), :, pl.ds((SK - W) // 32, W // 32), :],
            vx.at[pl.ds(8 * s, 8)], sems.at[0]) for s in range(2)]
        head += wcopies(wq_hbm, wqb, 0) + wcopies(wo_hbm, wob, 0, step=WOSTEP) + [kcopy(0, 0)]
        vlast = [vcopy((NP - 2 + s) * RH + 8, RM - 8, vb, (NP - 2) * RM + s * (RM - 8), 2) for s in range(2)]
        c1 = wcopies(w1_hbm, w1b, 1)
        w2_split = tuple(int(z) for z in W2SPLIT.split(','))
        c2 = [wcopies(w2_hbm, w2b, (0, 3, 4)[g], 64 * w2_split[g],
                      64 * (w2_split[g + 1] - w2_split[g]),
                      min(W2STEP, 64 * (w2_split[g + 1] - w2_split[g]))) for g in range(len(w2_split) - 1)]
        c2all = [c for g in c2 for c in g]
        for c in head:
            c.start()

        def chunk(c):
            s = 1 + (c & 1)
            return [kcopy(c + 1, s)] + [vcopy((2 * c + p) * RH, RM, vb, (2 * c + p) * RM, s) for p in range(2)]

        for c in chunk(0) + vstage(0) + chunk(1):
            c.start()

        for i_ in range(NP):
            tbl[i_] = i_

        def qproj_tile(wg, dst, n):
            j, kt = divmod(n, KD)
            dst[n] = _tile_dot(xl[:, pl.ds(kt * 128, 128)], wg[j, pl.ds(kt * 64, 64), :])

        def build_l(src, dst, j):
            row = lax.broadcasted_iota(jnp.int32, (8, 128), 0)
            lane = lax.broadcasted_iota(jnp.int32, (8, 128), 1)
            q = _tree_sum(src[j * KD + kt] for kt in range(KD)) * rs_ref[...]
            qp = pltpu.roll(q, 8, 1)
            qm = pltpu.roll(q, 120, 1)
            tgt = (lane >> 1) & 4
            if j == 1:
                tgt = tgt + (lane >> 6)
            elif j == 2:
                tgt = tgt + 1
            hit = row == tgt
            low = row < 4
            dst[2 * j] = _pack_rows(jnp.where(hit, jnp.where(low, q, qp), 0.0))
            dst[2 * j + 1] = _pack_rows(jnp.where(hit, jnp.where(low, qm, q), 0.0))

        def qk_tile(kg, lsrc, sdst, c0, n, ncp=NCP):
            c4, rem = divmod(n, 4 * NT)
            t, i = divmod(rem, min(4, ncp - c4 * 4))
            c = c4 * 4 + i
            w = kg[pl.ds((t // 2) * 8, 8), t % 2, pl.ds((c0 + c) * 8, 8), :].reshape(64, 128)
            sdst[c, t] = _tile_dot(lsrc[t], w)

        def s_group(st, src, c0, c1):
            s = [_tree_sum(src[c, t] for t in range(src.shape[1])) for c in range(c0, c1)]
            base = len(st.setdefault("s", []))
            if SSPILL:
                for k_, a_ in enumerate(s):
                    ssum[st.get("zero", 0) + base + k_] = a_
            st["s"] += s
            st["m"] = _tree(jnp.maximum, s + ([st["m"]] if "m" in st else []))

        def s_max(st):
            m = jnp.maximum(st["m"], pltpu.roll(st["m"], 4, 0))
            st["m"] = jnp.max(m, axis=1, keepdims=True)

        def s_exp(st, pdst, ldst, kdst=None):
            s = [ssum[cp] for cp in range(NCP)] if SSPILL else st["s"]
            e = [jnp.exp2(a - st["m"]) for a in s]
            for cp in range(NCP):
                pdst[:, pl.ds(cp * 128, 128)] = e[cp]
                if kdst is not None:
                    kdst[cp] = _pack_rows(e[cp])
            ldst[...] = _tree_sum(e)

        def softmax_steps(lo, hi, pdst, ldst, kdst=None, zero=None, mid=None, tail=None):
            st = {} if zero is None else {"zero": zero}
            srcs = [(lo, CA), (hi, CB)] if mid is None else [(lo, CA), (mid, CM), (hi, CB - CM)]
            if tail is not None:
                srcs = [(lo, CA), (hi, CB - NVQ), (tail, NVQ)]
            steps = [P(s_group, st, src, c0, min(c0 + 4, n)) for src, n in srcs for c0 in range(0, n, 4)]
            return steps + [P(s_max, st), P(s_exp, st, pdst, ldst, kdst)]

        def softmax(*args):
            for f in softmax_steps(*args):
                f()

        def l_inv(lsrc, ldst):
            l = lsrc[...]
            l = l + pltpu.roll(l, 4, 0)
            l = jnp.sum(l, axis=1, keepdims=True)
            ldst[...] = jnp.broadcast_to(1.0 / l, (8, 128))

        def pack_p(psrc, kdst):
            for cp in range(NCP):
                kdst[cp] = _pack_rows(psrc[:, pl.ds(cp * 128, 128)])

        def reduce_o(asrc, lsrc, odst, j):
            blk = asrc[pl.ds(j * 16, 16)].reshape(128, 128)
            t = blk.T.reshape(16, 8, 128)
            if j == 1:
                lane = lax.broadcasted_iota(jnp.int32, (1, 128), 1)
                r = jnp.where(lane < 64, lsrc[0:1, :], lsrc[1:2, :])
            else:
                r = lsrc[j // 2:j // 2 + 1, :]
            odst[j] = _pack_rows(_tree_sum(t[i] for i in range(16)) * r)

        def x_tile(vg, n):
            s, rem = divmod(n, 2 * NCP)
            cp, e = divmod(rem, 2)
            w = vg[pl.ds(8 * s, 8), e, pl.ds(cp * 8, 8), :].reshape(64, 128)
            shi0[divmod(n, NT)] = _tile_dot(pk[s][cp], w)

        def x_finish(s):
            row = lax.broadcasted_iota(jnp.int32, (8, 128), 0)
            lane = lax.broadcasted_iota(jnp.int32, (8, 128), 1)
            o0 = _tree_sum(shi0[divmod((s * NCP + cp) * 2, NT)] for cp in range(NCP))
            o1 = _tree_sum(shi0[divmod((s * NCP + cp) * 2 + 1, NT)] for cp in range(NCP))
            low = row < 4
            direct = jnp.where(low, o0, o1)
            moved = jnp.where(low, pltpu.roll(o1, 8, 1), pltpu.roll(o0, 120, 1))
            o = jnp.where(((lane >> 1) & 4) == (row & 4), direct, moved)
            o = jnp.where((row & 3) == 0, o, 0.0) * li[s][0:1, :]
            ol[s][0] = _pack_rows(o)
            return o

        def wo_tile(wg, osrc, ydst, n):
            j, nt = divmod(n, KD)
            ydst[n] = _tile_dot(osrc[j], wg[nt, pl.ds(j * 64, 64), :])

        def y_fold(ysrc):
            for nt in range(KD):
                ysum[nt] = _tree_sum([ysum[nt]] + [ysrc[j * KD + nt] for j in range(NJ)])

        def copy(src, dst):
            for i in range(src.shape[0]):
                dst[i] = src[i]

        def kpair(i):
            return kb.at[pl.ds(i * RH, RH)]

        def wqpair(i):
            return wqb.at[pl.ds(i * NJ, NJ)]

        def wopair(i):
            r0 = i * (PD // 2)
            if not isinstance(i, int):
                r0 = pl.multiple_of(r0, PD // 2)
            return wob.at[:, pl.ds(r0, PD // 2), :]

        def run_block(first, i, a, rg0, sets, kinds, order, rate, pace_n, side, moff=0, done=None):
            if rg0:
                vg = vb.at[pl.ds((NP - 2) * RM + a * (RM - 8), RM - 8)]
            else:
                vg = vb.at[pl.ds(i * RM, RM)]
            voff = rg0 // 2
            sg = vs.at[pl.ds((i & 3) * (RF // 2), RF // 2)]
            fg = vf.at[pl.ds(i * RF, RF)]
            plain, order_rg = list(range(rg0, RP - RF)), []
            n_all = RP - rg0
            f0 = min(F0, n_all - RF) * n_all // RP
            slots = {f0 + (k_ + 1) * (n_all - f0) // RF - 1 for k_ in range(RF)}
            nf = 0
            for pos_ in range(n_all):
                if pos_ in slots:
                    order_rg.append(RP - RF + nf)
                    nf += 1
                else:
                    order_rg.append(plain.pop(0))
            pace = dict(z=i, cnt=0, views={})

            def mxu_tile(key, n):
                if pace_n and pace["cnt"] % pace_n == 0:
                    z = pace["z"]
                    link = pace["cnt"] // pace_n
                    for _ in range(pace_n * 4 // 3 if link else D0):
                        z = tbl[z]
                    pace["z"] = z
                    pace["views"] = {}
                pace["cnt"] += 1
                if key not in pace["views"]:
                    pace["views"][key] = kinds[key][1](pace["z"])
                kinds[key][2](pace["views"][key], n)

            mxu = [P(mxu_tile, key, n) for key in order for n in range(kinds[key][0])]
            side = sorted(side + [(moff + int(n * rate), f) for n, f in enumerate(mxu)], key=lambda z: z[0])
            cnt = 0
            si = 0
            acc = {}
            sizes, ovl = sets.split(":") if ":" in sets else (sets, "0")
            groups = []
            for size in (int(z) for z in sizes.split(",")):
                groups.append(order_rg[:size])
                order_rg = order_rg[size:]
            step = NCP - int(ovl)
            seq = [(rgs, t - gi * step) for t in range((len(groups) - 1) * step + NCP)
                   for gi, rgs in enumerate(groups) if 0 <= t - gi * step < NCP]
            for rgs, cp in seq:
                mult = {hh: (pb[a][pl.ds(hh, 1), pl.ds(cp * 128, 128)],
                             pb[a][pl.ds(4 + hh, 1), pl.ds(cp * 128, 128)])
                        for hh in sorted({rg // RH for rg in rgs})}
                for rg in rgs:
                    while si < len(side) and side[si][0] <= cnt:
                        side[si][1]()
                        si += 1
                    cnt += 1
                    m0, m1 = mult[rg // RH]
                    r = rg - (RP - RF)
                    if r >= 0 and not first:
                        v0, v1 = fg[r, 2 * cp], fg[r, 2 * cp + 1]
                    else:
                        src = sg.at[r // 2, r % 2] if r >= 0 else vg.at[rg // 2 - voff, rg % 2]
                        v = src[pl.ds(cp * 16, 16), :].astype(f32)
                        v0, v1 = v[:8], v[8:]
                        if r >= 0:
                            fg[r, 2 * cp] = v0
                            fg[r, 2 * cp + 1] = v1
                    if rg not in acc:
                        acc[rg] = v0 * m0 + v1 * m1
                    else:
                        acc[rg] = acc[rg] + v0 * m0 + v1 * m1
                    if cp == NCP - 1:
                        ac[a][rg] = acc[rg]
                        if done is not None and cnt <= CIN * NCP:
                            done(rg)
            assert not order_rg
            for _, f in side[si:]:
                f()

        def layer(x, first):
            nvq = 0 if first else NVQ
            xc, rs = _center(x)
            xl[...] = _pack_rows(xc)
            rs_ref[...] = jnp.broadcast_to(rs * c_exp, (8, 128))
            ac1[...] = jnp.zeros(ac1.shape, f32)
            li1[...] = jnp.zeros(li1.shape, f32)
            if WLAG == 1:
                yr0[...] = jnp.zeros(yr0.shape, f32)
            else:
                ol0[...] = jnp.zeros(ol0.shape, u32)
                yr1[...] = jnp.zeros(yr1.shape, f32)
            ysum[...] = jnp.zeros(ysum.shape, f32)

            for i, dst in enumerate((qr2, qr3)):
                for n in range(NW):
                    qproj_tile(wqpair(i), dst, n)
            if Q2EARLY:
                for n in range(NW):
                    qproj_tile(wqpair(2), qr0, n)
            def vpu_qk():
                if not nvq:
                    return
                row = lax.broadcasted_iota(jnp.int32, (8, 128), 0)
                cols = jnp.concatenate(
                    [_columns((_tree_sum(qr2[j * KD + kt] for kt in range(KD)) * rs_ref[...])
                              .astype(bf16 if QRND else f32).astype(f32)) for j in range(NJ)], axis=0)
                sacc = {}
                for rg, cp in [(rg, cp) for c0_ in range(NCP - NVQ, NCP, VGRP) for rg in range(RP)
                               for cp in range(c0_, min(c0_ + VGRP, NCP))]:
                    if True:
                        kv = pltpu.bitcast(kb[rg // 2, rg % 2, pl.ds(cp * 8, 8), :], bf16).astype(f32)
                        for p_ in range(2):
                            t = kv[8 * p_:8 * p_ + 8] * cols[8 * rg:8 * rg + 8]
                            key = (cp, 4 * p_ + rg // RH)
                            prev = (cp - VGRP, key[1])
                            if key in sacc:
                                sacc[key] = sacc[key] + t
                            elif CUMQ and prev in sacc:
                                sacc[key] = sacc[prev] + t
                            else:
                                sacc[key] = t
                for cp in range(NCP - NVQ, NCP):
                    a_ = jnp.zeros((8, 128), f32)
                    for r_ in (0, 1, 4, 5):
                        z_ = sacc[cp, r_]
                        if CUMQ and (cp - VGRP, r_) in sacc:
                            z_ = z_ - sacc[cp - VGRP, r_]
                        a_ = jnp.where(row == r_, _sublane_sum(z_), a_)
                    svq[cp - (NCP - NVQ), 0] = a_

            for j in range(NJ):
                build_l(qr2, lp, j)
            if VFIRST:
                vpu_qk()
            for n in range(CA * NT):
                qk_tile(kpair(0), lp, slo0, 0, n)
            for n in range((CB - nvq) * NT):
                qk_tile(kpair(0), lp, shi0, CA, n, CB - nvq)
            if not VFIRST:
                vpu_qk()
            for j in range(NJ):
                build_l(qr3, ln1, j)
            for n in range(CA * NT):
                qk_tile(kpair(1), ln1, slo1, 0, n)
            if not Q2EARLY:
                for n in range(NW):
                    qproj_tile(wqpair(2), qr0, n)
            softmax(slo0, shi0, pb0, ls0, None, None, None, svq if nvq else None)

            wp = lambda a: 1 - a if WLAG == 1 else a

            def kinds(a):
                b = 1 - a
                return dict(
                    h=(CB * NT, lambda z: kpair(z + 1),
                       lambda w, n: qk_tile(w, ln[b], shi[b], CA, n)),
                    l=(CA * NT, lambda z: kpair(z + 2),
                       lambda w, n: qk_tile(w, ln[a], slo[a], 0, n)),
                    q=(NW, lambda z: wqpair(jnp.minimum(z + 3, NP - 1)),
                       lambda w, n: qproj_tile(w, qr[b], n)),
                    w=(NW, lambda z: wopair(jnp.maximum(z - WLAG, 0)),
                       lambda w, n: wo_tile(w, ol[wp(a)], yr[wp(a)], n)),
                    v=(2 * KD, lambda z: wopair(z - 1),
                       lambda w, n: wo_tile(w, ol[b], yr[b], KD + n)),
                    u=(NW, lambda z: wopair(z - 1),
                       lambda w, n: wo_tile(w, ol1, qr1, n)),
                    m=(CM * NT, lambda z: kpair(z + 2),
                       lambda w, n: qk_tile(w, ln[a], smid, CA, n, CM)),
                    g=((CB - CM) * NT, lambda z: kpair(z + 1),
                       lambda w, n: qk_tile(w, ln[b], shi[b], CA + CM, n, CB - CM)),
                    x=(4 * NCP, lambda z: vx.at[pl.ds((z - (NP - 1)) * 16, 16)], x_tile))

            def block(i, a, order=MORD, RATE=RATE, SETS=SETS, PACE=PACE):
                b = 1 - a
                steps = softmax_steps(slo[b], shi[b], pb[b], ls[b], None, tbl[i] - i if SSPILL == 2 else None)
                if STAGED:
                    pos = [GPOS] * XA + [MOFF + int(24 * (k_ + 1) * RATE) + GLAG for k_ in range(4 - XA)]
                    pos += [pos[-1] + 1, pos[-1] + ELAG]
                else:
                    pos = [max(SPOS, MOFF + int(CB * NT * RATE) + 1)] * len(steps)
                side = list(zip(pos, steps))
                side += [(IPOS, P(l_inv, ls[a], li[a])),
                         (YPOS, P(y_fold, yr[1 - wp(a)]))]
                for j in range(NJ):
                    side.append((LPOS + LSTEP * j, P(build_l, qr[a], ln[a], j)))
                    side.append((RPOS + RSTEP * j, P(reduce_o, ac[b], li[b], ol[b], j)))
                run_block(first, i, a, 0, SETS, kinds(a), order, RATE, PACE, side, MOFF)

            def block14(i):
                side = [(int((CB - CM) * NT * RATE14) + SL14, P(softmax, slo1, shi1, pb1, ls1, pk1, None, smid)),
                        (IPOS14, P(l_inv, ls0, li0)),
                        (KPOS, P(pack_p, pb0, pk0)),
                        (YP14, P(y_fold, yr[1 - wp(0)]))]
                for j in range(NJ):
                    side.append((RP14 + RS14 * j, P(reduce_o, ac1, li1, ol1, j)))
                run_block(first, i, 0, 16, SETS14, kinds(0), ORD14, RATE14, PACE14, side)

            cin = set()

            def col_sum(rg):
                cin.add(rg)
                ac0[rg - 16] = jnp.broadcast_to(jnp.sum(ac1[rg], axis=1, keepdims=True), (8, 128))

            def block15(i):
                side = [(IPOS15, P(l_inv, ls1, li1)),
                        (YP15, P(y_fold, yr[1 - wp(1)]))]
                if "u" in ORD14:
                    side.append((YP15 + 20, P(y_fold, qr1)))
                for j in range(1, NJ):
                    side.append((RP15 + RS15 * j, P(reduce_o, ac0, li0, ol0, j)))
                if RIN15 >= 1:
                    side.append((16 * NCP + 1, P(reduce_o, ac1, li1, ol1, 1)))
                if RIN15 >= 2:
                    side.append((32 * NCP + 1, P(reduce_o, ac1, li1, ol1, 2)))
                run_block(first, i, 1, 16, SETS15, kinds(1), ORD15, RATE15, PACE15, side, 0, col_sum)

            def body(i, c):
                if first:
                    @pl.when((i & 1) == 0)
                    def _():
                        ch = lax.shift_right_logical(i, 1)
                        for c in chunk(ch) + vstage(ch):
                            c.wait()
                        for c in vstage(ch + 1):
                            c.start()

                        @pl.when(ch + 2 < NC - 1)
                        def _():
                            for c in chunk(ch + 2):
                                c.start()

                        @pl.when(ch + 2 == NC - 1)
                        def _():
                            for c in vlast:
                                c.start()

                        @pl.when(ch + 1 == NC - 1)
                        def _():
                            for c in c1 + c2all:
                                c.start()

                for a in range(2):
                    pl.when((i & 1) == a)(P(block, i, a))
                return c

            lax.fori_loop(0, NP - 3, body, 0)

            def tail(i, c):
                pl.when(i == NP - 3)(P(block, i, 1, MORD13, RATE13, SETS13, PACE13))
                if first:
                    @pl.when(i == NP - 2)
                    def _():
                        for c in vlast + vstage(NC - 1):
                            c.wait()

                pl.when(i == NP - 2)(P(block14, i))
                pl.when(i == NP - 1)(P(block15, i))
                return c

            lax.fori_loop(NP - 3, NP, tail, 0)

            ox = [x_finish(0), x_finish(1)]
            for n in (list(range(KD, NW)) if "v" not in ORD15 else []) + list(range(KD)):
                wo_tile(wopair(NP - 2), ol0, yr0, n)
            for n in range(KD):
                wo_tile(wopair(NP - 1), ol1, qr0, n)
            wl = wopair(NP - 1)
            yv, mv = {}, {}
            for m in range(8, RH):
                c0, c1_ = [ac0[rg - 16] if rg in cin else jnp.sum(ac1[rg], axis=1, keepdims=True)
                           for rg in (2 * m, 2 * m + 1)]
                hh = 2 * m // RH
                for nt in range(KD):
                    w = pltpu.bitcast(wl[nt, pl.ds(8 * m, 8), :], bf16).astype(f32)
                    t = w[:8] * c0 + w[8:] * c1_
                    yv[hh, nt] = t if (hh, nt) not in yv else yv[hh, nt] + t
                t = wsc[2 * m - 16] * c0 + wsc[2 * m - 15] * c1_
                mv[hh] = t if hh not in mv else mv[hh] + t
            early = [_tree_sum([ysum[nt]] + [yr1[j * KD + nt] for j in range(NJ) if "u" not in ORD14]
                               + [yr0[j * KD + nt] for j in range(1, NJ)]) for nt in range(KD)]
            ys = [_tree_sum([early[nt], yr0[nt], qr0[nt],
                             yv[0, nt] * li1[0:1, :], yv[1, nt] * li1[1:2, :]]) for nt in range(KD)]
            y = jnp.sum(jnp.concatenate(ys, axis=1), axis=0, keepdims=True)
            lanes = _tree_sum(early + [x[:, nt * 128:(nt + 1) * 128] * 0.125 for nt in range(KD)]
                              + [ox[0] * wsl[0], ox[1] * wsl[1]])
            tot = (jnp.sum(lanes, axis=1, keepdims=True)
                   + mv[0] * li1[0:1, :] + mv[1] * li1[1:2, :])
            mean = jnp.concatenate([_sublane_sum(tot) * (1.0 / D)] * KD, axis=1)
            x = x + y

            xc, rs = _center(x, mean)
            xn = _pack_rows(xc)
            if first:
                for c in c1:
                    c.wait()
            nv = 0 if first else NV2
            gs = {}
            nv1 = 0 if first else NV1
            for n in range(KF - nv1):
                h = _tree_sum(_tile_dot(xn[:, kt * 128:(kt + 1) * 128], w1b[n, pl.ds(kt * 64, 64), :])
                              for kt in range(KD))
                gs[n] = _gelu(h * rs + b1v[n:n + 1, :].astype(f32))
            hacc = {}
            for kt in range(KD if nv1 else 0):
                col = _columns(xc[:, kt * 128:(kt + 1) * 128])
                for v in range(8):
                    for n in range(KF - nv1, KF):
                        w = pltpu.bitcast(w1b[n, pl.ds(kt * 64 + 8 * v, 8), :], bf16).astype(f32)
                        t = w[:8] * col[16 * v:16 * v + 8] + w[8:] * col[16 * v + 8:16 * v + 16]
                        hacc[n] = t if n not in hacc else hacc[n] + t
            for n in hacc:
                gs[n] = _gelu(_sublane_sum(hacc[n]) * rs + b1v[n:n + 1, :].astype(f32))
            vacc = [None] * KD
            for kt in range(nv):
                col = _columns(gs[kt])
                for v in range(8):
                    for nt in range(KD):
                        w = pltpu.bitcast(w2b[nt, pl.ds(kt * 64 + 8 * v, 8), :], bf16).astype(f32)
                        t = w[:8] * col[16 * v:16 * v + 8] + w[8:] * col[16 * v + 8:16 * v + 16]
                        vacc[nt] = t if vacc[nt] is None else vacc[nt] + t
            parts = []
            for kt in range(nv, KF):
                if first and kt in w2_split:
                    for c in c2[w2_split.index(kt)]:
                        c.wait()
                hk = _pack_rows(gs[kt])
                parts.append([_tile_dot(hk, w2b[nt, pl.ds(kt * 64, 64), :]) for nt in range(KD)])
            y2 = jnp.concatenate(
                [_tree_sum([p[nt] for p in parts] + [b2v[nt:nt + 1, :].astype(f32)]
                           + ([_sublane_sum(vacc[nt])] if nv else []))
                 for nt in range(KD)], axis=1)
            return x + y2

        for c in head:
            c.wait()

        def wo_rowsums(r0):
            w = _tree_sum(pltpu.bitcast(wob[nt, pl.ds(r0, 8), :], bf16).astype(f32) for nt in range(KD))
            return jnp.broadcast_to(jnp.sum(w, axis=1, keepdims=True), (16, 128))

        for m in range(8, RH):
            wsc[pl.ds(2 * m - 16, 2)] = wo_rowsums((NP - 1) * (PD // 2) + 8 * m).reshape(2, 8, 128)
        for s_ in range(2):
            cols = jnp.concatenate([wo_rowsums((NP - 2 + s_) * (PD // 2) + 8 * m) for m in range(8)], axis=0)
            wsl[s_] = cols.T[0:8]

        def transpose_tile(n, c):
            s8 = pl.multiple_of((n // (2 * NCP)) * 8, 8)
            e = n % 2
            c8 = pl.multiple_of(((n // 2) % NCP) * 8, 8)
            w = vx[pl.ds(s8, 8), e, pl.ds(c8, 8), :].reshape(64, 128)
            wt = pltpu.bitcast(w, bf16).astype(f32).T.astype(bf16)
            vx[pl.ds(s8, 8), e, pl.ds(c8, 8), :] = pltpu.bitcast(wt, u32).reshape(8, 8, 128)
            return c

        lax.fori_loop(0, 4 * NCP, transpose_tile, 0)

        if ONLY2:
            for c in chunk(0) + vstage(0) + chunk(1):
                c.wait()
        x = jnp.broadcast_to(xin[0].astype(f32), (8, D))
        for l_ in range(1 if ONLY2 else NL):
            x = layer(x, l_ == 0 and not ONLY2)
        o_ref[0] = x[0:1, :].astype(o_ref.dtype)

    return kernel


@jax.jit
def pallas_interleave_layers__sliding_block_cached__dense_activation_gelu__decode_kernel(
    A_x, A_k_cache, A_v_cache, A_wq, A_wo, B_x, B_w1, B_b1, B_w2, B_b2,
):
    SK = A_k_cache.shape[2]
    W = min(4096, max(256, SK // 4))
    NR = H * DH // 8

    def tiled(a):
        t = jnp.swapaxes(a, 2, 3).reshape(NR, 8, SK // 128, 128)
        return t.transpose(0, 2, 1, 3).reshape(NR // 2, 2, SK // 16, 128)

    b1 = B_b1.reshape(F // 128, 128)
    b2 = B_b2.reshape(D // 128, 128)
    anyspec = pl.BlockSpec(memory_space=pl.ANY)
    NCP = W // 256
    vreg = lambda n, dt: pltpu.VMEM(n + (8, 128), dt)
    return pl.pallas_call(
        _make_kernel(SK, W),
        out_shape=jax.ShapeDtypeStruct(A_x.shape, A_x.dtype),
        in_specs=[anyspec] * 9,
        out_specs=pl.BlockSpec(memory_space=pltpu.VMEM),
        scratch_shapes=[
            pltpu.VMEM((NR // 2, 2, W // 32, 128), u32),
            pltpu.VMEM((NR // 2 - 16 - NP * RF // 2, 2, W // 16, 128), bf16),
            pltpu.VMEM((2 * RF, 2, W // 16, 128), bf16),
            pltpu.VMEM((16, 2, W // 32, 128), u32),
            vreg((NP * max(RF, 1), 2 * NCP), f32),
            pltpu.VMEM((H * DH // 128, D // 2, 128), u32),
            pltpu.VMEM((KD, H * DH // 2, 128), u32),
            pltpu.VMEM((KF, D // 2, 128), u32),
            pltpu.VMEM((KD, F // 2, 128), u32),
            pltpu.VMEM((1, 1, D), bf16),
            pltpu.VMEM((KF, 128), bf16),
            pltpu.VMEM((KD, 128), bf16),
            pltpu.VMEM((8, D), u32),
            pltpu.VMEM((8, 128), f32),
            vreg((KD,), f32),
            vreg((NCP if SSPILL else 1,), f32),
        ] + [vreg((NT,), u32)] * 3
          + [vreg((NW,), f32)] * 4
          + [vreg((4 * XA, NT), f32)] * 2
          + [vreg((CM, NT), f32)]
          + [vreg((NCP - 4 * XA, NT), f32)] * 2
          + [pltpu.VMEM((8, NCP * 128), f32)] * 2
          + [pltpu.VMEM((8, 128), f32)] * 4
          + [vreg((RP,), f32)] * 2
          + [vreg((NJ,), u32)] * 2
          + [vreg((NW,), f32)] * 2
          + [vreg((NCP,), u32)] * 2
          + [vreg((32,), f32), vreg((2,), f32)]
          + [vreg((max(NVQ, 1), 1), f32)]
          + [pltpu.SMEM((NP,), jnp.int32)]
          + [pltpu.SemaphoreType.DMA((5,))],
        compiler_params=pltpu.CompilerParams(vmem_limit_bytes=128 * 1024 * 1024,
                                             disable_semaphore_checks=bool(NOSEM)),
    )(A_x, tiled(A_k_cache), tiled(A_v_cache), A_wq, A_wo, B_w1, b1, B_w2, b2)
```

```python
import functools
import jax
import jax.numpy as jnp
from jax import lax
import jax.experimental.pallas as pl
import jax.experimental.pallas.tpu as pltpu

D = 640
H = 32
DH = 192
F = 1536
NP = H // 2
PD = 2 * DH
RH = DH // 8
RP = 2 * RH
NJ = PD // 128
NT = 2 * NJ
KD = D // 128
KF = F // 128
NW = NJ * KD
EPS = 1e-5
LOG2E = 1.4426950408889634
bf16 = jnp.bfloat16
f32 = jnp.float32
u32 = jnp.uint32

RATE = 6.0
SPOS = 450
LPOS = 100
RPOS = 300
RSTEP = 80
YPOS = 5
IPOS = 150
IPOS14 = 10
IPOS15 = 10
SETS13 = "6,6,6,6,6,18"
CM = 2
RIN15 = 0
NV2 = 5
NV1 = 3
CIN = 0
ONEPASS = 0
NVQ = 6
VFIRST = 0
VGRP = 2
QRND = 1
CUMQ = 1
SL14 = 10
KPOS = 100
YP14 = 5
YP15 = 5
RS15 = 10
MORD13 = "hwlm"
RATE13 = 6.1
CPOS = 200
NL = 2
MORD = "hwql"
SSPILL = 0
PACE = 6
PACE13 = 3
D0 = 1
XA = 1
SETS = "10,10,10,18"
SETS14 = "8,8,8,8"
SETS15 = "8,8,10,6"
RATE14 = 5.6
RATE15 = 6.2
PACE14 = 3
PACE15 = 3
ONLY2 = 0
NOSEM = 0
STAGED = 0
GPOS = 30
GLAG = 60
ELAG = 80
MOFF = 0
LSTEP = 10
WOSTEP = 256
W2STEP = 192
W2SPLIT = "0,9,11,12"
RF = 8
F0 = 15
RP14 = 100
RP15 = 100
RS14 = 10
ORD14 = "gwu"
WLAG = 2
ORD15 = "xv"
Q2EARLY = 1


def _center(x, mean=None):
    if mean is not None:
        xc = x - mean
        v = jnp.mean(xc * xc, axis=-1, keepdims=True)
        return xc, lax.rsqrt(v + EPS)
    if ONEPASS:
        m = jnp.mean(x, axis=-1, keepdims=True)
        v = jnp.maximum(jnp.mean(x * x, axis=-1, keepdims=True) - m * m, 0.0)
        return x - m, lax.rsqrt(v + EPS)
    xc = x - jnp.mean(x, axis=-1, keepdims=True)
    v = jnp.mean(xc * xc, axis=-1, keepdims=True)
    return xc, lax.rsqrt(v + EPS)


def _gelu(x):
    c = 0.7978845608028654
    return 0.5 * x * (1.0 + jnp.tanh(c * (x + 0.044715 * (x * x * x))))


def _pack_rows(x8):
    x16 = jnp.concatenate([x8, x8], axis=0).astype(bf16)
    return pltpu.bitcast(x16, u32)


def _tile_dot(lhs_u32, w_u32):
    return jnp.dot(pltpu.bitcast(lhs_u32, bf16), pltpu.bitcast(w_u32, bf16),
                   preferred_element_type=f32)[0:8]


def _columns(x8):
    return jnp.concatenate([x8] * 16, axis=0).T


def _sublane_sum(x8):
    for sh in (4, 2, 1):
        x8 = x8 + pltpu.roll(x8, sh, 0)
    return x8


def _tree(op, xs):
    xs = list(xs)
    while len(xs) > 1:
        xs = [op(xs[i], xs[i + 1]) if i + 1 < len(xs) else xs[i] for i in range(0, len(xs), 2)]
    return xs[0]


def _tree_sum(xs):
    return _tree(jnp.add, xs)


def _make_kernel(SK, W):
    NCP = W // 256
    CA = 4 * XA
    CB = NCP - CA
    c_exp = (DH ** -0.5) * LOG2E
    P = functools.partial

    def kernel(x_hbm, k_hbm, v_hbm, wq_hbm, wo_hbm, w1_hbm, b1_hbm, w2_hbm, b2_hbm,
               o_ref,
               kb, vb, vs, vx, vf, wqb, wob, w1b, w2b, xin, b1v, b2v, xl, rs_ref, ysum, ssum,
               ln0, ln1, lp, qr0, qr1, qr2, qr3, slo0, slo1, smid, shi0, shi1, pb0, pb1,
               ls0, ls1, li0, li1, ac0, ac1, ol0, ol1, yr0, yr1, pk0, pk1, wsc, wsl, svq, tbl, sems):
        ln, qr, slo, shi = (ln0, ln1), (qr0, qr1), (slo0, slo1), (shi0, shi1)
        pb, ls, li, ac, ol, yr = (pb0, pb1), (ls0, ls1), (li0, li1), (ac0, ac1), (ol0, ol1), (yr0, yr1)
        pk = (pk0, pk1)
        ku = k_hbm.bitcast(u32)
        vu = v_hbm.bitcast(u32)
        NC = NP // 2

        def kcopy(c, s):
            return pltpu.make_async_copy(
                ku.at[pl.ds(c * RP, RP), :, pl.ds((SK - W) // 32, W // 32), :],
                kb.at[pl.ds(c * RP, RP)], sems.at[s])

        RM = RH - RF // 2

        def vcopy(src0, n, dst, dst0, s):
            return pltpu.make_async_copy(
                v_hbm.at[pl.ds(src0, n), :, pl.ds((SK - W) // 16, W // 16), :],
                dst.at[pl.ds(dst0, n)], sems.at[s])

        def vstage(c):
            return [vcopy((2 * c + p) * RH + RM, RF // 2, vs, ((2 * c + p) & 3) * (RF // 2), 1 + (c & 1))
                    for p in range(2)]

        def wcopies(src, dst, s, r0=0, nrows=None, step=None):
            su = src.bitcast(u32)
            nrows = dst.shape[1] if nrows is None else nrows
            step = nrows if step is None else step
            return [pltpu.make_async_copy(su.at[pl.ds(r, step), pl.ds(n * 128, 128)],
                                          dst.at[n, pl.ds(r, step)], sems.at[s])
                    for r in range(r0, r0 + nrows, step) for n in range(dst.shape[0])]

        head = [pltpu.make_async_copy(x_hbm, xin, sems.at[0]),
                pltpu.make_async_copy(b1_hbm, b1v, sems.at[0]),
                pltpu.make_async_copy(b2_hbm, b2v, sems.at[0])]
        head += [pltpu.make_async_copy(
            vu.at[pl.ds((NP - 2 + s) * RH, 8), :, pl.ds((SK - W) // 32, W // 32), :],
            vx.at[pl.ds(8 * s, 8)], sems.at[0]) for s in range(2)]
        head += wcopies(wq_hbm, wqb, 0) + wcopies(wo_hbm, wob, 0, step=WOSTEP) + [kcopy(0, 0)]
        vlast = [vcopy((NP - 2 + s) * RH + 8, RM - 8, vb, (NP - 2) * RM + s * (RM - 8), 2) for s in range(2)]
        c1 = wcopies(w1_hbm, w1b, 1)
        w2_split = tuple(int(z) for z in W2SPLIT.split(','))
        c2 = [wcopies(w2_hbm, w2b, (0, 3, 4)[g], 64 * w2_split[g],
                      64 * (w2_split[g + 1] - w2_split[g]),
                      min(W2STEP, 64 * (w2_split[g + 1] - w2_split[g]))) for g in range(len(w2_split) - 1)]
        c2all = [c for g in c2 for c in g]
        for c in head:
            c.start()

        def chunk(c):
            s = 1 + (c & 1)
            return [kcopy(c + 1, s)] + [vcopy((2 * c + p) * RH, RM, vb, (2 * c + p) * RM, s) for p in range(2)]

        for c in chunk(0) + vstage(0) + chunk(1):
            c.start()

        for i_ in range(NP):
            tbl[i_] = i_

        def qproj_tile(wg, dst, n):
            j, kt = divmod(n, KD)
            dst[n] = _tile_dot(xl[:, pl.ds(kt * 128, 128)], wg[j, pl.ds(kt * 64, 64), :])

        def build_l(src, dst, j):
            row = lax.broadcasted_iota(jnp.int32, (8, 128), 0)
            lane = lax.broadcasted_iota(jnp.int32, (8, 128), 1)
            q = _tree_sum(src[j * KD + kt] for kt in range(KD)) * rs_ref[...]
            qp = pltpu.roll(q, 8, 1)
            qm = pltpu.roll(q, 120, 1)
            tgt = (lane >> 1) & 4
            if j == 1:
                tgt = tgt + (lane >> 6)
            elif j == 2:
                tgt = tgt + 1
            hit = row == tgt
            low = row < 4
            dst[2 * j] = _pack_rows(jnp.where(hit, jnp.where(low, q, qp), 0.0))
            dst[2 * j + 1] = _pack_rows(jnp.where(hit, jnp.where(low, qm, q), 0.0))

        def qk_tile(kg, lsrc, sdst, c0, n, ncp=NCP):
            c4, rem = divmod(n, 4 * NT)
            t, i = divmod(rem, min(4, ncp - c4 * 4))
            c = c4 * 4 + i
            w = kg[pl.ds((t // 2) * 8, 8), t % 2, pl.ds((c0 + c) * 8, 8), :].reshape(64, 128)
            sdst[c, t] = _tile_dot(lsrc[t], w)

        def s_group(st, src, c0, c1):
            s = [_tree_sum(src[c, t] for t in range(src.shape[1])) for c in range(c0, c1)]
            base = len(st.setdefault("s", []))
            if SSPILL:
                for k_, a_ in enumerate(s):
                    ssum[st.get("zero", 0) + base + k_] = a_
            st["s"] += s
            st["m"] = _tree(jnp.maximum, s + ([st["m"]] if "m" in st else []))

        def s_max(st):
            m = jnp.maximum(st["m"], pltpu.roll(st["m"], 4, 0))
            st["m"] = jnp.max(m, axis=1, keepdims=True)

        def s_exp(st, pdst, ldst, kdst=None):
            s = [ssum[cp] for cp in range(NCP)] if SSPILL else st["s"]
            e = [jnp.exp2(a - st["m"]) for a in s]
            for cp in range(NCP):
                pdst[:, pl.ds(cp * 128, 128)] = e[cp]
                if kdst is not None:
                    kdst[cp] = _pack_rows(e[cp])
            ldst[...] = _tree_sum(e)

        def softmax_steps(lo, hi, pdst, ldst, kdst=None, zero=None, mid=None, tail=None):
            st = {} if zero is None else {"zero": zero}
            srcs = [(lo, CA), (hi, CB)] if mid is None else [(lo, CA), (mid, CM), (hi, CB - CM)]
            if tail is not None:
                srcs = [(lo, CA), (hi, CB - NVQ), (tail, NVQ)]
            steps = [P(s_group, st, src, c0, min(c0 + 4, n)) for src, n in srcs for c0 in range(0, n, 4)]
            return steps + [P(s_max, st), P(s_exp, st, pdst, ldst, kdst)]

        def softmax(*args):
            for f in softmax_steps(*args):
                f()

        def l_inv(lsrc, ldst):
            l = lsrc[...]
            l = l + pltpu.roll(l, 4, 0)
            l = jnp.sum(l, axis=1, keepdims=True)
            ldst[...] = jnp.broadcast_to(1.0 / l, (8, 128))

        def pack_p(psrc, kdst):
            for cp in range(NCP):
                kdst[cp] = _pack_rows(psrc[:, pl.ds(cp * 128, 128)])

        def reduce_o(asrc, lsrc, odst, j):
            blk = asrc[pl.ds(j * 16, 16)].reshape(128, 128)
            t = blk.T.reshape(16, 8, 128)
            if j == 1:
                lane = lax.broadcasted_iota(jnp.int32, (1, 128), 1)
                r = jnp.where(lane < 64, lsrc[0:1, :], lsrc[1:2, :])
            else:
                r = lsrc[j // 2:j // 2 + 1, :]
            odst[j] = _pack_rows(_tree_sum(t[i] for i in range(16)) * r)

        def x_tile(vg, n):
            s, rem = divmod(n, 2 * NCP)
            cp, e = divmod(rem, 2)
            w = vg[pl.ds(8 * s, 8), e, pl.ds(cp * 8, 8), :].reshape(64, 128)
            shi0[divmod(n, NT)] = _tile_dot(pk[s][cp], w)

        def x_finish(s):
            row = lax.broadcasted_iota(jnp.int32, (8, 128), 0)
            lane = lax.broadcasted_iota(jnp.int32, (8, 128), 1)
            o0 = _tree_sum(shi0[divmod((s * NCP + cp) * 2, NT)] for cp in range(NCP))
            o1 = _tree_sum(shi0[divmod((s * NCP + cp) * 2 + 1, NT)] for cp in range(NCP))
            low = row < 4
            direct = jnp.where(low, o0, o1)
            moved = jnp.where(low, pltpu.roll(o1, 8, 1), pltpu.roll(o0, 120, 1))
            o = jnp.where(((lane >> 1) & 4) == (row & 4), direct, moved)
            o = jnp.where((row & 3) == 0, o, 0.0) * li[s][0:1, :]
            ol[s][0] = _pack_rows(o)
            return o

        def wo_tile(wg, osrc, ydst, n):
            j, nt = divmod(n, KD)
            ydst[n] = _tile_dot(osrc[j], wg[nt, pl.ds(j * 64, 64), :])

        def y_fold(ysrc):
            for nt in range(KD):
                ysum[nt] = _tree_sum([ysum[nt]] + [ysrc[j * KD + nt] for j in range(NJ)])

        def copy(src, dst):
            for i in range(src.shape[0]):
                dst[i] = src[i]

        def kpair(i):
            return kb.at[pl.ds(i * RH, RH)]

        def wqpair(i):
            return wqb.at[pl.ds(i * NJ, NJ)]

        def wopair(i):
            r0 = i * (PD // 2)
            if not isinstance(i, int):
                r0 = pl.multiple_of(r0, PD // 2)
            return wob.at[:, pl.ds(r0, PD // 2), :]

        def run_block(first, i, a, rg0, sets, kinds, order, rate, pace_n, side, moff=0, done=None):
            if rg0:
                vg = vb.at[pl.ds((NP - 2) * RM + a * (RM - 8), RM - 8)]
            else:
                vg = vb.at[pl.ds(i * RM, RM)]
            voff = rg0 // 2
            sg = vs.at[pl.ds((i & 3) * (RF // 2), RF // 2)]
            fg = vf.at[pl.ds(i * RF, RF)]
            plain, order_rg = list(range(rg0, RP - RF)), []
            n_all = RP - rg0
            f0 = min(F0, n_all - RF) * n_all // RP
            slots = {f0 + (k_ + 1) * (n_all - f0) // RF - 1 for k_ in range(RF)}
            nf = 0
            for pos_ in range(n_all):
                if pos_ in slots:
                    order_rg.append(RP - RF + nf)
                    nf += 1
                else:
                    order_rg.append(plain.pop(0))
            pace = dict(z=i, cnt=0, views={})

            def mxu_tile(key, n):
                if pace_n and pace["cnt"] % pace_n == 0:
                    z = pace["z"]
                    link = pace["cnt"] // pace_n
                    for _ in range(pace_n * 4 // 3 if link else D0):
                        z = tbl[z]
                    pace["z"] = z
                    pace["views"] = {}
                pace["cnt"] += 1
                if key not in pace["views"]:
                    pace["views"][key] = kinds[key][1](pace["z"])
                kinds[key][2](pace["views"][key], n)

            mxu = [P(mxu_tile, key, n) for key in order for n in range(kinds[key][0])]
            side = sorted(side + [(moff + int(n * rate), f) for n, f in enumerate(mxu)], key=lambda z: z[0])
            cnt = 0
            si = 0
            acc = {}
            sizes, ovl = sets.split(":") if ":" in sets else (sets, "0")
            groups = []
            for size in (int(z) for z in sizes.split(",")):
                groups.append(order_rg[:size])
                order_rg = order_rg[size:]
            step = NCP - int(ovl)
            seq = [(rgs, t - gi * step) for t in range((len(groups) - 1) * step + NCP)
                   for gi, rgs in enumerate(groups) if 0 <= t - gi * step < NCP]
            for rgs, cp in seq:
                mult = {hh: (pb[a][pl.ds(hh, 1), pl.ds(cp * 128, 128)],
                             pb[a][pl.ds(4 + hh, 1), pl.ds(cp * 128, 128)])
                        for hh in sorted({rg // RH for rg in rgs})}
                for rg in rgs:
                    while si < len(side) and side[si][0] <= cnt:
                        side[si][1]()
                        si += 1
                    cnt += 1
                    m0, m1 = mult[rg // RH]
                    r = rg - (RP - RF)
                    if r >= 0 and not first:
                        v0, v1 = fg[r, 2 * cp], fg[r, 2 * cp + 1]
                    else:
                        src = sg.at[r // 2, r % 2] if r >= 0 else vg.at[rg // 2 - voff, rg % 2]
                        v = src[pl.ds(cp * 16, 16), :].astype(f32)
                        v0, v1 = v[:8], v[8:]
                        if r >= 0:
                            fg[r, 2 * cp] = v0
                            fg[r, 2 * cp + 1] = v1
                    if rg not in acc:
                        acc[rg] = v0 * m0 + v1 * m1
                    else:
                        acc[rg] = acc[rg] + v0 * m0 + v1 * m1
                    if cp == NCP - 1:
                        ac[a][rg] = acc[rg]
                        if done is not None and cnt <= CIN * NCP:
                            done(rg)
            assert not order_rg
            for _, f in side[si:]:
                f()

        def layer(x, first):
            nvq = 0 if first else NVQ
            xc, rs = _center(x)
            xl[...] = _pack_rows(xc)
            rs_ref[...] = jnp.broadcast_to(rs * c_exp, (8, 128))
            ac1[...] = jnp.zeros(ac1.shape, f32)
            li1[...] = jnp.zeros(li1.shape, f32)
            if WLAG == 1:
                yr0[...] = jnp.zeros(yr0.shape, f32)
            else:
                ol0[...] = jnp.zeros(ol0.shape, u32)
                yr1[...] = jnp.zeros(yr1.shape, f32)
            ysum[...] = jnp.zeros(ysum.shape, f32)

            for i, dst in enumerate((qr2, qr3)):
                for n in range(NW):
                    qproj_tile(wqpair(i), dst, n)
            if Q2EARLY:
                for n in range(NW):
                    qproj_tile(wqpair(2), qr0, n)
            def vpu_qk():
                if not nvq:
                    return
                row = lax.broadcasted_iota(jnp.int32, (8, 128), 0)
                cols = jnp.concatenate(
                    [_columns((_tree_sum(qr2[j * KD + kt] for kt in range(KD)) * rs_ref[...])
                              .astype(bf16 if QRND else f32).astype(f32)) for j in range(NJ)], axis=0)
                sacc = {}
                for rg, cp in [(rg, cp) for c0_ in range(NCP - NVQ, NCP, VGRP) for rg in range(RP)
                               for cp in range(c0_, min(c0_ + VGRP, NCP))]:
                    if True:
                        kv = pltpu.bitcast(kb[rg // 2, rg % 2, pl.ds(cp * 8, 8), :], bf16).astype(f32)
                        for p_ in range(2):
                            t = kv[8 * p_:8 * p_ + 8] * cols[8 * rg:8 * rg + 8]
                            key = (cp, 4 * p_ + rg // RH)
                            prev = (cp - VGRP, key[1])
                            if key in sacc:
                                sacc[key] = sacc[key] + t
                            elif CUMQ and prev in sacc:
                                sacc[key] = sacc[prev] + t
                            else:
                                sacc[key] = t
                for cp in range(NCP - NVQ, NCP):
                    a_ = jnp.zeros((8, 128), f32)
                    for r_ in (0, 1, 4, 5):
                        z_ = sacc[cp, r_]
                        if CUMQ and (cp - VGRP, r_) in sacc:
                            z_ = z_ - sacc[cp - VGRP, r_]
                        a_ = jnp.where(row == r_, _sublane_sum(z_), a_)
                    svq[cp - (NCP - NVQ), 0] = a_

            for j in range(NJ):
                build_l(qr2, lp, j)
            if VFIRST:
                vpu_qk()
            for n in range(CA * NT):
                qk_tile(kpair(0), lp, slo0, 0, n)
            for n in range((CB - nvq) * NT):
                qk_tile(kpair(0), lp, shi0, CA, n, CB - nvq)
            if not VFIRST:
                vpu_qk()
            for j in range(NJ):
                build_l(qr3, ln1, j)
            for n in range(CA * NT):
                qk_tile(kpair(1), ln1, slo1, 0, n)
            if not Q2EARLY:
                for n in range(NW):
                    qproj_tile(wqpair(2), qr0, n)
            softmax(slo0, shi0, pb0, ls0, None, None, None, svq if nvq else None)

            wp = lambda a: 1 - a if WLAG == 1 else a

            def kinds(a):
                b = 1 - a
                return dict(
                    h=(CB * NT, lambda z: kpair(z + 1),
                       lambda w, n: qk_tile(w, ln[b], shi[b], CA, n)),
                    l=(CA * NT, lambda z: kpair(z + 2),
                       lambda w, n: qk_tile(w, ln[a], slo[a], 0, n)),
                    q=(NW, lambda z: wqpair(jnp.minimum(z + 3, NP - 1)),
                       lambda w, n: qproj_tile(w, qr[b], n)),
                    w=(NW, lambda z: wopair(jnp.maximum(z - WLAG, 0)),
                       lambda w, n: wo_tile(w, ol[wp(a)], yr[wp(a)], n)),
                    v=(2 * KD, lambda z: wopair(z - 1),
                       lambda w, n: wo_tile(w, ol[b], yr[b], KD + n)),
                    u=(NW, lambda z: wopair(z - 1),
                       lambda w, n: wo_tile(w, ol1, qr1, n)),
                    m=(CM * NT, lambda z: kpair(z + 2),
                       lambda w, n: qk_tile(w, ln[a], smid, CA, n, CM)),
                    g=((CB - CM) * NT, lambda z: kpair(z + 1),
                       lambda w, n: qk_tile(w, ln[b], shi[b], CA + CM, n, CB - CM)),
                    x=(4 * NCP, lambda z: vx.at[pl.ds((z - (NP - 1)) * 16, 16)], x_tile))

            def block(i, a, order=MORD, RATE=RATE, SETS=SETS, PACE=PACE):
                b = 1 - a
                steps = softmax_steps(slo[b], shi[b], pb[b], ls[b], None, tbl[i] - i if SSPILL == 2 else None)
                if STAGED:
                    pos = [GPOS] * XA + [MOFF + int(24 * (k_ + 1) * RATE) + GLAG for k_ in range(4 - XA)]
                    pos += [pos[-1] + 1, pos[-1] + ELAG]
                else:
                    pos = [max(SPOS, MOFF + int(CB * NT * RATE) + 1)] * len(steps)
                side = list(zip(pos, steps))
                side += [(IPOS, P(l_inv, ls[a], li[a])),
                         (YPOS, P(y_fold, yr[1 - wp(a)]))]
                for j in range(NJ):
                    side.append((LPOS + LSTEP * j, P(build_l, qr[a], ln[a], j)))
                    side.append((RPOS + RSTEP * j, P(reduce_o, ac[b], li[b], ol[b], j)))
                run_block(first, i, a, 0, SETS, kinds(a), order, RATE, PACE, side, MOFF)

            def block14(i):
                side = [(int((CB - CM) * NT * RATE14) + SL14, P(softmax, slo1, shi1, pb1, ls1, pk1, None, smid)),
                        (IPOS14, P(l_inv, ls0, li0)),
                        (KPOS, P(pack_p, pb0, pk0)),
                        (YP14, P(y_fold, yr[1 - wp(0)]))]
                for j in range(NJ):
                    side.append((RP14 + RS14 * j, P(reduce_o, ac1, li1, ol1, j)))
                run_block(first, i, 0, 16, SETS14, kinds(0), ORD14, RATE14, PACE14, side)

            cin = set()

            def col_sum(rg):
                cin.add(rg)
                ac0[rg - 16] = jnp.broadcast_to(jnp.sum(ac1[rg], axis=1, keepdims=True), (8, 128))

            def block15(i):
                side = [(IPOS15, P(l_inv, ls1, li1)),
                        (YP15, P(y_fold, yr[1 - wp(1)]))]
                if "u" in ORD14:
                    side.append((YP15 + 20, P(y_fold, qr1)))
                for j in range(1, NJ):
                    side.append((RP15 + RS15 * j, P(reduce_o, ac0, li0, ol0, j)))
                if RIN15 >= 1:
                    side.append((16 * NCP + 1, P(reduce_o, ac1, li1, ol1, 1)))
                if RIN15 >= 2:
                    side.append((32 * NCP + 1, P(reduce_o, ac1, li1, ol1, 2)))
                run_block(first, i, 1, 16, SETS15, kinds(1), ORD15, RATE15, PACE15, side, 0, col_sum)

            def arrive(ch):
                for c in chunk(ch) + vstage(ch):
                    c.wait()
                for c in vstage(ch + 1):
                    c.start()

            def body(ch, one):
                if first:
                    arrive(ch)

                    @pl.when(ch + 2 < NC - 1)
                    def _():
                        for c in chunk(ch + 2):
                            c.start()

                    @pl.when(ch + 2 == NC - 1)
                    def _():
                        for c in vlast:
                            c.start()

                pl.when(one < 2)(P(block, 2 * ch, 0))
                pl.when(one > 0)(P(block, 2 * ch + 1, 1))
                return one

            one = lax.fori_loop(0, NC - 2, body, tbl[1])
            if first:
                arrive(NC - 2)
                for c in c1 + c2all:
                    c.start()
            block(one * (NP - 4), 0)
            pl.when(one > 0)(P(block, one * (NP - 3), 1, MORD13, RATE13, SETS13, PACE13))
            if first:
                for c in vlast + vstage(NC - 1):
                    c.wait()
            block14(one * (NP - 2))
            pl.when(one > 0)(P(block15, one * (NP - 1)))

            ox = [x_finish(0), x_finish(1)]
            for n in (list(range(KD, NW)) if "v" not in ORD15 else []) + list(range(KD)):
                wo_tile(wopair(NP - 2), ol0, yr0, n)
            for n in range(KD):
                wo_tile(wopair(NP - 1), ol1, qr0, n)
            wl = wopair(NP - 1)
            yv, mv = {}, {}
            for m in range(8, RH):
                c0, c1_ = [ac0[rg - 16] if rg in cin else jnp.sum(ac1[rg], axis=1, keepdims=True)
                           for rg in (2 * m, 2 * m + 1)]
                hh = 2 * m // RH
                for nt in range(KD):
                    w = pltpu.bitcast(wl[nt, pl.ds(8 * m, 8), :], bf16).astype(f32)
                    t = w[:8] * c0 + w[8:] * c1_
                    yv[hh, nt] = t if (hh, nt) not in yv else yv[hh, nt] + t
                t = wsc[2 * m - 16] * c0 + wsc[2 * m - 15] * c1_
                mv[hh] = t if hh not in mv else mv[hh] + t
            early = [_tree_sum([ysum[nt]] + [yr1[j * KD + nt] for j in range(NJ) if "u" not in ORD14]
                               + [yr0[j * KD + nt] for j in range(1, NJ)]) for nt in range(KD)]
            ys = [_tree_sum([early[nt], yr0[nt], qr0[nt],
                             yv[0, nt] * li1[0:1, :], yv[1, nt] * li1[1:2, :]]) for nt in range(KD)]
            y = jnp.sum(jnp.concatenate(ys, axis=1), axis=0, keepdims=True)
            lanes = _tree_sum(early + [x[:, nt * 128:(nt + 1) * 128] * 0.125 for nt in range(KD)]
                              + [ox[0] * wsl[0], ox[1] * wsl[1]])
            tot = (jnp.sum(lanes, axis=1, keepdims=True)
                   + mv[0] * li1[0:1, :] + mv[1] * li1[1:2, :])
            mean = jnp.concatenate([_sublane_sum(tot) * (1.0 / D)] * KD, axis=1)
            x = x + y

            xc, rs = _center(x, mean)
            xn = _pack_rows(xc)
            if first:
                for c in c1:
                    c.wait()
            nv = 0 if first else NV2
            gs = {}
            nv1 = 0 if first else NV1
            for n in range(KF - nv1):
                h = _tree_sum(_tile_dot(xn[:, kt * 128:(kt + 1) * 128], w1b[n, pl.ds(kt * 64, 64), :])
                              for kt in range(KD))
                gs[n] = _gelu(h * rs + b1v[n:n + 1, :].astype(f32))
            hacc = {}
            for kt in range(KD if nv1 else 0):
                col = _columns(xc[:, kt * 128:(kt + 1) * 128])
                for v in range(8):
                    for n in range(KF - nv1, KF):
                        w = pltpu.bitcast(w1b[n, pl.ds(kt * 64 + 8 * v, 8), :], bf16).astype(f32)
                        t = w[:8] * col[16 * v:16 * v + 8] + w[8:] * col[16 * v + 8:16 * v + 16]
                        hacc[n] = t if n not in hacc else hacc[n] + t
            for n in hacc:
                gs[n] = _gelu(_sublane_sum(hacc[n]) * rs + b1v[n:n + 1, :].astype(f32))
            vacc = [None] * KD
            for kt in range(nv):
                col = _columns(gs[kt])
                for v in range(8):
                    for nt in range(KD):
                        w = pltpu.bitcast(w2b[nt, pl.ds(kt * 64 + 8 * v, 8), :], bf16).astype(f32)
                        t = w[:8] * col[16 * v:16 * v + 8] + w[8:] * col[16 * v + 8:16 * v + 16]
                        vacc[nt] = t if vacc[nt] is None else vacc[nt] + t
            parts = []
            for kt in range(nv, KF):
                if first and kt in w2_split:
                    for c in c2[w2_split.index(kt)]:
                        c.wait()
                hk = _pack_rows(gs[kt])
                parts.append([_tile_dot(hk, w2b[nt, pl.ds(kt * 64, 64), :]) for nt in range(KD)])
            y2 = jnp.concatenate(
                [_tree_sum([p[nt] for p in parts] + [b2v[nt:nt + 1, :].astype(f32)]
                           + ([_sublane_sum(vacc[nt])] if nv else []))
                 for nt in range(KD)], axis=1)
            return x + y2

        for c in head:
            c.wait()

        def wo_rowsums(r0):
            w = _tree_sum(pltpu.bitcast(wob[nt, pl.ds(r0, 8), :], bf16).astype(f32) for nt in range(KD))
            return jnp.broadcast_to(jnp.sum(w, axis=1, keepdims=True), (16, 128))

        for m in range(8, RH):
            wsc[pl.ds(2 * m - 16, 2)] = wo_rowsums((NP - 1) * (PD // 2) + 8 * m).reshape(2, 8, 128)
        for s_ in range(2):
            cols = jnp.concatenate([wo_rowsums((NP - 2 + s_) * (PD // 2) + 8 * m) for m in range(8)], axis=0)
            wsl[s_] = cols.T[0:8]

        def transpose_tile(n, c):
            s8 = pl.multiple_of((n // (2 * NCP)) * 8, 8)
            e = n % 2
            c8 = pl.multiple_of(((n // 2) % NCP) * 8, 8)
            w = vx[pl.ds(s8, 8), e, pl.ds(c8, 8), :].reshape(64, 128)
            wt = pltpu.bitcast(w, bf16).astype(f32).T.astype(bf16)
            vx[pl.ds(s8, 8), e, pl.ds(c8, 8), :] = pltpu.bitcast(wt, u32).reshape(8, 8, 128)
            return c

        lax.fori_loop(0, 4 * NCP, transpose_tile, 0)

        if ONLY2:
            for c in chunk(0) + vstage(0) + chunk(1):
                c.wait()
        x = jnp.broadcast_to(xin[0].astype(f32), (8, D))
        for l_ in range(1 if ONLY2 else NL):
            x = layer(x, l_ == 0 and not ONLY2)
        o_ref[0] = x[0:1, :].astype(o_ref.dtype)

    return kernel


@jax.jit
def pallas_interleave_layers__sliding_block_cached__dense_activation_gelu__decode_kernel(
    A_x, A_k_cache, A_v_cache, A_wq, A_wo, B_x, B_w1, B_b1, B_w2, B_b2,
):
    SK = A_k_cache.shape[2]
    W = min(4096, max(256, SK // 4))
    NR = H * DH // 8

    def tiled(a):
        t = jnp.swapaxes(a, 2, 3).reshape(NR, 8, SK // 128, 128)
        return t.transpose(0, 2, 1, 3).reshape(NR // 2, 2, SK // 16, 128)

    b1 = B_b1.reshape(F // 128, 128)
    b2 = B_b2.reshape(D // 128, 128)
    anyspec = pl.BlockSpec(memory_space=pl.ANY)
    NCP = W // 256
    vreg = lambda n, dt: pltpu.VMEM(n + (8, 128), dt)
    return pl.pallas_call(
        _make_kernel(SK, W),
        out_shape=jax.ShapeDtypeStruct(A_x.shape, A_x.dtype),
        in_specs=[anyspec] * 9,
        out_specs=pl.BlockSpec(memory_space=pltpu.VMEM),
        scratch_shapes=[
            pltpu.VMEM((NR // 2, 2, W // 32, 128), u32),
            pltpu.VMEM((NR // 2 - 16 - NP * RF // 2, 2, W // 16, 128), bf16),
            pltpu.VMEM((2 * RF, 2, W // 16, 128), bf16),
            pltpu.VMEM((16, 2, W // 32, 128), u32),
            vreg((NP * max(RF, 1), 2 * NCP), f32),
            pltpu.VMEM((H * DH // 128, D // 2, 128), u32),
            pltpu.VMEM((KD, H * DH // 2, 128), u32),
            pltpu.VMEM((KF, D // 2, 128), u32),
            pltpu.VMEM((KD, F // 2, 128), u32),
            pltpu.VMEM((1, 1, D), bf16),
            pltpu.VMEM((KF, 128), bf16),
            pltpu.VMEM((KD, 128), bf16),
            pltpu.VMEM((8, D), u32),
            pltpu.VMEM((8, 128), f32),
            vreg((KD,), f32),
            vreg((NCP if SSPILL else 1,), f32),
        ] + [vreg((NT,), u32)] * 3
          + [vreg((NW,), f32)] * 4
          + [vreg((4 * XA, NT), f32)] * 2
          + [vreg((CM, NT), f32)]
          + [vreg((NCP - 4 * XA, NT), f32)] * 2
          + [pltpu.VMEM((8, NCP * 128), f32)] * 2
          + [pltpu.VMEM((8, 128), f32)] * 4
          + [vreg((RP,), f32)] * 2
          + [vreg((NJ,), u32)] * 2
          + [vreg((NW,), f32)] * 2
          + [vreg((NCP,), u32)] * 2
          + [vreg((32,), f32), vreg((2,), f32)]
          + [vreg((max(NVQ, 1), 1), f32)]
          + [pltpu.SMEM((NP,), jnp.int32)]
          + [pltpu.SemaphoreType.DMA((5,))],
        compiler_params=pltpu.CompilerParams(vmem_limit_bytes=128 * 1024 * 1024,
                                             disable_semaphore_checks=bool(NOSEM)),
    )(A_x, tiled(A_k_cache), tiled(A_v_cache), A_wq, A_wo, B_w1, b1, B_w2, b2)
```

```python
import functools
import jax
import jax.numpy as jnp
from jax import lax
import jax.experimental.pallas as pl
import jax.experimental.pallas.tpu as pltpu

D = 640
H = 32
DH = 192
F = 1536
NP = H // 2
PD = 2 * DH
RH = DH // 8
RP = 2 * RH
NJ = PD // 128
NT = 2 * NJ
KD = D // 128
KF = F // 128
NW = NJ * KD
EPS = 1e-5
LOG2E = 1.4426950408889634
bf16 = jnp.bfloat16
f32 = jnp.float32
u32 = jnp.uint32

RATE = 6.0
SPOS = 450
LPOS = 100
RPOS = 300
RSTEP = 80
YPOS = 5
IPOS = 150
IPOS14 = 10
IPOS15 = 10
SETS13 = "6,6,6,6,6,18"
CM = 2
RIN15 = 0
NV2 = 5
NV1 = 3
CIN = 0
ONEPASS = 0
NVQ = 6
VFIRST = 0
VGRP = 2
QRND = 1
CUMQ = 1
SL14 = 10
KPOS = 100
YP14 = 5
YP15 = 5
RS15 = 10
MORD13 = "hwlm"
RATE13 = 6.1
CPOS = 200
NL = 2
MORD = "hwql"
SSPILL = 0
PACE = 6
PACE13 = 3
D0 = 1
XA = 1
SETS = "10,10,10,18"
SETS14 = "8,8,8,8"
SETS15 = "8,8,10,6"
RATE14 = 5.6
RATE15 = 6.2
PACE14 = 3
PACE15 = 3
ONLY2 = 0
NOSEM = 0
STAGED = 0
GPOS = 30
GLAG = 60
ELAG = 80
MOFF = 0
LSTEP = 10
WOSTEP = 256
W2STEP = 192
W2SPLIT = "0,9,11,12"
RF = 8
F0 = 15
RP14 = 100
RP15 = 100
RS14 = 10
ORD14 = "gwu"
WLAG = 2
ORD15 = "xv"
Q2EARLY = 1


def _center(x, mean=None):
    if mean is not None:
        xc = x - mean
        v = jnp.mean(xc * xc, axis=-1, keepdims=True)
        return xc, lax.rsqrt(v + EPS)
    if ONEPASS:
        m = jnp.mean(x, axis=-1, keepdims=True)
        v = jnp.maximum(jnp.mean(x * x, axis=-1, keepdims=True) - m * m, 0.0)
        return x - m, lax.rsqrt(v + EPS)
    xc = x - jnp.mean(x, axis=-1, keepdims=True)
    v = jnp.mean(xc * xc, axis=-1, keepdims=True)
    return xc, lax.rsqrt(v + EPS)


def _gelu(x):
    c = 0.7978845608028654
    return 0.5 * x * (1.0 + jnp.tanh(c * (x + 0.044715 * (x * x * x))))


def _pack_rows(x8):
    x16 = jnp.concatenate([x8, x8], axis=0).astype(bf16)
    return pltpu.bitcast(x16, u32)


def _tile_dot(lhs_u32, w_u32):
    return jnp.dot(pltpu.bitcast(lhs_u32, bf16), pltpu.bitcast(w_u32, bf16),
                   preferred_element_type=f32)[0:8]


def _columns(x8):
    return jnp.concatenate([x8] * 16, axis=0).T


def _sublane_sum(x8):
    for sh in (4, 2, 1):
        x8 = x8 + pltpu.roll(x8, sh, 0)
    return x8


def _tree(op, xs):
    xs = list(xs)
    while len(xs) > 1:
        xs = [op(xs[i], xs[i + 1]) if i + 1 < len(xs) else xs[i] for i in range(0, len(xs), 2)]
    return xs[0]


def _tree_sum(xs):
    return _tree(jnp.add, xs)


def _make_kernel(SK, W):
    NCP = W // 256
    CA = 4 * XA
    CB = NCP - CA
    c_exp = (DH ** -0.5) * LOG2E
    P = functools.partial

    def kernel(x_hbm, k_hbm, v_hbm, wq_hbm, wo_hbm, w1_hbm, b1_hbm, w2_hbm, b2_hbm,
               o_ref,
               kb, vb, vs, vx, vf, wqb, wob, w1b, w2b, xin, b1v, b2v, xl, rs_ref, ysum, ssum,
               ln0, ln1, lp, qr0, qr1, qr2, qr3, slo0, slo1, smid, shi0, shi1, pb0, pb1,
               ls0, ls1, li0, li1, ac0, ac1, ol0, ol1, yr0, yr1, pk0, pk1, wsc, wsl, svq, tbl, sems):
        ln, qr, slo, shi = (ln0, ln1), (qr0, qr1), (slo0, slo1), (shi0, shi1)
        pb, ls, li, ac, ol, yr = (pb0, pb1), (ls0, ls1), (li0, li1), (ac0, ac1), (ol0, ol1), (yr0, yr1)
        pk = (pk0, pk1)
        ku = k_hbm.bitcast(u32)
        vu = v_hbm.bitcast(u32)
        NC = NP // 2

        def kcopy(c, s):
            return pltpu.make_async_copy(
                ku.at[pl.ds(c * RP, RP), :, pl.ds((SK - W) // 32, W // 32), :],
                kb.at[pl.ds(c * RP, RP)], sems.at[s])

        RM = RH - RF // 2

        def vcopy(src0, n, dst, dst0, s):
            return pltpu.make_async_copy(
                v_hbm.at[pl.ds(src0, n), :, pl.ds((SK - W) // 16, W // 16), :],
                dst.at[pl.ds(dst0, n)], sems.at[s])

        def vstage(c):
            return [vcopy((2 * c + p) * RH + RM, RF // 2, vs, ((2 * c + p) & 3) * (RF // 2), 1 + (c & 1))
                    for p in range(2)]

        def wcopies(src, dst, s, r0=0, nrows=None, step=None):
            su = src.bitcast(u32)
            nrows = dst.shape[1] if nrows is None else nrows
            step = nrows if step is None else step
            return [pltpu.make_async_copy(su.at[pl.ds(r, step), pl.ds(n * 128, 128)],
                                          dst.at[n, pl.ds(r, step)], sems.at[s])
                    for r in range(r0, r0 + nrows, step) for n in range(dst.shape[0])]

        head = [pltpu.make_async_copy(x_hbm, xin, sems.at[0]),
                pltpu.make_async_copy(b1_hbm, b1v, sems.at[0]),
                pltpu.make_async_copy(b2_hbm, b2v, sems.at[0])]
        head += [pltpu.make_async_copy(
            vu.at[pl.ds((NP - 2 + s) * RH, 8), :, pl.ds((SK - W) // 32, W // 32), :],
            vx.at[pl.ds(8 * s, 8)], sems.at[0]) for s in range(2)]
        head += wcopies(wq_hbm, wqb, 0) + wcopies(wo_hbm, wob, 0, step=WOSTEP) + [kcopy(0, 0)]
        vlast = [vcopy((NP - 2 + s) * RH + 8, RM - 8, vb, (NP - 2) * RM + s * (RM - 8), 2) for s in range(2)]
        c1 = wcopies(w1_hbm, w1b, 1)
        w2_split = tuple(int(z) for z in W2SPLIT.split(','))
        c2 = [wcopies(w2_hbm, w2b, (0, 3, 4)[g], 64 * w2_split[g],
                      64 * (w2_split[g + 1] - w2_split[g]),
                      min(W2STEP, 64 * (w2_split[g + 1] - w2_split[g]))) for g in range(len(w2_split) - 1)]
        c2all = [c for g in c2 for c in g]
        for c in head:
            c.start()

        def chunk(c):
            s = 1 + (c & 1)
            return [kcopy(c + 1, s)] + [vcopy((2 * c + p) * RH, RM, vb, (2 * c + p) * RM, s) for p in range(2)]

        for c in chunk(0) + vstage(0) + chunk(1):
            c.start()

        for i_ in range(NP):
            tbl[i_] = i_

        def qproj_tile(wg, dst, n):
            j, kt = divmod(n, KD)
            dst[n] = _tile_dot(xl[:, pl.ds(kt * 128, 128)], wg[j, pl.ds(kt * 64, 64), :])

        def build_l(src, dst, j):
            row = lax.broadcasted_iota(jnp.int32, (8, 128), 0)
            lane = lax.broadcasted_iota(jnp.int32, (8, 128), 1)
            q = _tree_sum(src[j * KD + kt] for kt in range(KD)) * rs_ref[...]
            qp = pltpu.roll(q, 8, 1)
            qm = pltpu.roll(q, 120, 1)
            tgt = (lane >> 1) & 4
            if j == 1:
                tgt = tgt + (lane >> 6)
            elif j == 2:
                tgt = tgt + 1
            hit = row == tgt
            low = row < 4
            dst[2 * j] = _pack_rows(jnp.where(hit, jnp.where(low, q, qp), 0.0))
            dst[2 * j + 1] = _pack_rows(jnp.where(hit, jnp.where(low, qm, q), 0.0))

        def qk_tile(kg, lsrc, sdst, c0, n, ncp=NCP):
            c4, rem = divmod(n, 4 * NT)
            t, i = divmod(rem, min(4, ncp - c4 * 4))
            c = c4 * 4 + i
            w = kg[pl.ds((t // 2) * 8, 8), t % 2, pl.ds((c0 + c) * 8, 8), :].reshape(64, 128)
            sdst[c, t] = _tile_dot(lsrc[t], w)

        def s_group(st, src, c0, c1):
            s = [_tree_sum(src[c, t] for t in range(src.shape[1])) for c in range(c0, c1)]
            base = len(st.setdefault("s", []))
            if SSPILL:
                for k_, a_ in enumerate(s):
                    ssum[st.get("zero", 0) + base + k_] = a_
            st["s"] += s
            st["m"] = _tree(jnp.maximum, s + ([st["m"]] if "m" in st else []))

        def s_max(st):
            m = jnp.maximum(st["m"], pltpu.roll(st["m"], 4, 0))
            st["m"] = jnp.max(m, axis=1, keepdims=True)

        def s_exp(st, pdst, ldst, kdst=None):
            s = [ssum[cp] for cp in range(NCP)] if SSPILL else st["s"]
            e = [jnp.exp2(a - st["m"]) for a in s]
            for cp in range(NCP):
                pdst[:, pl.ds(cp * 128, 128)] = e[cp]
                if kdst is not None:
                    kdst[cp] = _pack_rows(e[cp])
            ldst[...] = _tree_sum(e)

        def softmax_steps(lo, hi, pdst, ldst, kdst=None, zero=None, mid=None, tail=None):
            st = {} if zero is None else {"zero": zero}
            srcs = [(lo, CA), (hi, CB)] if mid is None else [(lo, CA), (mid, CM), (hi, CB - CM)]
            if tail is not None:
                srcs = [(lo, CA), (hi, CB - NVQ), (tail, NVQ)]
            steps = [P(s_group, st, src, c0, min(c0 + 4, n)) for src, n in srcs for c0 in range(0, n, 4)]
            return steps + [P(s_max, st), P(s_exp, st, pdst, ldst, kdst)]

        def softmax(*args):
            for f in softmax_steps(*args):
                f()

        def l_inv(lsrc, ldst):
            l = lsrc[...]
            l = l + pltpu.roll(l, 4, 0)
            l = jnp.sum(l, axis=1, keepdims=True)
            ldst[...] = jnp.broadcast_to(1.0 / l, (8, 128))

        def pack_p(psrc, kdst):
            for cp in range(NCP):
                kdst[cp] = _pack_rows(psrc[:, pl.ds(cp * 128, 128)])

        def reduce_o(asrc, lsrc, odst, j):
            blk = asrc[pl.ds(j * 16, 16)].reshape(128, 128)
            t = blk.T.reshape(16, 8, 128)
            if j == 1:
                lane = lax.broadcasted_iota(jnp.int32, (1, 128), 1)
                r = jnp.where(lane < 64, lsrc[0:1, :], lsrc[1:2, :])
            else:
                r = lsrc[j // 2:j // 2 + 1, :]
            odst[j] = _pack_rows(_tree_sum(t[i] for i in range(16)) * r)

        def x_tile(vg, n):
            s, rem = divmod(n, 2 * NCP)
            cp, e = divmod(rem, 2)
            w = vg[pl.ds(8 * s, 8), e, pl.ds(cp * 8, 8), :].reshape(64, 128)
            shi0[divmod(n, NT)] = _tile_dot(pk[s][cp], w)

        def x_finish(s):
            row = lax.broadcasted_iota(jnp.int32, (8, 128), 0)
            lane = lax.broadcasted_iota(jnp.int32, (8, 128), 1)
            o0 = _tree_sum(shi0[divmod((s * NCP + cp) * 2, NT)] for cp in range(NCP))
            o1 = _tree_sum(shi0[divmod((s * NCP + cp) * 2 + 1, NT)] for cp in range(NCP))
            low = row < 4
            direct = jnp.where(low, o0, o1)
            moved = jnp.where(low, pltpu.roll(o1, 8, 1), pltpu.roll(o0, 120, 1))
            o = jnp.where(((lane >> 1) & 4) == (row & 4), direct, moved)
            o = jnp.where((row & 3) == 0, o, 0.0) * li[s][0:1, :]
            ol[s][0] = _pack_rows(o)
            return o

        def wo_tile(wg, osrc, ydst, n):
            j, nt = divmod(n, KD)
            ydst[n] = _tile_dot(osrc[j], wg[nt, pl.ds(j * 64, 64), :])

        def y_fold(ysrc):
            for nt in range(KD):
                ysum[nt] = _tree_sum([ysum[nt]] + [ysrc[j * KD + nt] for j in range(NJ)])

        def copy(src, dst):
            for i in range(src.shape[0]):
                dst[i] = src[i]

        def kpair(i):
            return kb.at[pl.ds(i * RH, RH)]

        def wqpair(i):
            return wqb.at[pl.ds(i * NJ, NJ)]

        def wopair(i):
            r0 = i * (PD // 2)
            if not isinstance(i, int):
                r0 = pl.multiple_of(r0, PD // 2)
            return wob.at[:, pl.ds(r0, PD // 2), :]

        def run_block(first, i, a, rg0, sets, kinds, order, rate, pace_n, side, moff=0, done=None):
            if rg0:
                vg = vb.at[pl.ds((NP - 2) * RM + a * (RM - 8), RM - 8)]
            else:
                vg = vb.at[pl.ds(i * RM, RM)]
            voff = rg0 // 2
            sg = vs.at[pl.ds((i & 3) * (RF // 2), RF // 2)]
            fg = vf.at[pl.ds(i * RF, RF)]
            plain, order_rg = list(range(rg0, RP - RF)), []
            n_all = RP - rg0
            f0 = min(F0, n_all - RF) * n_all // RP
            slots = {f0 + (k_ + 1) * (n_all - f0) // RF - 1 for k_ in range(RF)}
            nf = 0
            for pos_ in range(n_all):
                if pos_ in slots:
                    order_rg.append(RP - RF + nf)
                    nf += 1
                else:
                    order_rg.append(plain.pop(0))
            pace = dict(z=i, cnt=0, views={})

            def mxu_tile(key, n):
                if pace_n and pace["cnt"] % pace_n == 0:
                    z = pace["z"]
                    link = pace["cnt"] // pace_n
                    for _ in range(pace_n * 4 // 3 if link else D0):
                        z = tbl[z]
                    pace["z"] = z
                    pace["views"] = {}
                pace["cnt"] += 1
                if key not in pace["views"]:
                    pace["views"][key] = kinds[key][1](pace["z"])
                kinds[key][2](pace["views"][key], n)

            mxu = [P(mxu_tile, key, n) for key in order for n in range(kinds[key][0])]
            side = sorted(side + [(moff + int(n * rate), f) for n, f in enumerate(mxu)], key=lambda z: z[0])
            cnt = 0
            si = 0
            acc = {}
            sizes, ovl = sets.split(":") if ":" in sets else (sets, "0")
            groups = []
            for size in (int(z) for z in sizes.split(",")):
                groups.append(order_rg[:size])
                order_rg = order_rg[size:]
            step = NCP - int(ovl)
            seq = [(rgs, t - gi * step) for t in range((len(groups) - 1) * step + NCP)
                   for gi, rgs in enumerate(groups) if 0 <= t - gi * step < NCP]
            for rgs, cp in seq:
                mult = {hh: (pb[a][pl.ds(hh, 1), pl.ds(cp * 128, 128)],
                             pb[a][pl.ds(4 + hh, 1), pl.ds(cp * 128, 128)])
                        for hh in sorted({rg // RH for rg in rgs})}
                for rg in rgs:
                    while si < len(side) and side[si][0] <= cnt:
                        side[si][1]()
                        si += 1
                    cnt += 1
                    m0, m1 = mult[rg // RH]
                    r = rg - (RP - RF)
                    if r >= 0 and not first:
                        v0, v1 = fg[r, 2 * cp], fg[r, 2 * cp + 1]
                    else:
                        src = sg.at[r // 2, r % 2] if r >= 0 else vg.at[rg // 2 - voff, rg % 2]
                        v = src[pl.ds(cp * 16, 16), :].astype(f32)
                        v0, v1 = v[:8], v[8:]
                        if r >= 0:
                            fg[r, 2 * cp] = v0
                            fg[r, 2 * cp + 1] = v1
                    if rg not in acc:
                        acc[rg] = v0 * m0 + v1 * m1
                    else:
                        acc[rg] = acc[rg] + v0 * m0 + v1 * m1
                    if cp == NCP - 1:
                        ac[a][rg] = acc[rg]
                        if done is not None and cnt <= CIN * NCP:
                            done(rg)
            assert not order_rg
            for _, f in side[si:]:
                f()

        def layer(x, first):
            nvq = 0 if first else NVQ
            xc, rs = _center(x)
            xl[...] = _pack_rows(xc)
            rs_ref[...] = jnp.broadcast_to(rs * c_exp, (8, 128))
            ac1[...] = jnp.zeros(ac1.shape, f32)
            li1[...] = jnp.zeros(li1.shape, f32)
            if WLAG == 1:
                yr0[...] = jnp.zeros(yr0.shape, f32)
            else:
                ol0[...] = jnp.zeros(ol0.shape, u32)
                yr1[...] = jnp.zeros(yr1.shape, f32)
            ysum[...] = jnp.zeros(ysum.shape, f32)

            for i, dst in enumerate((qr2, qr3)):
                for n in range(NW):
                    qproj_tile(wqpair(i), dst, n)
            if Q2EARLY:
                for n in range(NW):
                    qproj_tile(wqpair(2), qr0, n)
            def vpu_qk():
                if not nvq:
                    return
                row = lax.broadcasted_iota(jnp.int32, (8, 128), 0)
                cols = jnp.concatenate(
                    [_columns((_tree_sum(qr2[j * KD + kt] for kt in range(KD)) * rs_ref[...])
                              .astype(bf16 if QRND else f32).astype(f32)) for j in range(NJ)], axis=0)
                sacc = {}
                for rg, cp in [(rg, cp) for c0_ in range(NCP - NVQ, NCP, VGRP) for rg in range(RP)
                               for cp in range(c0_, min(c0_ + VGRP, NCP))]:
                    if True:
                        kv = pltpu.bitcast(kb[rg // 2, rg % 2, pl.ds(cp * 8, 8), :], bf16).astype(f32)
                        for p_ in range(2):
                            t = kv[8 * p_:8 * p_ + 8] * cols[8 * rg:8 * rg + 8]
                            key = (cp, 4 * p_ + rg // RH)
                            prev = (cp - VGRP, key[1])
                            if key in sacc:
                                sacc[key] = sacc[key] + t
                            elif CUMQ and prev in sacc:
                                sacc[key] = sacc[prev] + t
                            else:
                                sacc[key] = t
                for cp in range(NCP - NVQ, NCP):
                    a_ = jnp.zeros((8, 128), f32)
                    for r_ in (0, 1, 4, 5):
                        z_ = sacc[cp, r_]
                        if CUMQ and (cp - VGRP, r_) in sacc:
                            z_ = z_ - sacc[cp - VGRP, r_]
                        a_ = jnp.where(row == r_, _sublane_sum(z_), a_)
                    svq[cp - (NCP - NVQ), 0] = a_

            for j in range(NJ):
                build_l(qr2, lp, j)
            if VFIRST:
                vpu_qk()
            for n in range(CA * NT):
                qk_tile(kpair(0), lp, slo0, 0, n)
            for n in range((CB - nvq) * NT):
                qk_tile(kpair(0), lp, shi0, CA, n, CB - nvq)
            if not VFIRST:
                vpu_qk()
            for j in range(NJ):
                build_l(qr3, ln1, j)
            for n in range(CA * NT):
                qk_tile(kpair(1), ln1, slo1, 0, n)
            if not Q2EARLY:
                for n in range(NW):
                    qproj_tile(wqpair(2), qr0, n)
            softmax(slo0, shi0, pb0, ls0, None, None, None, svq if nvq else None)

            wp = lambda a: 1 - a if WLAG == 1 else a

            def kinds(a):
                b = 1 - a
                return dict(
                    h=(CB * NT, lambda z: kpair(z + 1),
                       lambda w, n: qk_tile(w, ln[b], shi[b], CA, n)),
                    l=(CA * NT, lambda z: kpair(z + 2),
                       lambda w, n: qk_tile(w, ln[a], slo[a], 0, n)),
                    q=(NW, lambda z: wqpair(jnp.minimum(z + 3, NP - 1)),
                       lambda w, n: qproj_tile(w, qr[b], n)),
                    w=(NW, lambda z: wopair(jnp.maximum(z - WLAG, 0)),
                       lambda w, n: wo_tile(w, ol[wp(a)], yr[wp(a)], n)),
                    v=(2 * KD, lambda z: wopair(z - 1),
                       lambda w, n: wo_tile(w, ol[b], yr[b], KD + n)),
                    u=(NW, lambda z: wopair(z - 1),
                       lambda w, n: wo_tile(w, ol1, qr1, n)),
                    m=(CM * NT, lambda z: kpair(z + 2),
                       lambda w, n: qk_tile(w, ln[a], smid, CA, n, CM)),
                    g=((CB - CM) * NT, lambda z: kpair(z + 1),
                       lambda w, n: qk_tile(w, ln[b], shi[b], CA + CM, n, CB - CM)),
                    x=(4 * NCP, lambda z: vx.at[pl.ds((z - (NP - 1)) * 16, 16)], x_tile))

            def block(i, a, order=MORD, RATE=RATE, SETS=SETS, PACE=PACE):
                b = 1 - a
                steps = softmax_steps(slo[b], shi[b], pb[b], ls[b], None, tbl[i] - i if SSPILL == 2 else None)
                if STAGED:
                    pos = [GPOS] * XA + [MOFF + int(24 * (k_ + 1) * RATE) + GLAG for k_ in range(4 - XA)]
                    pos += [pos[-1] + 1, pos[-1] + ELAG]
                else:
                    pos = [max(SPOS, MOFF + int(CB * NT * RATE) + 1)] * len(steps)
                side = list(zip(pos, steps))
                side += [(IPOS, P(l_inv, ls[a], li[a])),
                         (YPOS, P(y_fold, yr[1 - wp(a)]))]
                for j in range(NJ):
                    side.append((LPOS + LSTEP * j, P(build_l, qr[a], ln[a], j)))
                    side.append((RPOS + RSTEP * j, P(reduce_o, ac[b], li[b], ol[b], j)))
                run_block(first, i, a, 0, SETS, kinds(a), order, RATE, PACE, side, MOFF)

            def block14(i):
                side = [(int((CB - CM) * NT * RATE14) + SL14, P(softmax, slo1, shi1, pb1, ls1, pk1, None, smid)),
                        (IPOS14, P(l_inv, ls0, li0)),
                        (KPOS, P(pack_p, pb0, pk0)),
                        (YP14, P(y_fold, yr[1 - wp(0)]))]
                for j in range(NJ):
                    side.append((RP14 + RS14 * j, P(reduce_o, ac1, li1, ol1, j)))
                run_block(first, i, 0, 16, SETS14, kinds(0), ORD14, RATE14, PACE14, side)

            cin = set()

            def col_sum(rg):
                cin.add(rg)
                ac0[rg - 16] = jnp.broadcast_to(jnp.sum(ac1[rg], axis=1, keepdims=True), (8, 128))

            def block15(i):
                side = [(IPOS15, P(l_inv, ls1, li1)),
                        (YP15, P(y_fold, yr[1 - wp(1)]))]
                if "u" in ORD14:
                    side.append((YP15 + 20, P(y_fold, qr1)))
                for j in range(1, NJ):
                    side.append((RP15 + RS15 * j, P(reduce_o, ac0, li0, ol0, j)))
                if RIN15 >= 1:
                    side.append((16 * NCP + 1, P(reduce_o, ac1, li1, ol1, 1)))
                if RIN15 >= 2:
                    side.append((32 * NCP + 1, P(reduce_o, ac1, li1, ol1, 2)))
                run_block(first, i, 1, 16, SETS15, kinds(1), ORD15, RATE15, PACE15, side, 0, col_sum)

            def arrive(ch):
                for c in chunk(ch) + vstage(ch):
                    c.wait()
                for c in vstage(ch + 1):
                    c.start()

            def body(ch, one):
                if first:
                    arrive(ch)

                    @pl.when(ch + 2 < NC - 1)
                    def _():
                        for c in chunk(ch + 2):
                            c.start()

                    @pl.when(ch + 2 == NC - 1)
                    def _():
                        for c in vlast:
                            c.start()

                pl.when(one < 2)(P(block, 2 * ch, 0))
                pl.when(one > 0)(P(block, 2 * ch + 1, 1))
                return one

            one = lax.fori_loop(0, NC - 2, body, tbl[1])
            if first:
                arrive(NC - 2)
                for c in c1 + c2all:
                    c.start()
            block(one * (NP - 4), 0)
            pl.when(one > 0)(P(block, one * (NP - 3), 1, MORD13, RATE13, SETS13, PACE13))
            if first:
                for c in vlast + vstage(NC - 1):
                    c.wait()
            block14(one * (NP - 2))
            pl.when(one > 0)(P(block15, one * (NP - 1)))

            ox = [x_finish(0), x_finish(1)]
            for n in (list(range(KD, NW)) if "v" not in ORD15 else []) + list(range(KD)):
                wo_tile(wopair(NP - 2), ol0, yr0, n)
            for n in range(KD):
                wo_tile(wopair(NP - 1), ol1, qr0, n)
            wl = wopair(NP - 1)
            yv, mv = {}, {}
            for m in range(8, RH):
                c0, c1_ = [ac0[rg - 16] if rg in cin else jnp.sum(ac1[rg], axis=1, keepdims=True)
                           for rg in (2 * m, 2 * m + 1)]
                hh = 2 * m // RH
                for nt in range(KD):
                    w = pltpu.bitcast(wl[nt, pl.ds(8 * m, 8), :], bf16).astype(f32)
                    t = w[:8] * c0 + w[8:] * c1_
                    yv[hh, nt] = t if (hh, nt) not in yv else yv[hh, nt] + t
                t = wsc[2 * m - 16] * c0 + wsc[2 * m - 15] * c1_
                mv[hh] = t if hh not in mv else mv[hh] + t
            early = [_tree_sum([ysum[nt]] + [yr1[j * KD + nt] for j in range(NJ) if "u" not in ORD14]
                               + [yr0[j * KD + nt] for j in range(1, NJ)]) for nt in range(KD)]
            ys = [_tree_sum([early[nt], yr0[nt], qr0[nt],
                             yv[0, nt] * li1[0:1, :], yv[1, nt] * li1[1:2, :]]) for nt in range(KD)]
            y = jnp.sum(jnp.concatenate(ys, axis=1), axis=0, keepdims=True)
            lanes = _tree_sum(early + [x[:, nt * 128:(nt + 1) * 128] * 0.125 for nt in range(KD)]
                              + [ox[0] * wsl[0], ox[1] * wsl[1]])
            tot = (jnp.sum(lanes, axis=1, keepdims=True)
                   + mv[0] * li1[0:1, :] + mv[1] * li1[1:2, :])
            mean = jnp.concatenate([_sublane_sum(tot) * (1.0 / D)] * KD, axis=1)
            x = x + y

            xc, rs = _center(x, mean)
            xn = _pack_rows(xc)
            if first:
                for c in c1:
                    c.wait()
            nv = 0 if first else NV2
            gs = {}
            nv1 = 0 if first else NV1
            for n in range(KF - nv1):
                h = _tree_sum(_tile_dot(xn[:, kt * 128:(kt + 1) * 128], w1b[n, pl.ds(kt * 64, 64), :])
                              for kt in range(KD))
                gs[n] = _gelu(h * rs + b1v[n:n + 1, :].astype(f32))
            hacc = {}
            for kt in range(KD if nv1 else 0):
                col = _columns(xc[:, kt * 128:(kt + 1) * 128])
                for v in range(8):
                    for n in range(KF - nv1, KF):
                        w = pltpu.bitcast(w1b[n, pl.ds(kt * 64 + 8 * v, 8), :], bf16).astype(f32)
                        t = w[:8] * col[16 * v:16 * v + 8] + w[8:] * col[16 * v + 8:16 * v + 16]
                        hacc[n] = t if n not in hacc else hacc[n] + t
            for n in hacc:
                gs[n] = _gelu(_sublane_sum(hacc[n]) * rs + b1v[n:n + 1, :].astype(f32))
            vk = list(range(w2_split[1], KF)) if first else list(range(nv))
            cols = {kt: _columns(gs[kt]) for kt in vk}
            vacc = [None] * KD
            parts = []
            for kt in range(KF):
                if first and kt in w2_split:
                    for c in c2[w2_split.index(kt)]:
                        c.wait()
                if kt not in vk:
                    hk = _pack_rows(gs[kt])
                    parts.append([_tile_dot(hk, w2b[nt, pl.ds(kt * 64, 64), :]) for nt in range(KD)])
                    continue
                for v in range(8):
                    for nt in range(KD):
                        w = pltpu.bitcast(w2b[nt, pl.ds(kt * 64 + 8 * v, 8), :], bf16).astype(f32)
                        t = w[:8] * cols[kt][16 * v:16 * v + 8] + w[8:] * cols[kt][16 * v + 8:16 * v + 16]
                        vacc[nt] = t if vacc[nt] is None else vacc[nt] + t
            y2 = jnp.concatenate(
                [_tree_sum([p[nt] for p in parts] + [b2v[nt:nt + 1, :].astype(f32), _sublane_sum(vacc[nt])])
                 for nt in range(KD)], axis=1)
            return x + y2

        for c in head:
            c.wait()

        def wo_rowsums(r0):
            w = _tree_sum(pltpu.bitcast(wob[nt, pl.ds(r0, 8), :], bf16).astype(f32) for nt in range(KD))
            return jnp.broadcast_to(jnp.sum(w, axis=1, keepdims=True), (16, 128))

        for m in range(8, RH):
            wsc[pl.ds(2 * m - 16, 2)] = wo_rowsums((NP - 1) * (PD // 2) + 8 * m).reshape(2, 8, 128)
        for s_ in range(2):
            cols = jnp.concatenate([wo_rowsums((NP - 2 + s_) * (PD // 2) + 8 * m) for m in range(8)], axis=0)
            wsl[s_] = cols.T[0:8]

        def transpose_tile(n, c):
            s8 = pl.multiple_of((n // (2 * NCP)) * 8, 8)
            e = n % 2
            c8 = pl.multiple_of(((n // 2) % NCP) * 8, 8)
            w = vx[pl.ds(s8, 8), e, pl.ds(c8, 8), :].reshape(64, 128)
            wt = pltpu.bitcast(w, bf16).astype(f32).T.astype(bf16)
            vx[pl.ds(s8, 8), e, pl.ds(c8, 8), :] = pltpu.bitcast(wt, u32).reshape(8, 8, 128)
            return c

        lax.fori_loop(0, 4 * NCP, transpose_tile, 0)

        if ONLY2:
            for c in chunk(0) + vstage(0) + chunk(1):
                c.wait()
        x = jnp.broadcast_to(xin[0].astype(f32), (8, D))
        for l_ in range(1 if ONLY2 else NL):
            x = layer(x, l_ == 0 and not ONLY2)
        o_ref[0] = x[0:1, :].astype(o_ref.dtype)

    return kernel


@jax.jit
def pallas_interleave_layers__sliding_block_cached__dense_activation_gelu__decode_kernel(
    A_x, A_k_cache, A_v_cache, A_wq, A_wo, B_x, B_w1, B_b1, B_w2, B_b2,
):
    SK = A_k_cache.shape[2]
    W = min(4096, max(256, SK // 4))
    NR = H * DH // 8

    def tiled(a):
        t = jnp.swapaxes(a, 2, 3).reshape(NR, 8, SK // 128, 128)
        return t.transpose(0, 2, 1, 3).reshape(NR // 2, 2, SK // 16, 128)

    b1 = B_b1.reshape(F // 128, 128)
    b2 = B_b2.reshape(D // 128, 128)
    anyspec = pl.BlockSpec(memory_space=pl.ANY)
    NCP = W // 256
    vreg = lambda n, dt: pltpu.VMEM(n + (8, 128), dt)
    return pl.pallas_call(
        _make_kernel(SK, W),
        out_shape=jax.ShapeDtypeStruct(A_x.shape, A_x.dtype),
        in_specs=[anyspec] * 9,
        out_specs=pl.BlockSpec(memory_space=pltpu.VMEM),
        scratch_shapes=[
            pltpu.VMEM((NR // 2, 2, W // 32, 128), u32),
            pltpu.VMEM((NR // 2 - 16 - NP * RF // 2, 2, W // 16, 128), bf16),
            pltpu.VMEM((2 * RF, 2, W // 16, 128), bf16),
            pltpu.VMEM((16, 2, W // 32, 128), u32),
            vreg((NP * max(RF, 1), 2 * NCP), f32),
            pltpu.VMEM((H * DH // 128, D // 2, 128), u32),
            pltpu.VMEM((KD, H * DH // 2, 128), u32),
            pltpu.VMEM((KF, D // 2, 128), u32),
            pltpu.VMEM((KD, F // 2, 128), u32),
            pltpu.VMEM((1, 1, D), bf16),
            pltpu.VMEM((KF, 128), bf16),
            pltpu.VMEM((KD, 128), bf16),
            pltpu.VMEM((8, D), u32),
            pltpu.VMEM((8, 128), f32),
            vreg((KD,), f32),
            vreg((NCP if SSPILL else 1,), f32),
        ] + [vreg((NT,), u32)] * 3
          + [vreg((NW,), f32)] * 4
          + [vreg((4 * XA, NT), f32)] * 2
          + [vreg((CM, NT), f32)]
          + [vreg((NCP - 4 * XA, NT), f32)] * 2
          + [pltpu.VMEM((8, NCP * 128), f32)] * 2
          + [pltpu.VMEM((8, 128), f32)] * 4
          + [vreg((RP,), f32)] * 2
          + [vreg((NJ,), u32)] * 2
          + [vreg((NW,), f32)] * 2
          + [vreg((NCP,), u32)] * 2
          + [vreg((32,), f32), vreg((2,), f32)]
          + [vreg((max(NVQ, 1), 1), f32)]
          + [pltpu.SMEM((NP,), jnp.int32)]
          + [pltpu.SemaphoreType.DMA((5,))],
        compiler_params=pltpu.CompilerParams(vmem_limit_bytes=128 * 1024 * 1024,
                                             disable_semaphore_checks=bool(NOSEM)),
    )(A_x, tiled(A_k_cache), tiled(A_v_cache), A_wq, A_wo, B_w1, b1, B_w2, b2)
```

```python
import functools
import jax
import jax.numpy as jnp
from jax import lax
import jax.experimental.pallas as pl
import jax.experimental.pallas.tpu as pltpu

D = 640
H = 32
DH = 192
F = 1536
NP = H // 2
PD = 2 * DH
RH = DH // 8
RP = 2 * RH
NJ = PD // 128
NT = 2 * NJ
KD = D // 128
KF = F // 128
NW = NJ * KD
NC = NP // 2
EPS = 1e-5
LOG2E = 1.4426950408889634
bf16 = jnp.bfloat16
f32 = jnp.float32
u32 = jnp.uint32

RF = 8
CA = 4
CM = 2
NVQ = 6
NV1 = 3
NV2 = 5
WOSTEP = 256
W2STEP = 192
W2SPLIT = (0, 9, 11, KF)
F0 = 15
D0 = 1
RATE = 6.0
PACE = 6
SETS = "10,10,10,18"
MORD = "hwql"
SPOS = 450
LPOS = 100
RPOS = 300
RSTEP = 80
YPOS = 5
IPOS = 150
RATE13 = 6.1
PACE13 = 3
SETS13 = "8,8,8,8,16"
MORD13 = "hwlm"
RATE14 = 5.6
PACE14 = 3
SETS14 = "8,8,8,8"
RATE15 = 6.2
PACE15 = 3
SETS15 = "8,8,10,6"


def _center(x, mean=None):
    xc = x - (jnp.mean(x, axis=-1, keepdims=True) if mean is None else mean)
    v = jnp.mean(xc * xc, axis=-1, keepdims=True)
    return xc, lax.rsqrt(v + EPS)


def _gelu(x):
    c = 0.7978845608028654
    return 0.5 * x * (1.0 + jnp.tanh(c * (x + 0.044715 * (x * x * x))))


def _pack_rows(x8):
    return pltpu.bitcast(jnp.concatenate([x8, x8], axis=0).astype(bf16), u32)


def _tile_dot(lhs_u32, w_u32):
    return jnp.dot(pltpu.bitcast(lhs_u32, bf16), pltpu.bitcast(w_u32, bf16),
                   preferred_element_type=f32)[0:8]


def _widen(slab_u32):
    w = pltpu.bitcast(slab_u32, bf16).astype(f32)
    return w[:8], w[8:]


def _columns(x8):
    t = jnp.concatenate([x8] * 16, axis=0).T
    return [t[8 * v:8 * v + 8] for v in range(16)]


def _sublane_sum(x8):
    for sh in (4, 2, 1):
        x8 = x8 + pltpu.roll(x8, sh, 0)
    return x8


def _tree(op, xs):
    xs = list(xs)
    while len(xs) > 1:
        xs = [op(xs[i], xs[i + 1]) if i + 1 < len(xs) else xs[i] for i in range(0, len(xs), 2)]
    return xs[0]


def _tree_sum(xs):
    return _tree(jnp.add, xs)


def _accum(d, key, t):
    d[key] = d[key] + t if key in d else t


def _make_kernel(SK, W):
    NCP = W // 256
    CB = NCP - CA
    RM = RH - RF // 2
    c_exp = (DH ** -0.5) * LOG2E
    P = functools.partial

    def kernel(x_hbm, k_hbm, v_hbm, wq_hbm, wo_hbm, w1_hbm, b1_hbm, w2_hbm, b2_hbm,
               o_ref,
               kb, vb, vs, vx, vf, wqb, wob, w1b, w2b, xin, b1v, b2v, xl, rs_ref, ysum,
               ln0, ln1, lp, qr0, qr1, qr2, qr3, slo0, slo1, smid, shi0, shi1, pb0, pb1,
               ls0, ls1, li0, li1, ac0, ac1, ol0, ol1, yr0, yr1, pk0, pk1, wsc, wsl, svq,
               tbl, sems):
        ln, qr, slo, shi = (ln0, ln1), (qr0, qr1), (slo0, slo1), (shi0, shi1)
        pb, ls, li, ac, ol, yr = (pb0, pb1), (ls0, ls1), (li0, li1), (ac0, ac1), (ol0, ol1), (yr0, yr1)
        pk = (pk0, pk1)

        ku = k_hbm.bitcast(u32)
        vu = v_hbm.bitcast(u32)

        def kcopy(c, s):
            return pltpu.make_async_copy(
                ku.at[pl.ds(c * RP, RP), :, pl.ds((SK - W) // 32, W // 32), :],
                kb.at[pl.ds(c * RP, RP)], sems.at[s])

        def vcopy(src0, n, dst, dst0, s):
            return pltpu.make_async_copy(
                v_hbm.at[pl.ds(src0, n), :, pl.ds((SK - W) // 16, W // 16), :],
                dst.at[pl.ds(dst0, n)], sems.at[s])

        def chunk(c):
            s = 1 + (c & 1)
            return [kcopy(c + 1, s)] + [vcopy((2 * c + p) * RH, RM, vb, (2 * c + p) * RM, s)
                                        for p in range(2)]

        def vstage(c):
            return [vcopy((2 * c + p) * RH + RM, RF // 2, vs, ((2 * c + p) & 3) * (RF // 2), 1 + (c & 1))
                    for p in range(2)]

        def wcopies(src, dst, s, r0=0, nrows=None, step=None):
            su = src.bitcast(u32)
            nrows = dst.shape[1] if nrows is None else nrows
            step = nrows if step is None else min(step, nrows)
            return [pltpu.make_async_copy(su.at[pl.ds(r, step), pl.ds(n * 128, 128)],
                                          dst.at[n, pl.ds(r, step)], sems.at[s])
                    for r in range(r0, r0 + nrows, step) for n in range(dst.shape[0])]

        head = [pltpu.make_async_copy(x_hbm, xin, sems.at[0]),
                pltpu.make_async_copy(b1_hbm, b1v, sems.at[0]),
                pltpu.make_async_copy(b2_hbm, b2v, sems.at[0])]
        head += [pltpu.make_async_copy(
            vu.at[pl.ds((NP - 2 + s) * RH, 8), :, pl.ds((SK - W) // 32, W // 32), :],
            vx.at[pl.ds(8 * s, 8)], sems.at[0]) for s in range(2)]
        head += wcopies(wq_hbm, wqb, 0) + wcopies(wo_hbm, wob, 0, step=WOSTEP) + [kcopy(0, 0)]
        vlast = [vcopy((NP - 2 + s) * RH + 8, RM - 8, vb, (NP - 2) * RM + s * (RM - 8), 2)
                 for s in range(2)]
        c1 = wcopies(w1_hbm, w1b, 1)
        c2 = [wcopies(w2_hbm, w2b, (0, 3, 4)[g], 64 * W2SPLIT[g],
                      64 * (W2SPLIT[g + 1] - W2SPLIT[g]), W2STEP) for g in range(3)]
        for c in head + chunk(0) + vstage(0) + chunk(1):
            c.start()

        for i_ in range(NP):
            tbl[i_] = i_

        def qproj_tile(wg, dst, n):
            j, kt = divmod(n, KD)
            dst[n] = _tile_dot(xl[:, pl.ds(kt * 128, 128)], wg[j, pl.ds(kt * 64, 64), :])

        def q_tile(src, j):
            return _tree_sum(src[j * KD + kt] for kt in range(KD)) * rs_ref[...]

        def build_l(src, dst, j):
            row = lax.broadcasted_iota(jnp.int32, (8, 128), 0)
            lane = lax.broadcasted_iota(jnp.int32, (8, 128), 1)
            q = q_tile(src, j)
            qp = pltpu.roll(q, 8, 1)
            qm = pltpu.roll(q, 120, 1)
            tgt = (lane >> 1) & 4
            if j == 1:
                tgt = tgt + (lane >> 6)
            elif j == 2:
                tgt = tgt + 1
            hit = row == tgt
            low = row < 4
            dst[2 * j] = _pack_rows(jnp.where(hit, jnp.where(low, q, qp), 0.0))
            dst[2 * j + 1] = _pack_rows(jnp.where(hit, jnp.where(low, qm, q), 0.0))

        def qk_tile(kg, lsrc, sdst, c0, ncp, n):
            c4, rem = divmod(n, 4 * NT)
            t, i = divmod(rem, min(4, ncp - c4 * 4))
            c = c4 * 4 + i
            w = kg[pl.ds((t // 2) * 8, 8), t % 2, pl.ds((c0 + c) * 8, 8), :].reshape(64, 128)
            sdst[c, t] = _tile_dot(lsrc[t], w)

        def softmax(srcs, pdst, ldst, kdst=None):
            s, m = [], None
            for src, n in srcs:
                for c0 in range(0, n, 4):
                    g = [_tree_sum(src[c, t] for t in range(src.shape[1]))
                         for c in range(c0, min(c0 + 4, n))]
                    s += g
                    m = _tree(jnp.maximum, g + ([] if m is None else [m]))
            m = jnp.maximum(m, pltpu.roll(m, 4, 0))
            m = jnp.max(m, axis=1, keepdims=True)
            e = [jnp.exp2(a - m) for a in s]
            for cp in range(NCP):
                pdst[:, pl.ds(cp * 128, 128)] = e[cp]
                if kdst is not None:
                    kdst[cp] = _pack_rows(e[cp])
            ldst[...] = _tree_sum(e)

        def l_inv(lsrc, ldst):
            l = lsrc[...]
            l = l + pltpu.roll(l, 4, 0)
            l = jnp.sum(l, axis=1, keepdims=True)
            ldst[...] = jnp.broadcast_to(1.0 / l, (8, 128))

        def pack_p(psrc, kdst):
            for cp in range(NCP):
                kdst[cp] = _pack_rows(psrc[:, pl.ds(cp * 128, 128)])

        def reduce_o(asrc, lsrc, odst, j):
            t = asrc[pl.ds(j * 16, 16)].reshape(128, 128).T.reshape(16, 8, 128)
            if j == 1:
                lane = lax.broadcasted_iota(jnp.int32, (1, 128), 1)
                r = jnp.where(lane < 64, lsrc[0:1, :], lsrc[1:2, :])
            else:
                r = lsrc[j // 2:j // 2 + 1, :]
            odst[j] = _pack_rows(_tree_sum(t[i] for i in range(16)) * r)

        def x_tile(vg, n):
            s, rem = divmod(n, 2 * NCP)
            cp, e = divmod(rem, 2)
            w = vg[pl.ds(8 * s, 8), e, pl.ds(cp * 8, 8), :].reshape(64, 128)
            shi0[divmod(n, NT)] = _tile_dot(pk[s][cp], w)

        def x_finish(s):
            row = lax.broadcasted_iota(jnp.int32, (8, 128), 0)
            lane = lax.broadcasted_iota(jnp.int32, (8, 128), 1)
            o0, o1 = [_tree_sum(shi0[divmod((s * NCP + cp) * 2 + e, NT)] for cp in range(NCP))
                      for e in range(2)]
            low = row < 4
            direct = jnp.where(low, o0, o1)
            moved = jnp.where(low, pltpu.roll(o1, 8, 1), pltpu.roll(o0, 120, 1))
            o = jnp.where(((lane >> 1) & 4) == (row & 4), direct, moved)
            o = jnp.where((row & 3) == 0, o, 0.0) * li[s][0:1, :]
            ol[s][0] = _pack_rows(o)
            return o

        def wo_tile(wg, osrc, ydst, n):
            j, nt = divmod(n, KD)
            ydst[n] = _tile_dot(osrc[j], wg[nt, pl.ds(j * 64, 64), :])

        def y_fold(ysrc):
            for nt in range(KD):
                ysum[nt] = _tree_sum([ysum[nt]] + [ysrc[j * KD + nt] for j in range(NJ)])

        def kpair(i):
            return kb.at[pl.ds(i * RH, RH)]

        def wqpair(i):
            return wqb.at[pl.ds(i * NJ, NJ)]

        def wopair(i):
            r0 = i * (PD // 2)
            if not isinstance(i, int):
                r0 = pl.multiple_of(r0, PD // 2)
            return wob.at[:, pl.ds(r0, PD // 2), :]

        def mxu_kinds(a):
            b = 1 - a
            return dict(
                h=(CB * NT, lambda z: kpair(z + 1),
                   lambda w, n: qk_tile(w, ln[b], shi[b], CA, CB, n)),
                g=((CB - CM) * NT, lambda z: kpair(z + 1),
                   lambda w, n: qk_tile(w, ln[b], shi[b], CA + CM, CB - CM, n)),
                l=(CA * NT, lambda z: kpair(z + 2),
                   lambda w, n: qk_tile(w, ln[a], slo[a], 0, CA, n)),
                m=(CM * NT, lambda z: kpair(z + 2),
                   lambda w, n: qk_tile(w, ln[a], smid, CA, CM, n)),
                q=(NW, lambda z: wqpair(jnp.minimum(z + 3, NP - 1)),
                   lambda w, n: qproj_tile(w, qr[b], n)),
                w=(NW, lambda z: wopair(jnp.maximum(z - 2, 0)),
                   lambda w, n: wo_tile(w, ol[a], yr[a], n)),
                u=(NW, lambda z: wopair(z - 1),
                   lambda w, n: wo_tile(w, ol1, qr1, n)),
                v=(2 * KD, lambda z: wopair(z - 1),
                   lambda w, n: wo_tile(w, ol0, yr0, KD + n)),
                x=(4 * NCP, lambda z: vx.at[pl.ds((z - (NP - 1)) * 16, 16)], x_tile))

        def run_block(first, i, a, rg0, sets, order, rate, pace_n, side):
            if rg0:
                vg = vb.at[pl.ds((NP - 2) * RM + a * (RM - 8), RM - 8)]
            else:
                vg = vb.at[pl.ds(i * RM, RM)]
            sg = vs.at[pl.ds((i & 3) * (RF // 2), RF // 2)]
            fg = vf.at[pl.ds(i * RF, RF)]
            kinds = mxu_kinds(a)

            pace = dict(z=i, cnt=0, views={})

            def mxu_tile(key, n):
                if not first and pace["cnt"] % pace_n == 0:
                    for _ in range(pace_n * 4 // 3 if pace["cnt"] else D0):
                        pace["z"] = tbl[pace["z"]]
                    pace["views"] = {}
                pace["cnt"] += 1
                if key not in pace["views"]:
                    pace["views"][key] = kinds[key][1](pace["z"])
                kinds[key][2](pace["views"][key], n)

            mxu = [P(mxu_tile, key, n) for key in order for n in range(kinds[key][0])]
            side = sorted(side + [(int(n * rate), f) for n, f in enumerate(mxu)], key=lambda z: z[0])

            n_all = RP - rg0
            f0 = F0 * n_all // RP
            slots = sorted(f0 + (k + 1) * (n_all - f0) // RF - 1 for k in range(RF))
            todo = list(range(rg0, RP - RF))
            for k, pos in enumerate(slots):
                todo.insert(pos, RP - RF + k)
            cnt = 0
            acc = {}
            for size in (int(z) for z in sets.split(",")):
                rgs, todo = todo[:size], todo[size:]
                for cp in range(NCP):
                    mult = {hh: (pb[a][pl.ds(hh, 1), pl.ds(cp * 128, 128)],
                                 pb[a][pl.ds(4 + hh, 1), pl.ds(cp * 128, 128)])
                            for hh in sorted({rg // RH for rg in rgs})}
                    for rg in rgs:
                        while side and side[0][0] <= cnt:
                            side.pop(0)[1]()
                        cnt += 1
                        m0, m1 = mult[rg // RH]
                        r = rg - (RP - RF)
                        if r >= 0 and not first:
                            v0, v1 = fg[r, 2 * cp], fg[r, 2 * cp + 1]
                        else:
                            src = sg.at[r // 2, r % 2] if r >= 0 else vg.at[(rg - rg0) // 2, rg % 2]
                            v = src[pl.ds(cp * 16, 16), :].astype(f32)
                            v0, v1 = v[:8], v[8:]
                            if r >= 0:
                                fg[r, 2 * cp] = v0
                                fg[r, 2 * cp + 1] = v1
                        if rg in acc:
                            acc[rg] = acc[rg] + v0 * m0 + v1 * m1
                        else:
                            acc[rg] = v0 * m0 + v1 * m1
                        if cp == NCP - 1:
                            ac[a][rg] = acc[rg]
            assert not todo
            for _, f in side:
                f()

        def vpu_qk(nvq):
            row = lax.broadcasted_iota(jnp.int32, (8, 128), 0)
            cols = [c for j in range(NJ) for c in _columns(q_tile(qr2, j).astype(bf16).astype(f32))]
            run = {}
            tot = {}
            for c0 in range(NCP - nvq, NCP, 2):
                for rg in range(RP):
                    for cp in range(c0, min(c0 + 2, NCP)):
                        kv = _widen(kb[rg // 2, rg % 2, pl.ds(cp * 8, 8), :])
                        for p in range(2):
                            key = (cp - c0, 4 * p + rg // RH)
                            _accum(run, key, kv[p] * cols[rg])
                            tot[cp, key[1]] = run[key]
            for cp in range(NCP - nvq, NCP):
                a_ = jnp.zeros((8, 128), f32)
                for r in (0, 1, 4, 5):
                    z = tot[cp, r] - tot[cp - 2, r] if (cp - 2, r) in tot else tot[cp, r]
                    a_ = jnp.where(row == r, _sublane_sum(z), a_)
                svq[cp - (NCP - nvq), 0] = a_

        def layer(x, first):
            nvq = 0 if first else NVQ
            xc, rs = _center(x)
            xl[...] = _pack_rows(xc)
            rs_ref[...] = jnp.broadcast_to(rs * c_exp, (8, 128))
            ac1[...] = jnp.zeros(ac1.shape, f32)
            li1[...] = jnp.zeros(li1.shape, f32)
            ol0[...] = jnp.zeros(ol0.shape, u32)
            yr1[...] = jnp.zeros(yr1.shape, f32)
            ysum[...] = jnp.zeros(ysum.shape, f32)

            for i, dst in enumerate((qr2, qr3, qr0)):
                for n in range(NW):
                    qproj_tile(wqpair(i), dst, n)
            for j in range(NJ):
                build_l(qr2, lp, j)
            for n in range(CA * NT):
                qk_tile(kpair(0), lp, slo0, 0, CA, n)
            for n in range((CB - nvq) * NT):
                qk_tile(kpair(0), lp, shi0, CA, CB - nvq, n)
            if nvq:
                vpu_qk(nvq)
            for j in range(NJ):
                build_l(qr3, ln1, j)
            for n in range(CA * NT):
                qk_tile(kpair(1), ln1, slo1, 0, CA, n)
            softmax([(slo0, CA), (shi0, CB - nvq), (svq, nvq)], pb0, ls0)

            def block(i, a, order=MORD, rate=RATE, sets=SETS, pace_n=PACE):
                b = 1 - a
                side = [(max(SPOS, int(CB * NT * rate) + 1),
                         P(softmax, [(slo[b], CA), (shi[b], CB)], pb[b], ls[b])),
                        (IPOS, P(l_inv, ls[a], li[a])),
                        (YPOS, P(y_fold, yr[b]))]
                for j in range(NJ):
                    side.append((LPOS + 10 * j, P(build_l, qr[a], ln[a], j)))
                    side.append((RPOS + RSTEP * j, P(reduce_o, ac[b], li[b], ol[b], j)))
                run_block(first, i, a, 0, sets, order, rate, pace_n, side)

            def block14(i):
                side = [(int((CB - CM) * NT * RATE14) + 10,
                         P(softmax, [(slo1, CA), (smid, CM), (shi1, CB - CM)], pb1, ls1, pk1)),
                        (10, P(l_inv, ls0, li0)),
                        (100, P(pack_p, pb0, pk0)),
                        (5, P(y_fold, yr1))]
                side += [(100 + 10 * j, P(reduce_o, ac1, li1, ol1, j)) for j in range(NJ)]
                run_block(first, i, 0, 16, SETS14, "gwu", RATE14, PACE14, side)

            def block15(i):
                side = [(10, P(l_inv, ls1, li1)), (5, P(y_fold, yr0)), (25, P(y_fold, qr1))]
                side += [(100 + 10 * j, P(reduce_o, ac0, li0, ol0, j)) for j in range(1, NJ)]
                run_block(first, i, 1, 16, SETS15, "xv", RATE15, PACE15, side)

            def arrive(ch):
                for c in chunk(ch) + vstage(ch):
                    c.wait()
                for c in vstage(ch + 1):
                    c.start()

            def body(ch, one):
                if first:
                    arrive(ch)

                    @pl.when(ch + 2 < NC - 1)
                    def _():
                        for c in chunk(ch + 2):
                            c.start()

                    @pl.when(ch + 2 == NC - 1)
                    def _():
                        for c in vlast:
                            c.start()

                pl.when(one < 2)(P(block, 2 * ch, 0))
                pl.when(one > 0)(P(block, 2 * ch + 1, 1))
                return one

            one = lax.fori_loop(0, NC - 2, body, tbl[1])
            idx = (lambda i: i) if first else (lambda i: one * i)
            if first:
                arrive(NC - 2)
                for c in c1 + c2[0] + c2[1] + c2[2]:
                    c.start()
            block(idx(NP - 4), 0)
            pl.when(one > 0)(P(block, idx(NP - 3), 1, MORD13, RATE13, SETS13, PACE13))
            if first:
                for c in vlast + vstage(NC - 1):
                    c.wait()
            block14(idx(NP - 2))
            pl.when(one > 0)(P(block15, idx(NP - 1)))

            ox = [x_finish(0), x_finish(1)]
            for n in range(KD):
                wo_tile(wopair(NP - 2), ol0, yr0, n)
            for n in range(KD):
                wo_tile(wopair(NP - 1), ol1, qr0, n)
            wl = wopair(NP - 1)
            yv, mv = {}, {}
            for m in range(8, RH):
                ca, cb = [jnp.sum(ac1[rg], axis=1, keepdims=True) for rg in (2 * m, 2 * m + 1)]
                hh = 2 * m // RH
                for nt in range(KD):
                    wa, wb = _widen(wl[nt, pl.ds(8 * m, 8), :])
                    _accum(yv, (hh, nt), wa * ca + wb * cb)
                _accum(mv, hh, wsc[2 * m - 16] * ca + wsc[2 * m - 15] * cb)
            early = [_tree_sum([ysum[nt]] + [yr0[j * KD + nt] for j in range(1, NJ)])
                     for nt in range(KD)]
            ys = [_tree_sum([early[nt], yr0[nt], qr0[nt],
                             yv[0, nt] * li1[0:1, :], yv[1, nt] * li1[1:2, :]]) for nt in range(KD)]
            y = jnp.sum(jnp.concatenate(ys, axis=1), axis=0, keepdims=True)
            lanes = _tree_sum(early + [x[:, nt * 128:(nt + 1) * 128] * 0.125 for nt in range(KD)]
                              + [ox[0] * wsl[0], ox[1] * wsl[1]])
            tot = (jnp.sum(lanes, axis=1, keepdims=True)
                   + mv[0] * li1[0:1, :] + mv[1] * li1[1:2, :])
            mean = jnp.concatenate([_sublane_sum(tot) * (1.0 / D)] * KD, axis=1)
            x = x + y

            xc, rs = _center(x, mean)
            xn = _pack_rows(xc)
            if first:
                for c in c1:
                    c.wait()
            nv1 = 0 if first else NV1
            act = lambda h, n: _gelu(h * rs + b1v[n:n + 1, :].astype(f32))
            gs = {}
            for n in range(KF - nv1):
                gs[n] = act(_tree_sum(
                    _tile_dot(xn[:, kt * 128:(kt + 1) * 128], w1b[n, pl.ds(kt * 64, 64), :])
                    for kt in range(KD)), n)
            hv = {}
            for kt in range(KD if nv1 else 0):
                col = _columns(xc[:, kt * 128:(kt + 1) * 128])
                for v in range(8):
                    for n in range(KF - nv1, KF):
                        wa, wb = _widen(w1b[n, pl.ds(kt * 64 + 8 * v, 8), :])
                        _accum(hv, n, wa * col[2 * v] + wb * col[2 * v + 1])
            for n in hv:
                gs[n] = act(_sublane_sum(hv[n]), n)
            vk = range(W2SPLIT[1], KF) if first else range(NV2)
            cols = {kt: _columns(gs[kt]) for kt in vk}
            yv = {}
            parts = []
            for kt in range(KF):
                if first and kt in W2SPLIT:
                    for c in c2[W2SPLIT.index(kt)]:
                        c.wait()
                if kt not in vk:
                    hk = _pack_rows(gs[kt])
                    parts.append([_tile_dot(hk, w2b[nt, pl.ds(kt * 64, 64), :]) for nt in range(KD)])
                    continue
                for v in range(8):
                    for nt in range(KD):
                        wa, wb = _widen(w2b[nt, pl.ds(kt * 64 + 8 * v, 8), :])
                        _accum(yv, nt, wa * cols[kt][2 * v] + wb * cols[kt][2 * v + 1])
            y2 = jnp.concatenate(
                [_tree_sum([p[nt] for p in parts]
                           + [b2v[nt:nt + 1, :].astype(f32), _sublane_sum(yv[nt])])
                 for nt in range(KD)], axis=1)
            return x + y2

        for c in head:
            c.wait()

        def wo_rowsums(r0):
            w = _tree_sum(pltpu.bitcast(wob[nt, pl.ds(r0, 8), :], bf16).astype(f32) for nt in range(KD))
            return jnp.broadcast_to(jnp.sum(w, axis=1, keepdims=True), (16, 128))

        for m in range(8, RH):
            wsc[pl.ds(2 * m - 16, 2)] = wo_rowsums((NP - 1) * (PD // 2) + 8 * m).reshape(2, 8, 128)
        for s_ in range(2):
            rsum = jnp.concatenate([wo_rowsums((NP - 2 + s_) * (PD // 2) + 8 * m) for m in range(8)], axis=0)
            wsl[s_] = rsum.T[0:8]

        def transpose_tile(n, c):
            s8 = pl.multiple_of((n // (2 * NCP)) * 8, 8)
            e = n % 2
            c8 = pl.multiple_of(((n // 2) % NCP) * 8, 8)
            w = vx[pl.ds(s8, 8), e, pl.ds(c8, 8), :].reshape(64, 128)
            wt = pltpu.bitcast(w, bf16).astype(f32).T.astype(bf16)
            vx[pl.ds(s8, 8), e, pl.ds(c8, 8), :] = pltpu.bitcast(wt, u32).reshape(8, 8, 128)
            return c

        lax.fori_loop(0, 4 * NCP, transpose_tile, 0)

        x = jnp.broadcast_to(xin[0].astype(f32), (8, D))
        x = layer(x, True)
        x = layer(x, False)
        o_ref[0] = x[0:1, :].astype(o_ref.dtype)

    return kernel


@jax.jit
def pallas_interleave_layers__sliding_block_cached__dense_activation_gelu__decode_kernel(
    A_x, A_k_cache, A_v_cache, A_wq, A_wo, B_x, B_w1, B_b1, B_w2, B_b2,
):
    SK = A_k_cache.shape[2]
    W = min(4096, max(256, SK // 4))
    NR = H * DH // 8
    NCP = W // 256

    def tiled(a):
        t = jnp.swapaxes(a, 2, 3).reshape(NR, 8, SK // 128, 128)
        return t.transpose(0, 2, 1, 3).reshape(NR // 2, 2, SK // 16, 128)

    vreg = lambda n, dt: pltpu.VMEM(n + (8, 128), dt)
    return pl.pallas_call(
        _make_kernel(SK, W),
        out_shape=jax.ShapeDtypeStruct(A_x.shape, A_x.dtype),
        in_specs=[pl.BlockSpec(memory_space=pl.ANY)] * 9,
        out_specs=pl.BlockSpec(memory_space=pltpu.VMEM),
        scratch_shapes=[
            pltpu.VMEM((NR // 2, 2, W // 32, 128), u32),
            pltpu.VMEM((NR // 2 - 16 - NP * RF // 2, 2, W // 16, 128), bf16),
            pltpu.VMEM((2 * RF, 2, W // 16, 128), bf16),
            pltpu.VMEM((16, 2, W // 32, 128), u32),
            vreg((NP * RF, 2 * NCP), f32),
            pltpu.VMEM((H * DH // 128, D // 2, 128), u32),
            pltpu.VMEM((KD, H * DH // 2, 128), u32),
            pltpu.VMEM((KF, D // 2, 128), u32),
            pltpu.VMEM((KD, F // 2, 128), u32),
            pltpu.VMEM((1, 1, D), bf16),
            pltpu.VMEM((KF, 128), bf16),
            pltpu.VMEM((KD, 128), bf16),
            pltpu.VMEM((8, D), u32),
            pltpu.VMEM((8, 128), f32),
            vreg((KD,), f32),
        ] + [vreg((NT,), u32)] * 3
          + [vreg((NW,), f32)] * 4
          + [vreg((CA, NT), f32)] * 2
          + [vreg((CM, NT), f32)]
          + [vreg((NCP - CA, NT), f32)] * 2
          + [pltpu.VMEM((8, NCP * 128), f32)] * 2
          + [pltpu.VMEM((8, 128), f32)] * 4
          + [vreg((RP,), f32)] * 2
          + [vreg((NJ,), u32)] * 2
          + [vreg((NW,), f32)] * 2
          + [vreg((NCP,), u32)] * 2
          + [vreg((32,), f32), vreg((2,), f32)]
          + [vreg((NVQ, 1), f32)]
          + [pltpu.SMEM((NP,), jnp.int32), pltpu.SemaphoreType.DMA((5,))],
        compiler_params=pltpu.CompilerParams(vmem_limit_bytes=128 * 1024 * 1024),
    )(A_x, tiled(A_k_cache), tiled(A_v_cache), A_wq, A_wo, B_w1,
      B_b1.reshape(KF, 128), B_w2, B_b2.reshape(KD, 128))
```

```python
import functools
import jax
import jax.numpy as jnp
from jax import lax
import jax.experimental.pallas as pl
import jax.experimental.pallas.tpu as pltpu

D = 640
H = 32
DH = 192
F = 1536
NP = H // 2
PD = 2 * DH
RH = DH // 8
RP = 2 * RH
NJ = PD // 128
NT = 2 * NJ
KD = D // 128
KF = F // 128
NW = NJ * KD
NC = NP // 2
EPS = 1e-5
LOG2E = 1.4426950408889634
bf16 = jnp.bfloat16
f32 = jnp.float32
u32 = jnp.uint32

RF = 8
CA = 4
CM = 2
NVQ = 5
NV1 = 3
NV2 = 5
WOSTEP = 256
W2STEP = 192
W2SPLIT = (0, 9, 11, KF)
F0 = 15
D0 = 1
RATE = 6.0
PACE = 6
SETS = "10,10,10,18"
MORD = "hwql"
SPOS = 450
LPOS = 100
RPOS = 300
RSTEP = 80
YPOS = 5
IPOS = 150
RATE13 = 6.1
PACE13 = 3
SETS13 = "8,8,8,8,16"
MORD13 = "hwlm"
RATE14 = 5.6
PACE14 = 3
SETS14 = "8,8,8,8"
RATE15 = 6.2
PACE15 = 3
SETS15 = "8,8,10,6"
QRND = 1
QMEM = 1
QORD = 0
VG = 2


def _center(x, mean=None):
    xc = x - (jnp.mean(x, axis=-1, keepdims=True) if mean is None else mean)
    v = jnp.mean(xc * xc, axis=-1, keepdims=True)
    return xc, lax.rsqrt(v + EPS)


def _gelu(x):
    c = 0.7978845608028654
    return 0.5 * x * (1.0 + jnp.tanh(c * (x + 0.044715 * (x * x * x))))


def _pack_rows(x8):
    return pltpu.bitcast(jnp.concatenate([x8, x8], axis=0).astype(bf16), u32)


def _tile_dot(lhs_u32, w_u32):
    return jnp.dot(pltpu.bitcast(lhs_u32, bf16), pltpu.bitcast(w_u32, bf16),
                   preferred_element_type=f32)[0:8]


def _widen(slab_u32):
    w = pltpu.bitcast(slab_u32, bf16).astype(f32)
    return w[:8], w[8:]


def _columns(x8):
    t = jnp.concatenate([x8] * 16, axis=0).T
    return [t[8 * v:8 * v + 8] for v in range(16)]


def _sublane_sum(x8):
    for sh in (4, 2, 1):
        x8 = x8 + pltpu.roll(x8, sh, 0)
    return x8


def _tree(op, xs):
    xs = list(xs)
    while len(xs) > 1:
        xs = [op(xs[i], xs[i + 1]) if i + 1 < len(xs) else xs[i] for i in range(0, len(xs), 2)]
    return xs[0]


def _tree_sum(xs):
    return _tree(jnp.add, xs)


def _accum(d, key, t):
    d[key] = d[key] + t if key in d else t


def _make_kernel(SK, W):
    NCP = W // 256
    CB = NCP - CA
    RM = RH - RF // 2
    c_exp = (DH ** -0.5) * LOG2E
    P = functools.partial

    def kernel(x_hbm, k_hbm, v_hbm, wq_hbm, wo_hbm, w1_hbm, b1_hbm, w2_hbm, b2_hbm,
               o_ref,
               kb, vb, vs, vx, vf, wqb, wob, w1b, w2b, xin, b1v, b2v, xl, rs_ref, dm_ref, wcs, ysum,
               ln0, ln1, lp, qr0, qr1, qr2, qr3, slo0, slo1, smid, shi0, shi1, pb0, pb1,
               ls0, ls1, li0, li1, ac0, ac1, ol0, ol1, yr0, yr1, pk0, pk1, wsc, wsl, svq,
               tbl, sems):
        ln, qr, slo, shi = (ln0, ln1), (qr0, qr1), (slo0, slo1), (shi0, shi1)
        pb, ls, li, ac, ol, yr = (pb0, pb1), (ls0, ls1), (li0, li1), (ac0, ac1), (ol0, ol1), (yr0, yr1)
        pk = (pk0, pk1)

        ku = k_hbm.bitcast(u32)
        vu = v_hbm.bitcast(u32)

        def kcopy(c, s):
            return pltpu.make_async_copy(
                ku.at[pl.ds(c * RP, RP), :, pl.ds((SK - W) // 32, W // 32), :],
                kb.at[pl.ds(c * RP, RP)], sems.at[s])

        def vcopy(src0, n, dst, dst0, s):
            return pltpu.make_async_copy(
                v_hbm.at[pl.ds(src0, n), :, pl.ds((SK - W) // 16, W // 16), :],
                dst.at[pl.ds(dst0, n)], sems.at[s])

        def chunk(c):
            s = 1 + (c & 1)
            return [kcopy(c + 1, s)] + [vcopy((2 * c + p) * RH, RM, vb, (2 * c + p) * RM, s)
                                        for p in range(2)]

        def vstage(c):
            return [vcopy((2 * c + p) * RH + RM, RF // 2, vs, ((2 * c + p) & 3) * (RF // 2), 1 + (c & 1))
                    for p in range(2)]

        def wcopies(src, dst, s, r0=0, nrows=None, step=None):
            su = src.bitcast(u32)
            nrows = dst.shape[1] if nrows is None else nrows
            step = nrows if step is None else min(step, nrows)
            return [pltpu.make_async_copy(su.at[pl.ds(r, step), pl.ds(n * 128, 128)],
                                          dst.at[n, pl.ds(r, step)], sems.at[s])
                    for r in range(r0, r0 + nrows, step) for n in range(dst.shape[0])]

        head = [pltpu.make_async_copy(x_hbm, xin, sems.at[0]),
                pltpu.make_async_copy(b1_hbm, b1v, sems.at[0]),
                pltpu.make_async_copy(b2_hbm, b2v, sems.at[0])]
        head += [pltpu.make_async_copy(
            vu.at[pl.ds((NP - 2 + s) * RH, 8), :, pl.ds((SK - W) // 32, W // 32), :],
            vx.at[pl.ds(8 * s, 8)], sems.at[0]) for s in range(2)]
        head += wcopies(wq_hbm, wqb, 0) + wcopies(wo_hbm, wob, 0, step=WOSTEP) + [kcopy(0, 0)]
        vlast = [vcopy((NP - 2 + s) * RH + 8, RM - 8, vb, (NP - 2) * RM + s * (RM - 8), 2)
                 for s in range(2)]
        c1 = wcopies(w1_hbm, w1b, 1)
        c2 = [wcopies(w2_hbm, w2b, (0, 3, 4)[g], 64 * W2SPLIT[g],
                      64 * (W2SPLIT[g + 1] - W2SPLIT[g]), W2STEP) for g in range(3)]
        for c in head + chunk(0) + vstage(0) + chunk(1):
            c.start()

        for i_ in range(NP):
            tbl[i_] = i_

        live = {}

        def qproj_tile(wg, dst, n, cs=None):
            j, kt = divmod(n, KD)
            if cs is None:
                dst[n] = _tile_dot(xl[:, pl.ds(kt * 128, 128)], wg[j, pl.ds(kt * 64, 64), :])
                return
            r = jnp.dot(pltpu.bitcast(xl[:, pl.ds(kt * 128, 128)], bf16),
                        pltpu.bitcast(wg[j, pl.ds(kt * 64, 64), :], bf16), preferred_element_type=f32)
            dst[n] = r[0:8]
            _accum(live, j, r[8:16])
            if kt == KD - 1:
                cs[j] = live.pop(j)

        def q_tile(src, j, cs):
            q = _tree_sum(src[j * KD + kt] for kt in range(KD))
            if cs is not None:
                q = q - dm_ref[...] * cs[j]
            return q * rs_ref[...]

        def cspair(i):
            return wcs.at[pl.ds(i * NJ, NJ)]

        def build_l(src, dst, j, cs):
            row = lax.broadcasted_iota(jnp.int32, (8, 128), 0)
            lane = lax.broadcasted_iota(jnp.int32, (8, 128), 1)
            q = q_tile(src, j, cs)
            qp = pltpu.roll(q, 8, 1)
            qm = pltpu.roll(q, 120, 1)
            tgt = (lane >> 1) & 4
            if j == 1:
                tgt = tgt + (lane >> 6)
            elif j == 2:
                tgt = tgt + 1
            hit = row == tgt
            low = row < 4
            dst[2 * j] = _pack_rows(jnp.where(hit, jnp.where(low, q, qp), 0.0))
            dst[2 * j + 1] = _pack_rows(jnp.where(hit, jnp.where(low, qm, q), 0.0))

        def qk_tile(kg, lsrc, sdst, c0, ncp, n):
            c4, rem = divmod(n, 4 * NT)
            t, i = divmod(rem, min(4, ncp - c4 * 4))
            c = c4 * 4 + i
            w = kg[pl.ds((t // 2) * 8, 8), t % 2, pl.ds((c0 + c) * 8, 8), :].reshape(64, 128)
            sdst[c, t] = _tile_dot(lsrc[t], w)

        def softmax(srcs, pdst, ldst, kdst=None):
            s, m = [], None
            for src, n in srcs:
                for c0 in range(0, n, 4):
                    g = [_tree_sum(src[c, t] for t in range(src.shape[1]))
                         for c in range(c0, min(c0 + 4, n))]
                    s += g
                    m = _tree(jnp.maximum, g + ([] if m is None else [m]))
            m = jnp.maximum(m, pltpu.roll(m, 4, 0))
            m = jnp.max(m, axis=1, keepdims=True)
            e = [jnp.exp2(a - m) for a in s]
            for cp in range(NCP):
                pdst[:, pl.ds(cp * 128, 128)] = e[cp]
                if kdst is not None:
                    kdst[cp] = _pack_rows(e[cp])
            ldst[...] = _tree_sum(e)

        def l_inv(lsrc, ldst):
            l = lsrc[...]
            l = l + pltpu.roll(l, 4, 0)
            l = jnp.sum(l, axis=1, keepdims=True)
            ldst[...] = jnp.broadcast_to(1.0 / l, (8, 128))

        def pack_p(psrc, kdst):
            for cp in range(NCP):
                kdst[cp] = _pack_rows(psrc[:, pl.ds(cp * 128, 128)])

        def reduce_o(asrc, lsrc, odst, j):
            t = asrc[pl.ds(j * 16, 16)].reshape(128, 128).T.reshape(16, 8, 128)
            if j == 1:
                lane = lax.broadcasted_iota(jnp.int32, (1, 128), 1)
                r = jnp.where(lane < 64, lsrc[0:1, :], lsrc[1:2, :])
            else:
                r = lsrc[j // 2:j // 2 + 1, :]
            odst[j] = _pack_rows(_tree_sum(t[i] for i in range(16)) * r)

        def x_tile(vg, n):
            s, rem = divmod(n, 2 * NCP)
            cp, e = divmod(rem, 2)
            w = vg[pl.ds(8 * s, 8), e, pl.ds(cp * 8, 8), :].reshape(64, 128)
            shi0[divmod(n, NT)] = _tile_dot(pk[s][cp], w)

        def x_finish(s):
            row = lax.broadcasted_iota(jnp.int32, (8, 128), 0)
            lane = lax.broadcasted_iota(jnp.int32, (8, 128), 1)
            o0, o1 = [_tree_sum(shi0[divmod((s * NCP + cp) * 2 + e, NT)] for cp in range(NCP))
                      for e in range(2)]
            low = row < 4
            direct = jnp.where(low, o0, o1)
            moved = jnp.where(low, pltpu.roll(o1, 8, 1), pltpu.roll(o0, 120, 1))
            o = jnp.where(((lane >> 1) & 4) == (row & 4), direct, moved)
            o = jnp.where((row & 3) == 0, o, 0.0) * li[s][0:1, :]
            ol[s][0] = _pack_rows(o)
            return o

        def wo_tile(wg, osrc, ydst, n):
            j, nt = divmod(n, KD)
            ydst[n] = _tile_dot(osrc[j], wg[nt, pl.ds(j * 64, 64), :])

        def y_fold(ysrc):
            for nt in range(KD):
                ysum[nt] = _tree_sum([ysum[nt]] + [ysrc[j * KD + nt] for j in range(NJ)])

        def kpair(i):
            return kb.at[pl.ds(i * RH, RH)]

        def wqpair(i):
            return wqb.at[pl.ds(i * NJ, NJ)]

        def wopair(i):
            r0 = i * (PD // 2)
            if not isinstance(i, int):
                r0 = pl.multiple_of(r0, PD // 2)
            return wob.at[:, pl.ds(r0, PD // 2), :]

        def mxu_kinds(a, first):
            b = 1 - a
            return dict(
                h=(CB * NT, lambda z: kpair(z + 1),
                   lambda w, n: qk_tile(w, ln[b], shi[b], CA, CB, n)),
                g=((CB - CM) * NT, lambda z: kpair(z + 1),
                   lambda w, n: qk_tile(w, ln[b], shi[b], CA + CM, CB - CM, n)),
                l=(CA * NT, lambda z: kpair(z + 2),
                   lambda w, n: qk_tile(w, ln[a], slo[a], 0, CA, n)),
                m=(CM * NT, lambda z: kpair(z + 2),
                   lambda w, n: qk_tile(w, ln[a], smid, CA, CM, n)),
                q=(NW, lambda z: (wqpair(jnp.minimum(z + 3, NP - 1)),
                                  cspair(jnp.minimum(z + 3, NP - 1)) if first else None),
                   lambda w, n: qproj_tile(w[0], qr[b], n, w[1])),
                w=(NW, lambda z: wopair(jnp.maximum(z - 2, 0)),
                   lambda w, n: wo_tile(w, ol[a], yr[a], n)),
                u=(NW, lambda z: wopair(z - 1),
                   lambda w, n: wo_tile(w, ol1, qr1, n)),
                v=(2 * KD, lambda z: wopair(z - 1),
                   lambda w, n: wo_tile(w, ol0, yr0, KD + n)),
                x=(4 * NCP, lambda z: vx.at[pl.ds((z - (NP - 1)) * 16, 16)], x_tile))

        def run_block(first, i, a, rg0, sets, order, rate, pace_n, side):
            if rg0:
                vg = vb.at[pl.ds((NP - 2) * RM + a * (RM - 8), RM - 8)]
            else:
                vg = vb.at[pl.ds(i * RM, RM)]
            sg = vs.at[pl.ds((i & 3) * (RF // 2), RF // 2)]
            fg = vf.at[pl.ds(i * RF, RF)]
            kinds = mxu_kinds(a, first)

            pace = dict(z=i, cnt=0, views={})

            def mxu_tile(key, n):
                if not first and pace["cnt"] % pace_n == 0:
                    for _ in range(pace_n * 4 // 3 if pace["cnt"] else D0):
                        pace["z"] = tbl[pace["z"]]
                    pace["views"] = {}
                pace["cnt"] += 1
                if key not in pace["views"]:
                    pace["views"][key] = kinds[key][1](pace["z"])
                kinds[key][2](pace["views"][key], n)

            mxu = [P(mxu_tile, key, n) for key in order for n in range(kinds[key][0])]
            side = sorted(side + [(int(n * rate), f) for n, f in enumerate(mxu)], key=lambda z: z[0])

            n_all = RP - rg0
            f0 = F0 * n_all // RP
            slots = sorted(f0 + (k + 1) * (n_all - f0) // RF - 1 for k in range(RF))
            todo = list(range(rg0, RP - RF))
            for k, pos in enumerate(slots):
                todo.insert(pos, RP - RF + k)
            cnt = 0
            acc = {}
            for size in (int(z) for z in sets.split(",")):
                rgs, todo = todo[:size], todo[size:]
                for cp in range(NCP):
                    mult = {hh: (pb[a][pl.ds(hh, 1), pl.ds(cp * 128, 128)],
                                 pb[a][pl.ds(4 + hh, 1), pl.ds(cp * 128, 128)])
                            for hh in sorted({rg // RH for rg in rgs})}
                    for rg in rgs:
                        while side and side[0][0] <= cnt:
                            side.pop(0)[1]()
                        cnt += 1
                        m0, m1 = mult[rg // RH]
                        r = rg - (RP - RF)
                        if r >= 0 and not first:
                            v0, v1 = fg[r, 2 * cp], fg[r, 2 * cp + 1]
                        else:
                            src = sg.at[r // 2, r % 2] if r >= 0 else vg.at[(rg - rg0) // 2, rg % 2]
                            v = src[pl.ds(cp * 16, 16), :].astype(f32)
                            v0, v1 = v[:8], v[8:]
                            if r >= 0:
                                fg[r, 2 * cp] = v0
                                fg[r, 2 * cp + 1] = v1
                        if rg in acc:
                            acc[rg] = acc[rg] + v0 * m0 + v1 * m1
                        else:
                            acc[rg] = v0 * m0 + v1 * m1
                        if cp == NCP - 1:
                            ac[a][rg] = acc[rg]
            assert not todo
            for _, f in side:
                f()

        def vpu_qk(nvq):
            row = lax.broadcasted_iota(jnp.int32, (8, 128), 0)
            rnd = (lambda q: q.astype(bf16).astype(f32)) if QRND else (lambda q: q)
            cols = [c for j in range(NJ) for c in _columns(rnd(q_tile(qr2, j, cspair(0))))]
            if QMEM:
                for rg in range(RP):
                    ac0[rg] = cols[rg]
            run = {}
            tot = {}
            order = {0: range(RP), 1: [r for k in range(RH) for r in (k, RH + k)],
                     2: list(range(32, 48)) + list(range(32))}[QORD]
            for c0 in range(NCP - nvq, NCP, VG):
                for rg in order:
                    col = ac0[rg] if QMEM else cols[rg]
                    for cp in range(c0, min(c0 + VG, NCP)):
                        kv = _widen(kb[rg // 2, rg % 2, pl.ds(cp * 8, 8), :])
                        for p in range(2):
                            key = (cp - c0, 4 * p + rg // RH)
                            _accum(run, key, kv[p] * col)
                            tot[cp, key[1]] = run[key]
            for cp in range(NCP - nvq, NCP):
                a_ = jnp.zeros((8, 128), f32)
                for r in (0, 1, 4, 5):
                    z = tot[cp, r] - tot[cp - VG, r] if (cp - VG, r) in tot else tot[cp, r]
                    a_ = jnp.where(row == r, _sublane_sum(z), a_)
                svq[cp - (NCP - nvq), 0] = a_

        def layer(x, guess):
            first = guess is None
            nvq = 0 if first else NVQ
            if first:
                xc, rs = _center(x)
                xl[...] = pltpu.bitcast(
                    jnp.concatenate([xc, jnp.ones_like(xc)], axis=0).astype(bf16), u32)
            else:
                xc = x - jnp.concatenate([guess] * KD, axis=1)
                xl[...] = _pack_rows(xc)
                dm = jnp.mean(xc, axis=-1, keepdims=True)
                var = jnp.maximum(jnp.mean(xc * xc, axis=-1, keepdims=True) - dm * dm, 0.0)
                rs = lax.rsqrt(var + EPS)
                dm_ref[...] = jnp.broadcast_to(dm, (8, 128))
            rd = (lambda i: None) if first else cspair
            wr = cspair if first else (lambda i: None)
            rs_ref[...] = jnp.broadcast_to(rs * c_exp, (8, 128))
            ac1[...] = jnp.zeros(ac1.shape, f32)
            li1[...] = jnp.zeros(li1.shape, f32)
            ol0[...] = jnp.zeros(ol0.shape, u32)
            yr1[...] = jnp.zeros(yr1.shape, f32)
            ysum[...] = jnp.zeros(ysum.shape, f32)

            for i, dst in enumerate((qr2, qr3, qr0)):
                for n in range(NW):
                    qproj_tile(wqpair(i), dst, n, wr(i))
            for j in range(NJ):
                build_l(qr2, lp, j, rd(0))
            for n in range(CA * NT):
                qk_tile(kpair(0), lp, slo0, 0, CA, n)
            for n in range((CB - nvq) * NT):
                qk_tile(kpair(0), lp, shi0, CA, CB - nvq, n)
            if nvq:
                vpu_qk(nvq)
            for j in range(NJ):
                build_l(qr3, ln1, j, rd(1))
            for n in range(CA * NT):
                qk_tile(kpair(1), ln1, slo1, 0, CA, n)
            softmax([(slo0, CA), (shi0, CB - nvq), (svq, nvq)], pb0, ls0)

            def block(i, a, order=MORD, rate=RATE, sets=SETS, pace_n=PACE):
                b = 1 - a
                cs = rd(i + 2)
                side = [(max(SPOS, int(CB * NT * rate) + 1),
                         P(softmax, [(slo[b], CA), (shi[b], CB)], pb[b], ls[b])),
                        (IPOS, P(l_inv, ls[a], li[a])),
                        (YPOS, P(y_fold, yr[b]))]
                for j in range(NJ):
                    side.append((LPOS + 10 * j, P(build_l, qr[a], ln[a], j, cs)))
                    side.append((RPOS + RSTEP * j, P(reduce_o, ac[b], li[b], ol[b], j)))
                run_block(first, i, a, 0, sets, order, rate, pace_n, side)

            def block14(i):
                side = [(int((CB - CM) * NT * RATE14) + 10,
                         P(softmax, [(slo1, CA), (smid, CM), (shi1, CB - CM)], pb1, ls1, pk1)),
                        (10, P(l_inv, ls0, li0)),
                        (100, P(pack_p, pb0, pk0)),
                        (5, P(y_fold, yr1))]
                side += [(100 + 10 * j, P(reduce_o, ac1, li1, ol1, j)) for j in range(NJ)]
                run_block(first, i, 0, 16, SETS14, "gwu", RATE14, PACE14, side)

            def block15(i):
                side = [(10, P(l_inv, ls1, li1)), (5, P(y_fold, yr0)), (25, P(y_fold, qr1))]
                side += [(100 + 10 * j, P(reduce_o, ac0, li0, ol0, j)) for j in range(1, NJ)]
                run_block(first, i, 1, 16, SETS15, "xv", RATE15, PACE15, side)

            def arrive(ch):
                for c in chunk(ch) + vstage(ch):
                    c.wait()
                for c in vstage(ch + 1):
                    c.start()

            def body(ch, one):
                if first:
                    arrive(ch)

                    @pl.when(ch + 2 < NC - 1)
                    def _():
                        for c in chunk(ch + 2):
                            c.start()

                    @pl.when(ch + 2 == NC - 1)
                    def _():
                        for c in vlast:
                            c.start()

                pl.when(one < 2)(P(block, 2 * ch, 0))
                pl.when(one > 0)(P(block, 2 * ch + 1, 1))
                return one

            one = lax.fori_loop(0, NC - 2, body, tbl[1])
            idx = (lambda i: i) if first else (lambda i: one * i)
            if first:
                arrive(NC - 2)
                for c in c1 + c2[0] + c2[1] + c2[2]:
                    c.start()
            block(idx(NP - 4), 0)
            pl.when(one > 0)(P(block, idx(NP - 3), 1, MORD13, RATE13, SETS13, PACE13))
            if first:
                for c in vlast + vstage(NC - 1):
                    c.wait()
            block14(idx(NP - 2))
            pl.when(one > 0)(P(block15, idx(NP - 1)))

            ox = [x_finish(0), x_finish(1)]
            for n in range(KD):
                wo_tile(wopair(NP - 2), ol0, yr0, n)
            for n in range(KD):
                wo_tile(wopair(NP - 1), ol1, qr0, n)
            wl = wopair(NP - 1)
            yv, mv = {}, {}
            for m in range(8, RH):
                ca, cb = [jnp.sum(ac1[rg], axis=1, keepdims=True) for rg in (2 * m, 2 * m + 1)]
                hh = 2 * m // RH
                for nt in range(KD):
                    wa, wb = _widen(wl[nt, pl.ds(8 * m, 8), :])
                    _accum(yv, (hh, nt), wa * ca + wb * cb)
                _accum(mv, hh, wsc[2 * m - 16] * ca + wsc[2 * m - 15] * cb)
            early = [_tree_sum([ysum[nt]] + [yr0[j * KD + nt] for j in range(1, NJ)])
                     for nt in range(KD)]
            ys = [_tree_sum([early[nt], yr0[nt], qr0[nt],
                             yv[0, nt] * li1[0:1, :], yv[1, nt] * li1[1:2, :]]) for nt in range(KD)]
            y = jnp.sum(jnp.concatenate(ys, axis=1), axis=0, keepdims=True)
            lanes = _tree_sum(early + [x[:, nt * 128:(nt + 1) * 128] * 0.125 for nt in range(KD)]
                              + [ox[0] * wsl[0], ox[1] * wsl[1]])
            tot = (jnp.sum(lanes, axis=1, keepdims=True)
                   + mv[0] * li1[0:1, :] + mv[1] * li1[1:2, :])
            mean = jnp.concatenate([_sublane_sum(tot) * (1.0 / D)] * KD, axis=1)
            x = x + y

            xc, rs = _center(x, mean)
            xn = _pack_rows(xc)
            if first:
                for c in c1:
                    c.wait()
            nv1 = 0 if first else NV1
            act = lambda h, n: _gelu(h * rs + b1v[n:n + 1, :].astype(f32))
            gs = {}
            for n in range(KF - nv1):
                gs[n] = act(_tree_sum(
                    _tile_dot(xn[:, kt * 128:(kt + 1) * 128], w1b[n, pl.ds(kt * 64, 64), :])
                    for kt in range(KD)), n)
            hv = {}
            for kt in range(KD if nv1 else 0):
                col = _columns(xc[:, kt * 128:(kt + 1) * 128])
                for v in range(8):
                    for n in range(KF - nv1, KF):
                        wa, wb = _widen(w1b[n, pl.ds(kt * 64 + 8 * v, 8), :])
                        _accum(hv, n, wa * col[2 * v] + wb * col[2 * v + 1])
            for n in hv:
                gs[n] = act(_sublane_sum(hv[n]), n)
            vk = range(W2SPLIT[1], KF) if first else range(NV2)
            cols = {kt: _columns(gs[kt]) for kt in vk}
            yv = {}
            parts = []
            for kt in range(KF):
                if first and kt == W2SPLIT[2]:
                    known = [_tree_sum([p[nt] for p in parts] + [x[:, nt * 128:(nt + 1) * 128],
                                                                 b2v[nt:nt + 1, :].astype(f32),
                                                                 _sublane_sum(yv.pop(nt))])
                             for nt in range(KD)]
                    guess = jnp.broadcast_to(
                        jnp.sum(_tree_sum(known), axis=1, keepdims=True) * (1.0 / D), (8, 128))
                if first and kt in W2SPLIT:
                    for c in c2[W2SPLIT.index(kt)]:
                        c.wait()
                if kt not in vk:
                    hk = _pack_rows(gs[kt])
                    parts.append([_tile_dot(hk, w2b[nt, pl.ds(kt * 64, 64), :]) for nt in range(KD)])
                    continue
                for v in range(8):
                    for nt in range(KD):
                        wa, wb = _widen(w2b[nt, pl.ds(kt * 64 + 8 * v, 8), :])
                        _accum(yv, nt, wa * cols[kt][2 * v] + wb * cols[kt][2 * v + 1])
            if first:
                return jnp.concatenate([known[nt] + _sublane_sum(yv[nt]) for nt in range(KD)], axis=1), guess
            y2 = jnp.concatenate(
                [_tree_sum([p[nt] for p in parts]
                           + [b2v[nt:nt + 1, :].astype(f32), _sublane_sum(yv[nt])])
                 for nt in range(KD)], axis=1)
            return x + y2

        for c in head:
            c.wait()

        def wo_rowsums(r0):
            w = _tree_sum(pltpu.bitcast(wob[nt, pl.ds(r0, 8), :], bf16).astype(f32) for nt in range(KD))
            return jnp.broadcast_to(jnp.sum(w, axis=1, keepdims=True), (16, 128))

        for m in range(8, RH):
            wsc[pl.ds(2 * m - 16, 2)] = wo_rowsums((NP - 1) * (PD // 2) + 8 * m).reshape(2, 8, 128)
        for s_ in range(2):
            rsum = jnp.concatenate([wo_rowsums((NP - 2 + s_) * (PD // 2) + 8 * m) for m in range(8)], axis=0)
            wsl[s_] = rsum.T[0:8]

        def transpose_tile(n, c):
            s8 = pl.multiple_of((n // (2 * NCP)) * 8, 8)
            e = n % 2
            c8 = pl.multiple_of(((n // 2) % NCP) * 8, 8)
            w = vx[pl.ds(s8, 8), e, pl.ds(c8, 8), :].reshape(64, 128)
            wt = pltpu.bitcast(w, bf16).astype(f32).T.astype(bf16)
            vx[pl.ds(s8, 8), e, pl.ds(c8, 8), :] = pltpu.bitcast(wt, u32).reshape(8, 8, 128)
            return c

        lax.fori_loop(0, 4 * NCP, transpose_tile, 0)

        x = jnp.broadcast_to(xin[0].astype(f32), (8, D))
        x, guess = layer(x, None)
        x = layer(x, guess)
        o_ref[0] = x[0:1, :].astype(o_ref.dtype)

    return kernel


@jax.jit
def pallas_interleave_layers__sliding_block_cached__dense_activation_gelu__decode_kernel(
    A_x, A_k_cache, A_v_cache, A_wq, A_wo, B_x, B_w1, B_b1, B_w2, B_b2,
):
    SK = A_k_cache.shape[2]
    W = min(4096, max(256, SK // 4))
    NR = H * DH // 8
    NCP = W // 256

    def tiled(a):
        t = jnp.swapaxes(a, 2, 3).reshape(NR, 8, SK // 128, 128)
        return t.transpose(0, 2, 1, 3).reshape(NR // 2, 2, SK // 16, 128)

    vreg = lambda n, dt: pltpu.VMEM(n + (8, 128), dt)
    return pl.pallas_call(
        _make_kernel(SK, W),
        out_shape=jax.ShapeDtypeStruct(A_x.shape, A_x.dtype),
        in_specs=[pl.BlockSpec(memory_space=pl.ANY)] * 9,
        out_specs=pl.BlockSpec(memory_space=pltpu.VMEM),
        scratch_shapes=[
            pltpu.VMEM((NR // 2, 2, W // 32, 128), u32),
            pltpu.VMEM((NR // 2 - 16 - NP * RF // 2, 2, W // 16, 128), bf16),
            pltpu.VMEM((2 * RF, 2, W // 16, 128), bf16),
            pltpu.VMEM((16, 2, W // 32, 128), u32),
            vreg((NP * RF, 2 * NCP), f32),
            pltpu.VMEM((H * DH // 128, D // 2, 128), u32),
            pltpu.VMEM((KD, H * DH // 2, 128), u32),
            pltpu.VMEM((KF, D // 2, 128), u32),
            pltpu.VMEM((KD, F // 2, 128), u32),
            pltpu.VMEM((1, 1, D), bf16),
            pltpu.VMEM((KF, 128), bf16),
            pltpu.VMEM((KD, 128), bf16),
            pltpu.VMEM((8, D), u32),
            pltpu.VMEM((8, 128), f32),
            pltpu.VMEM((8, 128), f32),
            vreg((NP * NJ,), f32),
            vreg((KD,), f32),
        ] + [vreg((NT,), u32)] * 3
          + [vreg((NW,), f32)] * 4
          + [vreg((CA, NT), f32)] * 2
          + [vreg((CM, NT), f32)]
          + [vreg((NCP - CA, NT), f32)] * 2
          + [pltpu.VMEM((8, NCP * 128), f32)] * 2
          + [pltpu.VMEM((8, 128), f32)] * 4
          + [vreg((RP,), f32)] * 2
          + [vreg((NJ,), u32)] * 2
          + [vreg((NW,), f32)] * 2
          + [vreg((NCP,), u32)] * 2
          + [vreg((32,), f32), vreg((2,), f32)]
          + [vreg((NVQ, 1), f32)]
          + [pltpu.SMEM((NP,), jnp.int32), pltpu.SemaphoreType.DMA((5,))],
        compiler_params=pltpu.CompilerParams(vmem_limit_bytes=128 * 1024 * 1024),
    )(A_x, tiled(A_k_cache), tiled(A_v_cache), A_wq, A_wo, B_w1,
      B_b1.reshape(KF, 128), B_w2, B_b2.reshape(KD, 128))
```

```python
import functools
import jax
import jax.numpy as jnp
from jax import lax
import jax.experimental.pallas as pl
import jax.experimental.pallas.tpu as pltpu

D = 640
H = 32
DH = 192
F = 1536
NP = H // 2
PD = 2 * DH
RH = DH // 8
RP = 2 * RH
NJ = PD // 128
NT = 2 * NJ
KD = D // 128
KF = F // 128
NW = NJ * KD
NC = NP // 2
EPS = 1e-5
LOG2E = 1.4426950408889634
bf16 = jnp.bfloat16
f32 = jnp.float32
u32 = jnp.uint32

RF = 8
CA = 4
CM = 2
NVQ = 5
NV1 = 3
NV2 = 5
WOSTEP = 256
W2STEP = 192
W2SPLIT = (0, 9, 11, KF)
F0 = 15
D0 = 1
RATE = 6.0
PACE = 6
SETS = "10,10,10,18"
MORD = "hwql"
SPOS = 450
LPOS = 100
RPOS = 300
RSTEP = 80
YPOS = 5
IPOS = 150
RATE13 = 6.1
PACE13 = 3
SETS13 = "8,8,8,8,16"
MORD13 = "hwlm"
RATE14 = 5.6
PACE14 = 3
SETS14 = "8,8,8,8"
RATE15 = 6.2
PACE15 = 3
SETS15 = "8,8,10,6"


def _center(x, mean=None):
    xc = x - (jnp.mean(x, axis=-1, keepdims=True) if mean is None else mean)
    v = jnp.mean(xc * xc, axis=-1, keepdims=True)
    return xc, lax.rsqrt(v + EPS)


def _gelu(x):
    c = 0.7978845608028654
    return 0.5 * x * (1.0 + jnp.tanh(c * (x + 0.044715 * (x * x * x))))


def _pack_rows(x8):
    return pltpu.bitcast(jnp.concatenate([x8, x8], axis=0).astype(bf16), u32)


def _tile_dot(lhs_u32, w_u32):
    return jnp.dot(pltpu.bitcast(lhs_u32, bf16), pltpu.bitcast(w_u32, bf16),
                   preferred_element_type=f32)[0:8]


def _widen(slab_u32):
    w = pltpu.bitcast(slab_u32, bf16).astype(f32)
    return w[:8], w[8:]


def _columns(x8):
    t = jnp.concatenate([x8] * 16, axis=0).T
    return [t[8 * v:8 * v + 8] for v in range(16)]


def _sublane_sum(x8):
    for sh in (4, 2, 1):
        x8 = x8 + pltpu.roll(x8, sh, 0)
    return x8


def _tree(op, xs):
    xs = list(xs)
    while len(xs) > 1:
        xs = [op(xs[i], xs[i + 1]) if i + 1 < len(xs) else xs[i] for i in range(0, len(xs), 2)]
    return xs[0]


def _tree_sum(xs):
    return _tree(jnp.add, xs)


def _accum(d, key, t):
    d[key] = d[key] + t if key in d else t


def _make_kernel(SK, W):
    NCP = W // 256
    CB = NCP - CA
    RM = RH - RF // 2
    c_exp = (DH ** -0.5) * LOG2E
    P = functools.partial

    def kernel(x_hbm, k_hbm, v_hbm, wq_hbm, wo_hbm, w1_hbm, b1_hbm, w2_hbm, b2_hbm,
               o_ref,
               kb, vb, vs, vx, vf, wqb, wob, w1b, w2b, xin, b1v, b2v, xl, rs_ref, dm_ref, wcs, ysum,
               ln0, ln1, lp, qr0, qr1, qr2, qr3, slo0, slo1, smid, shi0, shi1, pb0, pb1,
               ls0, ls1, li0, li1, ac0, ac1, ol0, ol1, yr0, yr1, pk0, pk1, wsc, wsl, svq,
               tbl, sems):
        ln, qr, slo, shi = (ln0, ln1), (qr0, qr1), (slo0, slo1), (shi0, shi1)
        pb, ls, li, ac, ol, yr = (pb0, pb1), (ls0, ls1), (li0, li1), (ac0, ac1), (ol0, ol1), (yr0, yr1)
        pk = (pk0, pk1)

        ku = k_hbm.bitcast(u32)
        vu = v_hbm.bitcast(u32)

        def kcopy(c, s):
            return pltpu.make_async_copy(
                ku.at[pl.ds(c * RP, RP), :, pl.ds((SK - W) // 32, W // 32), :],
                kb.at[pl.ds(c * RP, RP)], sems.at[s])

        def vcopy(src0, n, dst, dst0, s):
            return pltpu.make_async_copy(
                v_hbm.at[pl.ds(src0, n), :, pl.ds((SK - W) // 16, W // 16), :],
                dst.at[pl.ds(dst0, n)], sems.at[s])

        def chunk(c):
            s = 1 + (c & 1)
            return [kcopy(c + 1, s)] + [vcopy((2 * c + p) * RH, RM, vb, (2 * c + p) * RM, s)
                                        for p in range(2)]

        def vstage(c):
            return [vcopy((2 * c + p) * RH + RM, RF // 2, vs, ((2 * c + p) & 3) * (RF // 2), 1 + (c & 1))
                    for p in range(2)]

        def wcopies(src, dst, s, r0=0, nrows=None, step=None):
            su = src.bitcast(u32)
            nrows = dst.shape[1] if nrows is None else nrows
            step = nrows if step is None else min(step, nrows)
            return [pltpu.make_async_copy(su.at[pl.ds(r, step), pl.ds(n * 128, 128)],
                                          dst.at[n, pl.ds(r, step)], sems.at[s])
                    for r in range(r0, r0 + nrows, step) for n in range(dst.shape[0])]

        head = [pltpu.make_async_copy(x_hbm, xin, sems.at[0]),
                pltpu.make_async_copy(b1_hbm, b1v, sems.at[0]),
                pltpu.make_async_copy(b2_hbm, b2v, sems.at[0])]
        head += [pltpu.make_async_copy(
            vu.at[pl.ds((NP - 2 + s) * RH, 8), :, pl.ds((SK - W) // 32, W // 32), :],
            vx.at[pl.ds(8 * s, 8)], sems.at[0]) for s in range(2)]
        head += wcopies(wq_hbm, wqb, 0) + wcopies(wo_hbm, wob, 0, step=WOSTEP) + [kcopy(0, 0)]
        vlast = [vcopy((NP - 2 + s) * RH + 8, RM - 8, vb, (NP - 2) * RM + s * (RM - 8), 2)
                 for s in range(2)]
        c1 = wcopies(w1_hbm, w1b, 1)
        c2 = [wcopies(w2_hbm, w2b, (0, 3, 4)[g], 64 * W2SPLIT[g],
                      64 * (W2SPLIT[g + 1] - W2SPLIT[g]), W2STEP) for g in range(3)]
        for c in head + chunk(0) + vstage(0) + chunk(1):
            c.start()

        for i_ in range(NP):
            tbl[i_] = i_

        live = {}

        def qproj_tile(wg, dst, n, cs=None):
            j, kt = divmod(n, KD)
            if cs is None:
                dst[n] = _tile_dot(xl[:, pl.ds(kt * 128, 128)], wg[j, pl.ds(kt * 64, 64), :])
                return
            r = jnp.dot(pltpu.bitcast(xl[:, pl.ds(kt * 128, 128)], bf16),
                        pltpu.bitcast(wg[j, pl.ds(kt * 64, 64), :], bf16), preferred_element_type=f32)
            dst[n] = r[0:8]
            _accum(live, j, r[8:16])
            if kt == KD - 1:
                cs[j] = live.pop(j)

        def q_tile(src, j, cs):
            q = _tree_sum(src[j * KD + kt] for kt in range(KD))
            if cs is not None:
                q = q - dm_ref[...] * cs[j]
            return q * rs_ref[...]

        def cspair(i):
            return wcs.at[pl.ds(i * NJ, NJ)]

        def build_l(src, dst, j, cs):
            row = lax.broadcasted_iota(jnp.int32, (8, 128), 0)
            lane = lax.broadcasted_iota(jnp.int32, (8, 128), 1)
            q = q_tile(src, j, cs)
            qp = pltpu.roll(q, 8, 1)
            qm = pltpu.roll(q, 120, 1)
            tgt = (lane >> 1) & 4
            if j == 1:
                tgt = tgt + (lane >> 6)
            elif j == 2:
                tgt = tgt + 1
            hit = row == tgt
            low = row < 4
            dst[2 * j] = _pack_rows(jnp.where(hit, jnp.where(low, q, qp), 0.0))
            dst[2 * j + 1] = _pack_rows(jnp.where(hit, jnp.where(low, qm, q), 0.0))

        def qk_tile(kg, lsrc, sdst, c0, ncp, n):
            c4, rem = divmod(n, 4 * NT)
            t, i = divmod(rem, min(4, ncp - c4 * 4))
            c = c4 * 4 + i
            w = kg[pl.ds((t // 2) * 8, 8), t % 2, pl.ds((c0 + c) * 8, 8), :].reshape(64, 128)
            sdst[c, t] = _tile_dot(lsrc[t], w)

        def softmax(srcs, pdst, ldst, kdst=None):
            s, m = [], None
            for src, n in srcs:
                for c0 in range(0, n, 4):
                    g = [_tree_sum(src[c, t] for t in range(src.shape[1]))
                         for c in range(c0, min(c0 + 4, n))]
                    s += g
                    m = _tree(jnp.maximum, g + ([] if m is None else [m]))
            m = jnp.maximum(m, pltpu.roll(m, 4, 0))
            m = jnp.max(m, axis=1, keepdims=True)
            e = [jnp.exp2(a - m) for a in s]
            for cp in range(NCP):
                pdst[:, pl.ds(cp * 128, 128)] = e[cp]
                if kdst is not None:
                    kdst[cp] = _pack_rows(e[cp])
            ldst[...] = _tree_sum(e)

        def l_inv(lsrc, ldst):
            l = lsrc[...]
            l = l + pltpu.roll(l, 4, 0)
            l = jnp.sum(l, axis=1, keepdims=True)
            ldst[...] = jnp.broadcast_to(1.0 / l, (8, 128))

        def pack_p(psrc, kdst):
            for cp in range(NCP):
                kdst[cp] = _pack_rows(psrc[:, pl.ds(cp * 128, 128)])

        def reduce_o(asrc, lsrc, odst, j):
            t = asrc[pl.ds(j * 16, 16)].reshape(128, 128).T.reshape(16, 8, 128)
            if j == 1:
                lane = lax.broadcasted_iota(jnp.int32, (1, 128), 1)
                r = jnp.where(lane < 64, lsrc[0:1, :], lsrc[1:2, :])
            else:
                r = lsrc[j // 2:j // 2 + 1, :]
            odst[j] = _pack_rows(_tree_sum(t[i] for i in range(16)) * r)

        def x_tile(vg, n):
            s, rem = divmod(n, 2 * NCP)
            cp, e = divmod(rem, 2)
            w = vg[pl.ds(8 * s, 8), e, pl.ds(cp * 8, 8), :].reshape(64, 128)
            shi0[divmod(n, NT)] = _tile_dot(pk[s][cp], w)

        def x_finish(s):
            row = lax.broadcasted_iota(jnp.int32, (8, 128), 0)
            lane = lax.broadcasted_iota(jnp.int32, (8, 128), 1)
            o0, o1 = [_tree_sum(shi0[divmod((s * NCP + cp) * 2 + e, NT)] for cp in range(NCP))
                      for e in range(2)]
            low = row < 4
            direct = jnp.where(low, o0, o1)
            moved = jnp.where(low, pltpu.roll(o1, 8, 1), pltpu.roll(o0, 120, 1))
            o = jnp.where(((lane >> 1) & 4) == (row & 4), direct, moved)
            o = jnp.where((row & 3) == 0, o, 0.0) * li[s][0:1, :]
            ol[s][0] = _pack_rows(o)
            return o

        def wo_tile(wg, osrc, ydst, n):
            j, nt = divmod(n, KD)
            ydst[n] = _tile_dot(osrc[j], wg[nt, pl.ds(j * 64, 64), :])

        def y_fold(ysrc):
            for nt in range(KD):
                ysum[nt] = _tree_sum([ysum[nt]] + [ysrc[j * KD + nt] for j in range(NJ)])

        def kpair(i):
            return kb.at[pl.ds(i * RH, RH)]

        def wqpair(i):
            return wqb.at[pl.ds(i * NJ, NJ)]

        def wopair(i):
            r0 = i * (PD // 2)
            if not isinstance(i, int):
                r0 = pl.multiple_of(r0, PD // 2)
            return wob.at[:, pl.ds(r0, PD // 2), :]

        def mxu_kinds(a, first):
            b = 1 - a
            return dict(
                h=(CB * NT, lambda z: kpair(z + 1),
                   lambda w, n: qk_tile(w, ln[b], shi[b], CA, CB, n)),
                g=((CB - CM) * NT, lambda z: kpair(z + 1),
                   lambda w, n: qk_tile(w, ln[b], shi[b], CA + CM, CB - CM, n)),
                l=(CA * NT, lambda z: kpair(z + 2),
                   lambda w, n: qk_tile(w, ln[a], slo[a], 0, CA, n)),
                m=(CM * NT, lambda z: kpair(z + 2),
                   lambda w, n: qk_tile(w, ln[a], smid, CA, CM, n)),
                q=(NW, lambda z: (wqpair(jnp.minimum(z + 3, NP - 1)),
                                  cspair(jnp.minimum(z + 3, NP - 1)) if first else None),
                   lambda w, n: qproj_tile(w[0], qr[b], n, w[1])),
                w=(NW, lambda z: wopair(jnp.maximum(z - 2, 0)),
                   lambda w, n: wo_tile(w, ol[a], yr[a], n)),
                u=(NW, lambda z: wopair(z - 1),
                   lambda w, n: wo_tile(w, ol1, qr1, n)),
                v=(2 * KD, lambda z: wopair(z - 1),
                   lambda w, n: wo_tile(w, ol0, yr0, KD + n)),
                x=(4 * NCP, lambda z: vx.at[pl.ds((z - (NP - 1)) * 16, 16)], x_tile))

        def run_block(first, i, a, rg0, sets, order, rate, pace_n, side):
            if rg0:
                vg = vb.at[pl.ds((NP - 2) * RM + a * (RM - 8), RM - 8)]
            else:
                vg = vb.at[pl.ds(i * RM, RM)]
            sg = vs.at[pl.ds((i & 3) * (RF // 2), RF // 2)]
            fg = vf.at[pl.ds(i * RF, RF)]
            kinds = mxu_kinds(a, first)

            pace = dict(z=i, cnt=0, views={})

            def mxu_tile(key, n):
                if not first and pace["cnt"] % pace_n == 0:
                    for _ in range(pace_n * 4 // 3 if pace["cnt"] else D0):
                        pace["z"] = tbl[pace["z"]]
                    pace["views"] = {}
                pace["cnt"] += 1
                if key not in pace["views"]:
                    pace["views"][key] = kinds[key][1](pace["z"])
                kinds[key][2](pace["views"][key], n)

            mxu = [P(mxu_tile, key, n) for key in order for n in range(kinds[key][0])]
            side = sorted(side + [(int(n * rate), f) for n, f in enumerate(mxu)], key=lambda z: z[0])

            n_all = RP - rg0
            f0 = F0 * n_all // RP
            slots = sorted(f0 + (k + 1) * (n_all - f0) // RF - 1 for k in range(RF))
            todo = list(range(rg0, RP - RF))
            for k, pos in enumerate(slots):
                todo.insert(pos, RP - RF + k)
            cnt = 0
            acc = {}
            for size in (int(z) for z in sets.split(",")):
                rgs, todo = todo[:size], todo[size:]
                for cp in range(NCP):
                    mult = {hh: (pb[a][pl.ds(hh, 1), pl.ds(cp * 128, 128)],
                                 pb[a][pl.ds(4 + hh, 1), pl.ds(cp * 128, 128)])
                            for hh in sorted({rg // RH for rg in rgs})}
                    for rg in rgs:
                        while side and side[0][0] <= cnt:
                            side.pop(0)[1]()
                        cnt += 1
                        m0, m1 = mult[rg // RH]
                        r = rg - (RP - RF)
                        if r >= 0 and not first:
                            v0, v1 = fg[r, 2 * cp], fg[r, 2 * cp + 1]
                        else:
                            src = sg.at[r // 2, r % 2] if r >= 0 else vg.at[(rg - rg0) // 2, rg % 2]
                            v = src[pl.ds(cp * 16, 16), :].astype(f32)
                            v0, v1 = v[:8], v[8:]
                            if r >= 0:
                                fg[r, 2 * cp] = v0
                                fg[r, 2 * cp + 1] = v1
                        if rg in acc:
                            acc[rg] = acc[rg] + v0 * m0 + v1 * m1
                        else:
                            acc[rg] = v0 * m0 + v1 * m1
                        if cp == NCP - 1:
                            ac[a][rg] = acc[rg]
            assert not todo
            for _, f in side:
                f()

        def vpu_qk(nvq):
            row = lax.broadcasted_iota(jnp.int32, (8, 128), 0)
            for j in range(NJ):
                q = q_tile(qr2, j, cspair(0)).astype(bf16).astype(f32)
                for v, c in enumerate(_columns(q)):
                    ac0[16 * j + v] = c
            run = {}
            tot = {}
            for c0 in range(NCP - nvq, NCP, 2):
                for rg in range(RP):
                    col = ac0[rg]
                    for cp in range(c0, min(c0 + 2, NCP)):
                        kv = _widen(kb[rg // 2, rg % 2, pl.ds(cp * 8, 8), :])
                        for p in range(2):
                            key = (cp - c0, 4 * p + rg // RH)
                            _accum(run, key, kv[p] * col)
                            tot[cp, key[1]] = run[key]
            for cp in range(NCP - nvq, NCP):
                a_ = jnp.zeros((8, 128), f32)
                for r in (0, 1, 4, 5):
                    z = tot[cp, r] - tot[cp - 2, r] if (cp - 2, r) in tot else tot[cp, r]
                    a_ = jnp.where(row == r, _sublane_sum(z), a_)
                svq[cp - (NCP - nvq), 0] = a_

        def layer(x, guess):
            first = guess is None
            nvq = 0 if first else NVQ
            if first:
                xc, rs = _center(x)
                xl[...] = pltpu.bitcast(
                    jnp.concatenate([xc, jnp.ones_like(xc)], axis=0).astype(bf16), u32)
            else:
                xc = x - jnp.concatenate([guess] * KD, axis=1)
                xl[...] = _pack_rows(xc)
                dm = jnp.mean(xc, axis=-1, keepdims=True)
                var = jnp.maximum(jnp.mean(xc * xc, axis=-1, keepdims=True) - dm * dm, 0.0)
                rs = lax.rsqrt(var + EPS)
                dm_ref[...] = jnp.broadcast_to(dm, (8, 128))
            rd = (lambda i: None) if first else cspair
            wr = cspair if first else (lambda i: None)
            rs_ref[...] = jnp.broadcast_to(rs * c_exp, (8, 128))
            ac1[...] = jnp.zeros(ac1.shape, f32)
            li1[...] = jnp.zeros(li1.shape, f32)
            ol0[...] = jnp.zeros(ol0.shape, u32)
            yr1[...] = jnp.zeros(yr1.shape, f32)
            ysum[...] = jnp.zeros(ysum.shape, f32)

            for i, dst in enumerate((qr2, qr3, qr0)):
                for n in range(NW):
                    qproj_tile(wqpair(i), dst, n, wr(i))
            for j in range(NJ):
                build_l(qr2, lp, j, rd(0))
            for n in range(CA * NT):
                qk_tile(kpair(0), lp, slo0, 0, CA, n)
            for n in range((CB - nvq) * NT):
                qk_tile(kpair(0), lp, shi0, CA, CB - nvq, n)
            if nvq:
                vpu_qk(nvq)
            for j in range(NJ):
                build_l(qr3, ln1, j, rd(1))
            for n in range(CA * NT):
                qk_tile(kpair(1), ln1, slo1, 0, CA, n)
            softmax([(slo0, CA), (shi0, CB - nvq), (svq, nvq)], pb0, ls0)

            def block(i, a, order=MORD, rate=RATE, sets=SETS, pace_n=PACE):
                b = 1 - a
                cs = rd(i + 2)
                side = [(max(SPOS, int(CB * NT * rate) + 1),
                         P(softmax, [(slo[b], CA), (shi[b], CB)], pb[b], ls[b])),
                        (IPOS, P(l_inv, ls[a], li[a])),
                        (YPOS, P(y_fold, yr[b]))]
                for j in range(NJ):
                    side.append((LPOS + 10 * j, P(build_l, qr[a], ln[a], j, cs)))
                    side.append((RPOS + RSTEP * j, P(reduce_o, ac[b], li[b], ol[b], j)))
                run_block(first, i, a, 0, sets, order, rate, pace_n, side)

            def block14(i):
                side = [(int((CB - CM) * NT * RATE14) + 10,
                         P(softmax, [(slo1, CA), (smid, CM), (shi1, CB - CM)], pb1, ls1, pk1)),
                        (10, P(l_inv, ls0, li0)),
                        (100, P(pack_p, pb0, pk0)),
                        (5, P(y_fold, yr1))]
                side += [(100 + 10 * j, P(reduce_o, ac1, li1, ol1, j)) for j in range(NJ)]
                run_block(first, i, 0, 16, SETS14, "gwu", RATE14, PACE14, side)

            def block15(i):
                side = [(10, P(l_inv, ls1, li1)), (5, P(y_fold, yr0)), (25, P(y_fold, qr1))]
                side += [(100 + 10 * j, P(reduce_o, ac0, li0, ol0, j)) for j in range(1, NJ)]
                run_block(first, i, 1, 16, SETS15, "xv", RATE15, PACE15, side)

            def arrive(ch):
                for c in chunk(ch) + vstage(ch):
                    c.wait()
                for c in vstage(ch + 1):
                    c.start()

            def body(ch, one):
                if first:
                    arrive(ch)

                    @pl.when(ch + 2 < NC - 1)
                    def _():
                        for c in chunk(ch + 2):
                            c.start()

                    @pl.when(ch + 2 == NC - 1)
                    def _():
                        for c in vlast:
                            c.start()

                pl.when(one < 2)(P(block, 2 * ch, 0))
                pl.when(one > 0)(P(block, 2 * ch + 1, 1))
                return one

            one = lax.fori_loop(0, NC - 2, body, tbl[1])
            idx = (lambda i: i) if first else (lambda i: one * i)
            if first:
                arrive(NC - 2)
                for c in c1 + c2[0] + c2[1] + c2[2]:
                    c.start()
            block(idx(NP - 4), 0)
            pl.when(one > 0)(P(block, idx(NP - 3), 1, MORD13, RATE13, SETS13, PACE13))
            if first:
                for c in vlast + vstage(NC - 1):
                    c.wait()
            block14(idx(NP - 2))
            pl.when(one > 0)(P(block15, idx(NP - 1)))

            ox = [x_finish(0), x_finish(1)]
            for n in range(KD):
                wo_tile(wopair(NP - 2), ol0, yr0, n)
            for n in range(KD):
                wo_tile(wopair(NP - 1), ol1, qr0, n)
            wl = wopair(NP - 1)
            yv, mv = {}, {}
            for m in range(8, RH):
                ca, cb = [jnp.sum(ac1[rg], axis=1, keepdims=True) for rg in (2 * m, 2 * m + 1)]
                hh = 2 * m // RH
                for nt in range(KD):
                    wa, wb = _widen(wl[nt, pl.ds(8 * m, 8), :])
                    _accum(yv, (hh, nt), wa * ca + wb * cb)
                _accum(mv, hh, wsc[2 * m - 16] * ca + wsc[2 * m - 15] * cb)
            early = [_tree_sum([ysum[nt]] + [yr0[j * KD + nt] for j in range(1, NJ)])
                     for nt in range(KD)]
            ys = [_tree_sum([early[nt], yr0[nt], qr0[nt],
                             yv[0, nt] * li1[0:1, :], yv[1, nt] * li1[1:2, :]]) for nt in range(KD)]
            y = jnp.sum(jnp.concatenate(ys, axis=1), axis=0, keepdims=True)
            lanes = _tree_sum(early + [x[:, nt * 128:(nt + 1) * 128] * 0.125 for nt in range(KD)]
                              + [ox[0] * wsl[0], ox[1] * wsl[1]])
            tot = (jnp.sum(lanes, axis=1, keepdims=True)
                   + mv[0] * li1[0:1, :] + mv[1] * li1[1:2, :])
            mean = jnp.concatenate([_sublane_sum(tot) * (1.0 / D)] * KD, axis=1)
            x = x + y

            xc, rs = _center(x, mean)
            xn = _pack_rows(xc)
            if first:
                for c in c1:
                    c.wait()
            nv1 = 0 if first else NV1
            act = lambda h, n: _gelu(h * rs + b1v[n:n + 1, :].astype(f32))
            gs = {}
            for n in range(KF - nv1):
                gs[n] = act(_tree_sum(
                    _tile_dot(xn[:, kt * 128:(kt + 1) * 128], w1b[n, pl.ds(kt * 64, 64), :])
                    for kt in range(KD)), n)
            hv = {}
            for kt in range(KD if nv1 else 0):
                col = _columns(xc[:, kt * 128:(kt + 1) * 128])
                for v in range(8):
                    for n in range(KF - nv1, KF):
                        wa, wb = _widen(w1b[n, pl.ds(kt * 64 + 8 * v, 8), :])
                        _accum(hv, n, wa * col[2 * v] + wb * col[2 * v + 1])
            for n in hv:
                gs[n] = act(_sublane_sum(hv[n]), n)
            vk = range(W2SPLIT[1], KF) if first else range(NV2)
            cols = {kt: _columns(gs[kt]) for kt in vk}
            yv = {}
            parts = []
            for kt in range(KF):
                if first and kt == W2SPLIT[2]:
                    known = [_tree_sum([p[nt] for p in parts] + [x[:, nt * 128:(nt + 1) * 128],
                                                                 b2v[nt:nt + 1, :].astype(f32),
                                                                 _sublane_sum(yv.pop(nt))])
                             for nt in range(KD)]
                    guess = jnp.broadcast_to(
                        jnp.sum(_tree_sum(known), axis=1, keepdims=True) * (1.0 / D), (8, 128))
                if first and kt in W2SPLIT:
                    for c in c2[W2SPLIT.index(kt)]:
                        c.wait()
                if kt not in vk:
                    hk = _pack_rows(gs[kt])
                    parts.append([_tile_dot(hk, w2b[nt, pl.ds(kt * 64, 64), :]) for nt in range(KD)])
                    continue
                for v in range(8):
                    for nt in range(KD):
                        wa, wb = _widen(w2b[nt, pl.ds(kt * 64 + 8 * v, 8), :])
                        _accum(yv, nt, wa * cols[kt][2 * v] + wb * cols[kt][2 * v + 1])
            if first:
                return jnp.concatenate([known[nt] + _sublane_sum(yv[nt]) for nt in range(KD)], axis=1), guess
            y2 = jnp.concatenate(
                [_tree_sum([p[nt] for p in parts]
                           + [b2v[nt:nt + 1, :].astype(f32), _sublane_sum(yv[nt])])
                 for nt in range(KD)], axis=1)
            return x + y2

        for c in head:
            c.wait()

        def wo_rowsums(r0):
            w = _tree_sum(pltpu.bitcast(wob[nt, pl.ds(r0, 8), :], bf16).astype(f32) for nt in range(KD))
            return jnp.broadcast_to(jnp.sum(w, axis=1, keepdims=True), (16, 128))

        for m in range(8, RH):
            wsc[pl.ds(2 * m - 16, 2)] = wo_rowsums((NP - 1) * (PD // 2) + 8 * m).reshape(2, 8, 128)
        for s_ in range(2):
            rsum = jnp.concatenate([wo_rowsums((NP - 2 + s_) * (PD // 2) + 8 * m) for m in range(8)], axis=0)
            wsl[s_] = rsum.T[0:8]

        def transpose_tile(n, c):
            s8 = pl.multiple_of((n // (2 * NCP)) * 8, 8)
            e = n % 2
            c8 = pl.multiple_of(((n // 2) % NCP) * 8, 8)
            w = vx[pl.ds(s8, 8), e, pl.ds(c8, 8), :].reshape(64, 128)
            wt = pltpu.bitcast(w, bf16).astype(f32).T.astype(bf16)
            vx[pl.ds(s8, 8), e, pl.ds(c8, 8), :] = pltpu.bitcast(wt, u32).reshape(8, 8, 128)
            return c

        lax.fori_loop(0, 4 * NCP, transpose_tile, 0)

        x = jnp.broadcast_to(xin[0].astype(f32), (8, D))
        x, guess = layer(x, None)
        x = layer(x, guess)
        o_ref[0] = x[0:1, :].astype(o_ref.dtype)

    return kernel


@jax.jit
def pallas_interleave_layers__sliding_block_cached__dense_activation_gelu__decode_kernel(
    A_x, A_k_cache, A_v_cache, A_wq, A_wo, B_x, B_w1, B_b1, B_w2, B_b2,
):
    SK = A_k_cache.shape[2]
    W = min(4096, max(256, SK // 4))
    NR = H * DH // 8
    NCP = W // 256

    def tiled(a):
        t = jnp.swapaxes(a, 2, 3).reshape(NR, 8, SK // 128, 128)
        return t.transpose(0, 2, 1, 3).reshape(NR // 2, 2, SK // 16, 128)

    vreg = lambda n, dt: pltpu.VMEM(n + (8, 128), dt)
    return pl.pallas_call(
        _make_kernel(SK, W),
        out_shape=jax.ShapeDtypeStruct(A_x.shape, A_x.dtype),
        in_specs=[pl.BlockSpec(memory_space=pl.ANY)] * 9,
        out_specs=pl.BlockSpec(memory_space=pltpu.VMEM),
        scratch_shapes=[
            pltpu.VMEM((NR // 2, 2, W // 32, 128), u32),
            pltpu.VMEM((NR // 2 - 16 - NP * RF // 2, 2, W // 16, 128), bf16),
            pltpu.VMEM((2 * RF, 2, W // 16, 128), bf16),
            pltpu.VMEM((16, 2, W // 32, 128), u32),
            vreg((NP * RF, 2 * NCP), f32),
            pltpu.VMEM((H * DH // 128, D // 2, 128), u32),
            pltpu.VMEM((KD, H * DH // 2, 128), u32),
            pltpu.VMEM((KF, D // 2, 128), u32),
            pltpu.VMEM((KD, F // 2, 128), u32),
            pltpu.VMEM((1, 1, D), bf16),
            pltpu.VMEM((KF, 128), bf16),
            pltpu.VMEM((KD, 128), bf16),
            pltpu.VMEM((8, D), u32),
            pltpu.VMEM((8, 128), f32),
            pltpu.VMEM((8, 128), f32),
            vreg((NP * NJ,), f32),
            vreg((KD,), f32),
        ] + [vreg((NT,), u32)] * 3
          + [vreg((NW,), f32)] * 4
          + [vreg((CA, NT), f32)] * 2
          + [vreg((CM, NT), f32)]
          + [vreg((NCP - CA, NT), f32)] * 2
          + [pltpu.VMEM((8, NCP * 128), f32)] * 2
          + [pltpu.VMEM((8, 128), f32)] * 4
          + [vreg((RP,), f32)] * 2
          + [vreg((NJ,), u32)] * 2
          + [vreg((NW,), f32)] * 2
          + [vreg((NCP,), u32)] * 2
          + [vreg((32,), f32), vreg((2,), f32)]
          + [vreg((NVQ, 1), f32)]
          + [pltpu.SMEM((NP,), jnp.int32), pltpu.SemaphoreType.DMA((5,))],
        compiler_params=pltpu.CompilerParams(vmem_limit_bytes=128 * 1024 * 1024),
    )(A_x, tiled(A_k_cache), tiled(A_v_cache), A_wq, A_wo, B_w1,
      B_b1.reshape(KF, 128), B_w2, B_b2.reshape(KD, 128))
```
